```python
import jax
import jax.numpy as jnp

def _softmax(x, axis=-1):
    return jax.nn.softmax(x, axis=axis)

def _gelu(x):
    return jax.nn.gelu(x, approximate=True)

def _silu(x):
    return jax.nn.silu(x)

def _sigmoid(x):
    return jax.nn.sigmoid(x)

def _layernorm(x, axis=-1, eps=1e-05):
    m = jnp.mean(x, axis=axis, keepdims=True)
    v = jnp.var(x, axis=axis, keepdims=True)
    return (x - m) / jnp.sqrt(v + eps)

def _scatter_add(tgt, idx, src, axis=0):
    return tgt.at[idx].add(src)

def _segment_sum(src, seg, n):
    return jax.ops.segment_sum(src, seg, n)

class _Rng:

    def __init__(self, key):
        self._k = key

    def _next(self):
        self._k, sub = jax.random.split(self._k)
        return sub

    def normal(self, shape):
        return jax.random.normal(self._next(), shape, dtype=jnp.bfloat16)

    def randint(self, lo, hi, shape):
        return jax.random.randint(self._next(), shape, lo, hi, dtype=jnp.int32)

    def uniform(self, shape, lo=0.0, hi=1.0):
        return jax.random.uniform(self._next(), shape, jnp.bfloat16, lo, hi)

    def permutation(self, n):
        return jax.random.permutation(self._next(), n)
kernel_name = 'concat_heads__memory_aug_recurrent_mem_tr__ssm_conv_s4__prompt'

def setup_inputs():
    _rng = _Rng(jax.random.key(int.from_bytes(__import__("os").urandom(4), "little")))
    _w = lambda a: (lambda t: t.astype(jnp.bfloat16) if jnp.issubdtype(t.dtype, jnp.floating) else t)(jnp.asarray(a))

    def _A_setup():
        B, S, Dm = (1, 2048, 1024)
        H, Dh = (32, 128)
        M, seg = (8, 32)
        seg = min(seg, S)
        S = S // seg * seg
        return {'x': _w((lambda *s: _rng.normal(s) * 0.05)(B, S, Dm)), 'mem0': _w((lambda *s: _rng.normal(s) * 0.05)(B, M, Dm)), 'Wq': _w((lambda *s: _rng.normal(s) * 0.05)(Dm, H, Dh) * Dm ** (-0.5)), 'Wk': _w((lambda *s: _rng.normal(s) * 0.05)(Dm, H, Dh) * Dm ** (-0.5)), 'Wv': _w((lambda *s: _rng.normal(s) * 0.05)(Dm, H, Dh) * Dm ** (-0.5)), 'Wo': _w((lambda *s: _rng.normal(s) * 0.05)(H, Dh, Dm) * (H * Dh) ** (-0.5)), 'seg_len': seg}
    _A_in = _A_setup()

    def _B_setup():
        B, L, D, N = (1, 2048, 1024, 128)
        A_re = -jnp.exp((lambda *s: _rng.normal(s) * 0.05)(D, N))
        A_im = jnp.pi * (lambda *s: _rng.normal(s) * 0.05)(D, N)
        B_re = (lambda *s: _rng.normal(s) * 0.05)(D, N)
        B_im = (lambda *s: _rng.normal(s) * 0.05)(D, N)
        C_re = (lambda *s: _rng.normal(s) * 0.05)(D, N)
        C_im = (lambda *s: _rng.normal(s) * 0.05)(D, N)
        log_dt = (lambda *s: _rng.normal(s) * 0.05)(D) * 0.5 - 4.0
        Dskip = (lambda *s: _rng.normal(s) * 0.05)(D)
        return {'u': _w((lambda *s: _rng.normal(s) * 0.05)(B, L, D)), 'A_re': _w(A_re), 'A_im': _w(A_im), 'B_re': _w(B_re), 'B_im': _w(B_im), 'C_re': _w(C_re), 'C_im': _w(C_im), 'log_dt': _w(log_dt), 'Dskip': _w(Dskip)}
    _B_in = _B_setup()
    return {'A_x': _A_in['x'], 'A_mem0': _A_in['mem0'], 'A_Wq': _A_in['Wq'], 'A_Wk': _A_in['Wk'], 'A_Wv': _A_in['Wv'], 'A_Wo': _A_in['Wo'], 'A_seg_len': _A_in['seg_len'], 'B_u': _B_in['u'], 'B_A_re': _B_in['A_re'], 'B_A_im': _B_in['A_im'], 'B_B_re': _B_in['B_re'], 'B_B_im': _B_in['B_im'], 'B_C_re': _B_in['C_re'], 'B_C_im': _B_in['C_im'], 'B_log_dt': _B_in['log_dt'], 'B_Dskip': _B_in['Dskip']}

def reference(A_x, A_mem0, A_Wq, A_Wk, A_Wv, A_Wo, A_seg_len, B_u, B_A_re, B_A_im, B_B_re, B_B_im, B_C_re, B_C_im, B_log_dt, B_Dskip):

    def _A_ref(x, mem0, Wq, Wk, Wv, Wo, seg_len):
        B, S, Dm = x.shape
        H, Dh = (Wq.shape[1], Wq.shape[2])
        M = mem0.shape[1]
        scale = Dh ** (-0.5)
        n_seg = S // seg_len
        L = M + seg_len
        idx = jnp.arange(L)
        mask = (idx[:, None] < M) | (idx[:, None] >= idx[None, :])
        mem = mem0
        outs = []
        for s in range(n_seg):
            xs = x[:, s * seg_len:(s + 1) * seg_len, :].copy()
            h = jnp.concatenate([mem, xs], axis=1)
            q = jnp.einsum('btd,dhe->bhte', h, Wq)
            k = jnp.einsum('btd,dhe->bhte', h, Wk)
            v = jnp.einsum('btd,dhe->bhte', h, Wv)
            scores = jnp.einsum('bhqe,bhke->bhqk', q, k) * scale
            scores = jnp.where(mask[None, None], scores, -1000000000.0)
            p = _softmax(scores, axis=-1)
            o = jnp.einsum('bhqk,bhke->bhqe', p, v)
            o = jnp.einsum('bhte,hed->btd', o, Wo)
            mem = o[:, :M, :].copy()
            outs.append(o[:, M:, :])
        return jnp.concatenate(outs, axis=1)

    def _B_ref(u, A_re, A_im, B_re, B_im, C_re, C_im, log_dt, Dskip):
        Bsz, L, D = u.shape
        dt = jnp.exp(log_dt)[:, None]
        A = A_re + 1j * A_im
        Bc = B_re + 1j * B_im
        Cc = C_re + 1j * C_im
        logdA = dt * A
        dB = dt * Bc
        l = (lambda x, dt: x.astype(dt))(jnp.arange(L), A_re.dtype)
        P = jnp.exp(logdA[:, :, None] * l[None, None, :])
        K = jnp.einsum('dn,dnl,dn->dl', Cc, P, dB).real
        L2 = 2 * L
        Kp = jnp.pad(K, ((0, 0), (0, L)))
        up = (lambda x, *d: x.transpose(*d))(u, 0, 2, 1)
        up = jnp.pad(up, ((0, 0), (0, 0), (0, L)))
        Kf = (lambda x, axes=(-2, -1): jnp.fft.rfft2(x.astype(jnp.float32), axes=axes))(Kp[:, None, :], axes=(-2, -1))
        Uf = (lambda x, axes=(-2, -1): jnp.fft.rfft2(x.astype(jnp.float32), axes=axes))(up[:, :, None, :], axes=(-2, -1))
        Yf = Uf * Kf[None, :, :, :]
        y = (lambda x, s, axes=(-2, -1): jnp.fft.irfft2(x, s=s, axes=axes).astype(jnp.bfloat16))(Yf, (1, L2), axes=(-2, -1))[:, :, 0, :L]
        y = (lambda x, *d: x.transpose(*d))(y, 0, 2, 1) + u * Dskip[None, None, :]
        return y
    a = _A_ref(A_x, A_mem0, A_Wq, A_Wk, A_Wv, A_Wo, A_seg_len)
    b = _B_ref(B_u, B_A_re, B_A_im, B_B_re, B_B_im, B_C_re, B_C_im, B_log_dt, B_Dskip)
    return jnp.concatenate([a, b], axis=-1)
```

```python
import functools

import jax
import jax.numpy as jnp
from jax import lax
import jax.experimental.pallas as pl
import jax.experimental.pallas.tpu as pltpu

F32 = jnp.float32
BF16 = jnp.bfloat16
U32 = jnp.uint32

NN = (((1,), (0,)), ((), ()))
NT = (((1,), (1,)), ((), ()))

T = 128
GC = 128
PITCH = 17
BPITCH = 9


def _dot(a, b, dims=NN):
    return lax.dot_general(a, b, dims, preferred_element_type=F32)


def _kernel(x_hbm, mem0_ref, wq_hbm, wk_hbm, wv_hbm, wo_hbm,
            u_hbm, are_hbm, aim_hbm, bre_hbm, bim_hbm, cre_hbm, cim_hbm, ldt_ref, dsk_ref,
            out_hbm,
            x_v, u_v, par_v, stage_w, stage_o, wqkv_v, wo_v, outa_v, outb_v,
            h_v, o_v,
            bre_v, bim_v, mu_v, cf_v, uf_v, ur_v, sre_v, sim_v, y_v,
            sem_x, sem_u, sem_par, sem_w, sem_oa, sem_ob,
            *, seg, n_mem, n_heads, cb, lag, do_a, do_b):
    S, Dm = x_v.shape
    D = Dm
    n_groups = D // GC
    n_chunks = S // T
    n_seg = S // seg
    L = n_mem + seg
    Dh = 128
    DC = Dm // n_groups
    RO = n_heads * Dh // n_groups
    n_slots = stage_w.shape[0]
    n_hg = n_heads // 8

    def w_copies(g, slot):
        cps = []
        for i, w in enumerate((wq_hbm, wk_hbm, wv_hbm)):
            for hg in range(n_hg):
                cps.append(pltpu.make_async_copy(
                    w.at[pl.ds(pl.multiple_of(g * (DC * 8), DC * 8), DC * 8), pl.ds(128 * hg, 128)],
                    stage_w.at[slot, i * n_hg + hg],
                    sem_w.at[slot]))
        cps.append(pltpu.make_async_copy(
            wo_hbm.at[pl.ds(pl.multiple_of(g * RO, RO), RO), :], stage_o.at[slot], sem_w.at[slot]))
        return cps

    def u_copy(g):
        return pltpu.make_async_copy(
            u_hbm.at[:, pl.ds(pl.multiple_of(g * GC, GC), GC)], u_v.at[g], sem_u.at[g])

    def par_copies():
        return [pltpu.make_async_copy(p, par_v.at[i], sem_par)
                for i, p in enumerate((are_hbm, aim_hbm, bre_hbm, bim_hbm, cre_hbm, cim_hbm))]

    def outb_copy(g):
        return pltpu.make_async_copy(
            outb_v.at[g], out_hbm.at[:, pl.ds(pl.multiple_of(Dm + g * GC, GC), GC)], sem_ob)

    def outa_copy(s):
        r = pl.ds(pl.multiple_of(s * seg, seg), seg)
        return pltpu.make_async_copy(outa_v.at[r, :], out_hbm.at[r, pl.ds(0, Dm)], sem_oa)

    x_copy = pltpu.make_async_copy(x_hbm, x_v, sem_x)

    for cp in par_copies():
        cp.start()
    for g in range(n_slots):
        u_copy(g).start()
        for cp in w_copies(g, g):
            cp.start()

    def relayout(g, slot):
        for i in range(3):
            for hg in range(n_hg):
                src = stage_w.at[slot, i * n_hg + hg].bitcast(U32)
                for pp in range(4):
                    ev = src[pl.ds(pp, DC // 2, stride=8), :]
                    od = src[pl.ds(pp + 4, DC // 2, stride=8), :]
                    h = hg * 8 + 2 * pp
                    rows = pl.ds(pl.multiple_of(g * (DC // 2), DC // 2), DC // 2)
                    wqkv_v[h * 3 + i, rows, :] = (ev & 0xFFFF) | (od << 16)
                    wqkv_v[(h + 1) * 3 + i, rows, :] = (ev >> 16) | (od & jnp.uint32(0xFFFF0000))
        for j in range(Dm // 128):
            rows = pl.ds(pl.multiple_of(g * (RO // 2), RO // 2), RO // 2)
            wo_v[j, rows, :] = pltpu.bitcast(stage_o[slot, :, 128 * j:128 * (j + 1)], U32)

    def cmul(ar, ai, br, bi):
        return ar * br - ai * bi, ar * bi + ai * br

    n_it = GC // cb

    def ssm_group(g, ldt_all, dsk_all):
        rows = pl.ds(pl.multiple_of(g * GC, GC), GC)
        sel = lax.broadcasted_iota(jnp.int32, (n_groups, GC), 0) == g
        ldt = jnp.sum(jnp.where(sel, ldt_all, 0.0), axis=0, keepdims=True)
        dsk = jnp.sum(jnp.where(sel, dsk_all, 0.0), axis=0, keepdims=True)
        dt_row = jnp.exp(ldt).astype(BF16).astype(F32)
        dt = jnp.broadcast_to(dt_row, (GC, GC)).T
        zr = dt * par_v[0, rows, :].astype(F32)
        zi = dt * par_v[1, rows, :].astype(F32)
        c_re, c_im = cmul(par_v[4, rows, :].astype(F32), par_v[5, rows, :].astype(F32),
                          dt * par_v[2, rows, :].astype(F32), dt * par_v[3, rows, :].astype(F32))
        mag = jnp.exp(zr)
        l1 = (mag * jnp.cos(zi), mag * jnp.sin(zi))
        l2 = cmul(*l1, *l1)
        l3 = cmul(*l2, *l1)
        l4 = cmul(*l2, *l2)
        pw = [(jnp.ones_like(mag), jnp.zeros_like(mag)), l1, l2, l3, l4,
              cmul(*l4, *l1), cmul(*l4, *l2), cmul(*l4, *l3)]
        for it in range(n_it):
            sl = slice(it * cb, (it + 1) * cb)
            for r in range(8):
                bre_v[it, pl.ds(r, cb, stride=BPITCH), :] = pw[r][0][sl]
                bim_v[it, pl.ds(r, cb, stride=BPITCH), :] = pw[r][1][sl]
        l8 = cmul(*l4, *l4)
        for it in range(n_it):
            sl = slice(it * cb, (it + 1) * cb)
            mu_v[0, it] = l8[0][sl]
            mu_v[1, it] = l8[1][sl]
        lt = l8
        for _ in range(4):
            lt = cmul(*lt, *lt)
        cl = cmul(c_re, c_im, *l1)

        ri = lax.broadcasted_iota(jnp.int32, (T, T), 0)
        ci = lax.broadcasted_iota(jnp.int32, (T, T), 1)
        flip = jnp.where(ri + ci == T - 1, 1.0, 0.0).astype(BF16)
        for c in range(n_chunks):
            ut = u_v[g, c * T:(c + 1) * T, :].astype(F32).T
            urev = _dot(ut, flip)
            for it in range(n_it):
                sl = slice(it * cb, (it + 1) * cb)
                uf_v[it, pl.ds(c, cb, stride=PITCH), :] = ut[sl]
                ur_v[it, pl.ds(c, cb, stride=PITCH), :] = urev[sl]

        cf_v[0] = lt[0]
        cf_v[1] = lt[1]
        cf_v[2] = cl[0]
        cf_v[3] = cl[1]
        cf_v[4] = c_re
        cf_v[5] = c_im

        row8 = lax.broadcasted_iota(jnp.int32, (8, 128), 0)
        lane8 = lax.broadcasted_iota(jnp.int32, (8, 128), 1)
        masks = []
        for m in range(T // 16):
            first = 16 * m + 2 * row8
            masks.append(jnp.where(lane8 > first, jnp.uint32(0xFFFFFFFF),
                                   jnp.where(lane8 == first, jnp.uint32(0xFFFF), jnp.uint32(0))))
        not_first = lax.broadcasted_iota(jnp.int32, (n_chunks, 128), 0) > 0

        def batch(it, carry):
            ps = []
            for k in range(cb):
                pr = [bre_v[it, k * BPITCH:k * BPITCH + 8, :]]
                pi = [bim_v[it, k * BPITCH:k * BPITCH + 8, :]]
                mr = jnp.broadcast_to(mu_v[0, it, k:k + 1, :], (8, 128))
                mi = jnp.broadcast_to(mu_v[1, it, k:k + 1, :], (8, 128))
                for _ in range(T // 8 - 1):
                    nr, ni = cmul(pr[-1], pi[-1], mr, mi)
                    pr.append(nr)
                    pi.append(ni)
                p_re = jnp.concatenate(pr, axis=0).astype(BF16)
                p_im = jnp.concatenate(pi, axis=0).astype(BF16)
                ps.append((p_re, p_im))
                r = slice(k * PITCH, k * PITCH + n_chunks)
                urev = ur_v[it, r, :]
                sre_v[it, r, :] = _dot(urev, p_re)
                sim_v[it, r, :] = _dot(urev, p_im)

            sl = pl.ds(pl.multiple_of(it * cb, cb), cb)
            ltr, lti, clr, cli, gr, gi = (cf_v[i, sl, :] for i in range(6))
            for c in range(n_chunks):
                idx = pl.ds(c, cb, stride=PITCH)
                if c < n_chunks - 1:
                    sr, si = cmul(sre_v[it, idx, :], sim_v[it, idx, :], clr, cli)
                sre_v[it, idx, :] = gr
                sim_v[it, idx, :] = -gi
                if c == 0:
                    gr, gi = sr, si
                elif c < n_chunks - 1:
                    gr, gi = cmul(gr, gi, ltr, lti)
                    gr, gi = gr + sr, gi + si

            ys = {}
            for k in range(cb + lag):
                if k < cb:
                    r = slice(k * PITCH, k * PITCH + n_chunks)
                    ys[k] = _dot(sre_v[it, r, :], ps[k][0], NT) + _dot(sim_v[it, r, :], ps[k][1], NT)
                if k >= lag:
                    r = slice((k - lag) * PITCH, (k - lag) * PITCH + n_chunks)
                    y = ys.pop(k - lag)
                    kb = jnp.broadcast_to(y[0:1, :], (8, 128))
                    base = jnp.concatenate(
                        [pltpu.roll(kb, 0, 1, stride=1, stride_axis=0),
                         pltpu.roll(kb, 8, 1, stride=1, stride_axis=0)], axis=0).astype(BF16)
                    base = pltpu.bitcast(base, U32)
                    tz = [base & masks[0]]
                    for m in range(1, T // 16):
                        tz.append(pltpu.roll(base, 16 * m, 1) & masks[m])
                    tz = pltpu.bitcast(jnp.concatenate(tz, axis=0), BF16)
                    y_v[it, r, :] = _dot(uf_v[it, r, :], tz) + jnp.where(not_first, y, 0.0)
            return carry

        lax.fori_loop(0, n_it, batch, 0)

        for c in range(n_chunks):
            yc = jnp.concatenate([y_v[it, pl.ds(c, cb, stride=PITCH), :] for it in range(n_it)], axis=0)
            yc = yc.T.astype(BF16).astype(F32)
            skip = (u_v[g, c * T:(c + 1) * T, :].astype(F32) * dsk).astype(BF16).astype(F32)
            outb_v[g, c * T:(c + 1) * T, :] = (yc + skip).astype(BF16)

    ldt_all = ldt_ref[...].astype(F32).reshape(n_groups, GC)
    dsk_all = dsk_ref[...].astype(F32).reshape(n_groups, GC)
    for cp in par_copies():
        cp.wait()

    def phase1(g, carry):
        slot = lax.rem(g, n_slots)
        u_copy(g).wait()
        if do_b:
            ssm_group(g, ldt_all, dsk_all)
        else:
            outb_v[g] = u_v[g]
        for cp in w_copies(g, slot):
            cp.wait()
        relayout(g, slot)

        @pl.when(g + n_slots < n_groups)
        def _():
            u_copy(g + n_slots).start()
            for cp in w_copies(g + n_slots, slot):
                cp.start()

        @pl.when(g + n_slots == n_groups)
        def _():
            x_copy.start()
        return carry

    lax.fori_loop(0, n_groups, phase1, 0)
    for g in range(n_groups):
        outb_copy(g).start()
    x_copy.wait()

    scale = Dh ** -0.5
    qi = lax.broadcasted_iota(jnp.int32, (L, 128), 0)
    ki = lax.broadcasted_iota(jnp.int32, (L, 128), 1)
    keep = (qi < n_mem) | (qi >= ki)
    fill = jnp.where(ki < L, -1000000000.0, -jnp.inf)
    keep = keep & (ki < L)
    zpad = jnp.zeros((128 - L, Dh), F32)

    def proj(h, i):
        return _dot(h_v[...], pltpu.bitcast(wqkv_v[h * 3 + i], BF16))

    def step(s, carry):
        r = pl.ds(pl.multiple_of(s * seg, seg), seg)
        h_v[n_mem:, :] = x_v[r, :].astype(F32)
        qs, ks, vs, es = {}, {}, {}, {}
        HG = 8
        n_og = n_heads // HG

        def scores(h):
            sc = _dot(qs.pop(h), ks.pop(h), NT)
            sc = jnp.where(keep, sc * scale, fill)
            e = jnp.exp(sc - jnp.max(sc, axis=1, keepdims=True))
            es[h] = (e, 1.0 / jnp.sum(e, axis=1, keepdims=True))

        def mix(h):
            e, inv = es.pop(h)
            o_v[:, h * Dh:(h + 1) * Dh] = _dot(e, vs.pop(h)) * inv

        def oproj(j, g):
            w = pltpu.bitcast(wo_v[j, g * HG * Dh // 2:(g + 1) * HG * Dh // 2, :], BF16)
            return _dot(o_v[:, g * HG * Dh:(g + 1) * HG * Dh], w)

        def emit(j, res):
            h_v[:n_mem, 128 * j:128 * (j + 1)] = res[:n_mem]
            outa_v[r, 128 * j:128 * (j + 1)] = res[n_mem:].astype(BF16)

        for h in range(n_heads):
            qs[h] = proj(h, 0)
            if h >= 1:
                scores(h - 1)
            ks[h] = jnp.concatenate([proj(h, 1), zpad], axis=0).astype(BF16)
            if h >= 2:
                mix(h - 2)
            vs[h] = jnp.concatenate([proj(h, 2), zpad], axis=0).astype(BF16)
        a0 = oproj(0, 0)
        scores(n_heads - 1)
        a0 = a0 + oproj(0, 1)
        mix(n_heads - 2)
        a0 = a0 + oproj(0, 2)
        a1 = oproj(1, 0)
        a1 = a1 + oproj(1, 1)
        mix(n_heads - 1)
        a1 = a1 + oproj(1, 2)
        a2 = oproj(2, 0)
        a2 = a2 + oproj(2, 1)
        emit(0, a0 + oproj(0, 3))
        emit(1, a1 + oproj(1, 3))
        emit(2, a2 + oproj(2, 2) + oproj(2, 3))
        for j in range(3, Dm // 128):
            acc = oproj(j, 0)
            for g in range(1, n_og):
                acc = acc + oproj(j, g)
            emit(j, acc)
        outa_copy(s).start()
        return carry

    h_v[:n_mem, :] = mem0_ref[...].astype(F32)
    if do_a:
        lax.fori_loop(0, n_seg, step, 0)
    else:
        def dummy(s, carry):
            r = pl.ds(pl.multiple_of(s * seg, seg), seg)
            outa_v[r, :] = x_v[r, :]
            outa_copy(s).start()
            return carry
        lax.fori_loop(0, n_seg, dummy, 0)

    for g in range(n_groups):
        outb_copy(g).wait()

    def drain(s, carry):
        outa_copy(s).wait()
        return carry
    lax.fori_loop(0, n_seg, drain, 0)


@functools.partial(jax.jit, static_argnames=("A_seg_len", "cb", "lag", "do_a", "do_b"))
def pallas_concat_heads__memory_aug_recurrent_mem_tr__ssm_conv_s4__prompt_kernel(A_x, A_mem0, A_Wq, A_Wk, A_Wv, A_Wo, A_seg_len, B_u, B_A_re, B_A_im, B_B_re, B_B_im,
           B_C_re, B_C_im, B_log_dt, B_Dskip, cb=32, lag=32, do_a=True, do_b=True):
    Bsz, S, Dm = A_x.shape
    H, Dh = A_Wq.shape[1], A_Wq.shape[2]
    M = A_mem0.shape[1]
    D, N = B_A_re.shape
    seg = int(A_seg_len)
    assert Bsz == 1 and Dh == 128 and N == 128 and D == Dm and B_u.shape == A_x.shape
    L = M + seg
    n_groups = D // GC
    n_chunks = S // T
    n_it = GC // cb
    n_slots = 3
    DC = Dm // n_groups

    def head_tiles(w):
        return w.reshape(Dm, H // 8, 8, Dh).transpose(0, 2, 1, 3).reshape(Dm * 8, H // 8 * Dh)

    any_spec = pl.BlockSpec(memory_space=pl.ANY)
    vmem_spec = pl.BlockSpec(memory_space=pltpu.VMEM)
    out = pl.pallas_call(
        functools.partial(_kernel, seg=seg, n_mem=M, n_heads=H, cb=cb, lag=lag, do_a=do_a, do_b=do_b),
        out_shape=jax.ShapeDtypeStruct((S, Dm + D), BF16),
        in_specs=[any_spec, vmem_spec] + [any_spec] * 11 + [vmem_spec, vmem_spec],
        out_specs=any_spec,
        scratch_shapes=[
            pltpu.VMEM((S, Dm), BF16),
            pltpu.VMEM((n_groups, S, GC), BF16),
            pltpu.VMEM((6, D, N), BF16),
            pltpu.VMEM((n_slots, 3 * H // 8, DC * 8, 128), BF16),
            pltpu.VMEM((n_slots, H * Dh // n_groups, Dm), BF16),
            pltpu.VMEM((3 * H, Dm // 2, Dh), U32),
            pltpu.VMEM((Dm // 128, H * Dh // 2, 128), U32),
            pltpu.VMEM((S, Dm), BF16),
            pltpu.VMEM((n_groups, S, GC), BF16),
            pltpu.VMEM((L, Dm), F32),
            pltpu.VMEM((L, H * Dh), F32),
            pltpu.VMEM((n_it, cb * BPITCH, N), F32),
            pltpu.VMEM((n_it, cb * BPITCH, N), F32),
            pltpu.VMEM((2, n_it, cb, N), F32),
            pltpu.VMEM((6, GC, N), F32),
            pltpu.VMEM((n_it, cb * PITCH, T), F32),
            pltpu.VMEM((n_it, cb * PITCH, T), F32),
            pltpu.VMEM((n_it, cb * PITCH, N), F32),
            pltpu.VMEM((n_it, cb * PITCH, N), F32),
            pltpu.VMEM((n_it, cb * PITCH, T), F32),
            pltpu.SemaphoreType.DMA(()),
            pltpu.SemaphoreType.DMA((n_groups,)),
            pltpu.SemaphoreType.DMA(()),
            pltpu.SemaphoreType.DMA((n_slots,)),
            pltpu.SemaphoreType.DMA(()),
            pltpu.SemaphoreType.DMA(()),
        ],
        compiler_params=pltpu.CompilerParams(vmem_limit_bytes=110 * 1024 * 1024),
    )(A_x.reshape(S, Dm), A_mem0.reshape(M, Dm), head_tiles(A_Wq), head_tiles(A_Wk), head_tiles(A_Wv),
      A_Wo.reshape(H * Dh, Dm), B_u.reshape(S, D), B_A_re, B_A_im, B_B_re, B_B_im, B_C_re, B_C_im,
      B_log_dt, B_Dskip)
    return out.reshape(Bsz, S, Dm + D)
```

```python
import functools

import jax
import jax.numpy as jnp
from jax import lax
import jax.experimental.pallas as pl
import jax.experimental.pallas.tpu as pltpu

F32 = jnp.float32
BF16 = jnp.bfloat16
U32 = jnp.uint32

NN = (((1,), (0,)), ((), ()))
NT = (((1,), (1,)), ((), ()))

T = 128
TC = T // 2
GC = 128
PITCH = 17
SPITCH = 33
BPITCH = 9


def _dot(a, b, dims=NN):
    return lax.dot_general(a, b, dims, preferred_element_type=F32)


def _kernel(x_hbm, mem0_ref, wq_hbm, wk_hbm, wv_hbm, wo_hbm,
            u_hbm, are_hbm, aim_hbm, bre_hbm, bim_hbm, cre_hbm, cim_hbm, ldt_ref, dsk_ref,
            out_hbm,
            x_v, u_v, par_v, stage_w, stage_o, wqkv_v, wo_v, outa_v, outb_v,
            h_v, o_v,
            bre_v, bim_v, cf_v, p_v, uf_v, ur_v, sre_v, sim_v, gre_v, gim_v, y_v, taps_v,
            sem_x, sem_u, sem_par, sem_w, sem_oa, sem_ob,
            *, seg, n_mem, n_heads, cb, lag, mode, fill_n, unroll, do_a, do_b):
    S, Dm = x_v.shape
    D = Dm
    n_groups = D // GC
    n_chunks = S // T
    n_seg = S // seg
    L = n_mem + seg
    Dh = 128
    DC = Dm // n_groups
    RO = n_heads * Dh // n_groups
    n_slots = stage_w.shape[0]
    n_hg = n_heads // 8

    def w_copies(g, slot):
        cps = []
        for i, w in enumerate((wq_hbm, wk_hbm, wv_hbm)):
            for hg in range(n_hg):
                cps.append(pltpu.make_async_copy(
                    w.at[pl.ds(pl.multiple_of(g * (DC * 8), DC * 8), DC * 8), pl.ds(128 * hg, 128)],
                    stage_w.at[slot, i * n_hg + hg],
                    sem_w.at[slot]))
        cps.append(pltpu.make_async_copy(
            wo_hbm.at[pl.ds(pl.multiple_of(g * RO, RO), RO), :], stage_o.at[slot], sem_w.at[slot]))
        return cps

    def u_copy(g):
        return pltpu.make_async_copy(
            u_hbm.at[:, pl.ds(pl.multiple_of(g * GC, GC), GC)], u_v.at[g], sem_u.at[g])

    def par_copies():
        return [pltpu.make_async_copy(p, par_v.at[i], sem_par)
                for i, p in enumerate((are_hbm, aim_hbm, bre_hbm, bim_hbm, cre_hbm, cim_hbm))]

    def outb_copy(g):
        return pltpu.make_async_copy(
            outb_v.at[g], out_hbm.at[:, pl.ds(pl.multiple_of(Dm + g * GC, GC), GC)], sem_ob)

    def outa_copy(s):
        r = pl.ds(pl.multiple_of(s * seg, seg), seg)
        return pltpu.make_async_copy(outa_v.at[r, :], out_hbm.at[r, pl.ds(0, Dm)], sem_oa)

    x_copy = pltpu.make_async_copy(x_hbm, x_v, sem_x)

    for cp in par_copies():
        cp.start()
    u_copy(0).start()
    u_copy(1).start()

    def relayout(g, slot):
        def qkv_piece(t, carry):
            i = t // n_hg
            hg = t - i * n_hg
            src = stage_w.at[slot, t].bitcast(U32)
            rows = pl.ds(pl.multiple_of(g * (DC // 2), DC // 2), DC // 2)
            for pp in range(4):
                ev = src[pl.ds(pp, DC // 2, stride=8), :]
                od = src[pl.ds(pp + 4, DC // 2, stride=8), :]
                m = (hg * 8 + 2 * pp) * 3 + i
                wqkv_v[m, rows, :] = (ev & 0xFFFF) | (od << 16)
                wqkv_v[m + 3, rows, :] = (ev >> 16) | (od & jnp.uint32(0xFFFF0000))
            return carry

        lax.fori_loop(0, 3 * n_hg, qkv_piece, 0)

        def o_piece(t, carry):
            src = pl.ds(pl.multiple_of(t * 64, 64), 64)
            dst = pl.ds(pl.multiple_of(g * (RO // 2) + t * 32, 32), 32)
            for j in range(Dm // 128):
                wo_v[j, dst, :] = pltpu.bitcast(stage_o[slot, src, 128 * j:128 * (j + 1)], U32)
            return carry

        lax.fori_loop(0, RO // 64, o_piece, 0)

    def cmul(ar, ai, br, bi):
        return ar * br - ai * bi, ar * bi + ai * br

    n_it = GC // cb

    def ssm_group(g, ldt_all, dsk_all):
        rows = pl.ds(pl.multiple_of(g * GC, GC), GC)
        sel = lax.broadcasted_iota(jnp.int32, (n_groups, GC), 0) == g
        ldt = jnp.sum(jnp.where(sel, ldt_all, 0.0), axis=0, keepdims=True)
        dsk = jnp.sum(jnp.where(sel, dsk_all, 0.0), axis=0, keepdims=True)
        dt_row = jnp.exp(ldt).astype(BF16).astype(F32)
        dt = jnp.broadcast_to(dt_row, (GC, GC)).T
        zr = dt * par_v[0, rows, :].astype(F32)
        zi = dt * par_v[1, rows, :].astype(F32)
        c_re, c_im = cmul(par_v[4, rows, :].astype(F32), par_v[5, rows, :].astype(F32),
                          dt * par_v[2, rows, :].astype(F32), dt * par_v[3, rows, :].astype(F32))
        mag = jnp.exp(zr)
        l1 = (mag * jnp.cos(zi), mag * jnp.sin(zi))
        l2 = cmul(*l1, *l1)
        l3 = cmul(*l2, *l1)
        l4 = cmul(*l2, *l2)
        pw = [(jnp.ones_like(mag), jnp.zeros_like(mag)), l1, l2, l3, l4,
              cmul(*l4, *l1), cmul(*l4, *l2), cmul(*l4, *l3)]
        its = [slice(it * cb, (it + 1) * cb) for it in range(n_it)]
        for it, sl in enumerate(its):
            for r in range(8):
                bre_v[it, pl.ds(r, cb, stride=BPITCH), :] = pw[r][0][sl]
                bim_v[it, pl.ds(r, cb, stride=BPITCH), :] = pw[r][1][sl]
        l8 = cmul(*l4, *l4)
        lt = l8
        for _ in range(3):
            lt = cmul(*lt, *lt)
        cl = cmul(c_re, c_im, *l1)
        for i, val in enumerate((lt[0], -lt[1], cl[0], cl[1], c_re, -c_im, *l8)):
            for it, sl in enumerate(its):
                cf_v[it, i] = val[sl]

        ri = lax.broadcasted_iota(jnp.int32, (T, T), 0)
        ci = lax.broadcasted_iota(jnp.int32, (T, T), 1)
        flip = jnp.where((ri ^ ci) == TC - 1, 1.0, 0.0).astype(BF16)

        def u_chunks(q, carry):
            nq = 4
            uts = [u_v[g, pl.ds(pl.multiple_of((q * nq + c) * T, T), T), :].astype(F32).T for c in range(nq)]
            urev = _dot(jnp.concatenate(uts, axis=0), flip)
            for c in range(nq):
                for it, sl in enumerate(its):
                    idx = pl.ds(q * nq + c, cb, stride=PITCH)
                    uf_v[it, idx, :] = uts[c][sl]
                    ur_v[it, idx, :] = urev[c * GC + it * cb:c * GC + (it + 1) * cb]
            return carry

        lax.fori_loop(0, n_chunks // 4, u_chunks, 0)

        def chan(k):
            return slice(k * PITCH, k * PITCH + n_chunks)

        def states(k):
            return slice(k * SPITCH, k * SPITCH + 2 * n_chunks)

        even = lax.broadcasted_iota(jnp.int32, (n_chunks, T), 1) < TC

        def state_in(it, carry):
            for k in range(cb):
                pr = [bre_v[it, k * BPITCH:k * BPITCH + 8, :]]
                pi = [bim_v[it, k * BPITCH:k * BPITCH + 8, :]]
                mr = jnp.broadcast_to(cf_v[it, 6, k:k + 1, :], (8, 128))
                mi = jnp.broadcast_to(cf_v[it, 7, k:k + 1, :], (8, 128))
                for _ in range(TC // 8 - 1):
                    nr, ni = cmul(pr[-1], pi[-1], mr, mi)
                    pr.append(nr)
                    pi.append(ni)
                p_v[it, k] = jnp.concatenate(
                    [jnp.concatenate(pr, axis=0), jnp.concatenate(pi, axis=0)], axis=1).astype(BF16)
                ur = ur_v[it, chan(k), :]
                ur = jnp.concatenate([jnp.where(even, ur, 0.0), jnp.where(even, 0.0, ur)], axis=0)
                sre_v[it, states(k), :] = _dot(ur, jnp.concatenate(pr + pr, axis=0).astype(BF16))
                sim_v[it, states(k), :] = _dot(ur, jnp.concatenate(pi + pi, axis=0).astype(BF16))
            return carry

        lax.fori_loop(0, n_it, state_in, 0)

        def scan(it, carry):
            ltr, lti, clr, cli, gr, gi = (cf_v[it, i] for i in range(6))
            nclr = -clr
            for c in range(2 * n_chunks):
                idx = pl.ds((c % 2) * n_chunks + c // 2, cb, stride=SPITCH)
                gre_v[it, idx, :] = gr
                gim_v[it, idx, :] = gi
                if c < 2 * n_chunks - 1:
                    xr, xi = sre_v[it, idx, :], sim_v[it, idx, :]
                    sr, si = clr * xr - cli * xi, nclr * xi - cli * xr
                    if c == 0:
                        gr, gi = sr, si
                    else:
                        gr, gi = cmul(gr, gi, ltr, lti)
                        gr, gi = gr + sr, gi + si
            return carry

        lax.fori_loop(0, n_it, scan, 0)

        ti = lax.broadcasted_iota(jnp.int32, (TC, T), 0)
        tj = lax.broadcasted_iota(jnp.int32, (TC, T), 1)
        causal_even = (tj >= ti) & (tj < TC)
        causal_odd = tj >= ti + TC
        has_state = lax.broadcasted_iota(jnp.int32, (n_chunks, T), 0) > 0

        def state_out(it, carry):
            for k in range(cb):
                gg = jnp.concatenate([gre_v[it, states(k), :], gim_v[it, states(k), :]], axis=1)
                p = p_v[it, k]
                y = _dot(gg, jnp.concatenate([p, jnp.zeros_like(p)], axis=0), NT)
                taps_v[it, 8 * k:8 * k + 8, :] = y[0:8, :] + pltpu.roll(y[0:8, :], TC, 1)
                y_v[it, chan(k), :] = jnp.where(has_state, y[:n_chunks], 0.0) + pltpu.roll(y[n_chunks:], TC, 1)
            return carry

        lax.fori_loop(0, n_it, state_out, 0)

        def in_chunk(it, carry):
            for k in range(cb):
                kb = jnp.broadcast_to(taps_v[it, 8 * k:8 * k + 1, :], (TC, T))
                tz = pltpu.roll(kb, 0, 1, stride=1, stride_axis=0)
                tz = jnp.concatenate([jnp.where(causal_even, tz, 0.0),
                                      jnp.where(causal_odd, tz, 0.0)], axis=0)
                y_v[it, chan(k), :] += _dot(uf_v[it, chan(k), :], tz.astype(BF16))
            return carry

        lax.fori_loop(0, n_it, in_chunk, 0)

        def y_chunks(q, carry):
            nq = 4
            for c in range(nq):
                tt = pl.ds(pl.multiple_of((q * nq + c) * T, T), T)
                idx = pl.ds(q * nq + c, cb, stride=PITCH)
                yc = jnp.concatenate([y_v[it, idx, :] for it in range(n_it)], axis=0)
                yc = yc.T.astype(BF16).astype(F32)
                skip = (u_v[g, tt, :].astype(F32) * dsk).astype(BF16).astype(F32)
                outb_v[g, tt, :] = (yc + skip).astype(BF16)
            return carry

        lax.fori_loop(0, n_chunks // 4, y_chunks, 0)

    ldt_all = ldt_ref[...].astype(F32).reshape(n_groups, GC)
    dsk_all = dsk_ref[...].astype(F32).reshape(n_groups, GC)
    for cp in par_copies():
        cp.wait()

    for g in range(n_slots):
        if g > 1:
            u_copy(g).start()
        for cp in w_copies(g, g):
            cp.start()

    def weights_step(g):
        slot = lax.rem(g, n_slots)
        for cp in w_copies(g, slot):
            cp.wait()
        relayout(g, slot)

        @pl.when(g + n_slots < n_groups)
        def _():
            for cp in w_copies(g + n_slots, slot):
                cp.start()

        @pl.when(g + n_slots == n_groups)
        def _():
            x_copy.start()

    def phase1(g, carry):
        u_copy(g).wait()

        @pl.when(g + n_slots < n_groups)
        def _():
            u_copy(g + n_slots).start()

        if do_b:
            ssm_group(g, ldt_all, dsk_all)
        else:
            outb_v[g] = u_v[g]
        weights_step(g)
        return carry

    lax.fori_loop(0, n_groups, phase1, 0)
    for g in range(n_groups):
        outb_copy(g).start()
    x_copy.wait()

    scale = Dh ** -0.5
    qi = lax.broadcasted_iota(jnp.int32, (L, 128), 0)
    ki = lax.broadcasted_iota(jnp.int32, (L, 128), 1)
    keep = (qi < n_mem) | (qi >= ki)
    fill = jnp.where(ki < L, -1000000000.0, -jnp.inf)
    keep = keep & (ki < L)
    zpad = jnp.zeros((128 - L, Dh), F32)

    def proj(h, i):
        return _dot(h_v[...], pltpu.bitcast(wqkv_v[h * 3 + i], BF16))

    HG = 8
    n_og = n_heads // HG
    n_j = Dm // 128

    def step(s, carry):
        r = pl.ds(pl.multiple_of(s * seg, seg), seg)
        h_v[n_mem:, :] = x_v[r, :].astype(F32)
        qs, ks, vs, es, os_ = {}, {}, {}, {}, {}

        def scores(h):
            sc = _dot(qs.pop(h), ks.pop(h), NT)
            sc = jnp.where(keep, sc * scale, fill)
            e = jnp.exp(sc - jnp.max(sc, axis=1, keepdims=True))
            es[h] = (e, 1.0 / jnp.sum(e, axis=1, keepdims=True))

        def mix(h):
            e, inv = es.pop(h)
            o = _dot(e, vs.pop(h)) * inv
            if mode & 1:
                os_[h] = o
            else:
                o_v[:, h * Dh:(h + 1) * Dh] = o

        def oproj(j, g):
            w = pltpu.bitcast(wo_v[j, g * HG * Dh // 2:(g + 1) * HG * Dh // 2, :], BF16)
            if mode & 1:
                lhs = jnp.concatenate([os_[h] for h in range(g * HG, (g + 1) * HG)], axis=1)
            else:
                lhs = o_v[:, g * HG * Dh:(g + 1) * HG * Dh]
            return _dot(lhs, w)

        def emit(j, res):
            h_v[:n_mem, 128 * j:128 * (j + 1)] = res[:n_mem]
            outa_v[r, 128 * j:128 * (j + 1)] = res[n_mem:].astype(BF16)

        AG = 4
        for h0 in range(0, n_heads, AG):
            for i in range(AG):
                h = h0 + i
                qs[h] = proj(h, 0)
                if h0 and i == 0:
                    for hh in range(h0 - AG, h0):
                        scores(hh)
                ks[h] = jnp.concatenate([proj(h, 1), zpad], axis=0).astype(BF16)
                if h0 and i == lag:
                    for hh in range(h0 - AG, h0):
                        mix(hh)
                vs[h] = jnp.concatenate([proj(h, 2), zpad], axis=0).astype(BF16)

        acc = {}

        def early(t):
            j, g = divmod(t, n_og - 1)
            acc[j] = oproj(j, g) if g == 0 else acc[j] + oproj(j, g)

        t = 0
        early(t)
        t += 1
        for hh in range(n_heads - AG, n_heads):
            scores(hh)
        for _ in range(fill_n):
            early(t)
            t += 1
        for hh in range(n_heads - AG, n_heads):
            mix(hh)
        for _ in range(3):
            early(t)
            t += 1
        for j in range(n_j):
            while t < (j + 1) * (n_og - 1):
                early(t)
                t += 1
            emit(j, acc.pop(j) + oproj(j, n_og - 1))
        outa_copy(s).start()
        return carry

    h_v[:n_mem, :] = mem0_ref[...].astype(F32)
    if do_a:
        lax.fori_loop(0, n_seg, step, 0, unroll=unroll)
    else:
        def dummy(s, carry):
            r = pl.ds(pl.multiple_of(s * seg, seg), seg)
            outa_v[r, :] = x_v[r, :]
            outa_copy(s).start()
            return carry
        lax.fori_loop(0, n_seg, dummy, 0)

    for g in range(n_groups):
        outb_copy(g).wait()

    def drain(s, carry):
        outa_copy(s).wait()
        return carry
    lax.fori_loop(0, n_seg, drain, 0)


@functools.partial(jax.jit, static_argnames=("A_seg_len", "cb", "lag", "mode", "fill_n", "unroll", "do_a", "do_b"))
def pallas_concat_heads__memory_aug_recurrent_mem_tr__ssm_conv_s4__prompt_kernel(A_x, A_mem0, A_Wq, A_Wk, A_Wv, A_Wo, A_seg_len, B_u, B_A_re, B_A_im, B_B_re, B_B_im,
           B_C_re, B_C_im, B_log_dt, B_Dskip, cb=64, lag=3, mode=1, fill_n=5, unroll=1, do_a=True, do_b=True):
    Bsz, S, Dm = A_x.shape
    H, Dh = A_Wq.shape[1], A_Wq.shape[2]
    M = A_mem0.shape[1]
    D, N = B_A_re.shape
    seg = int(A_seg_len)
    assert Bsz == 1 and Dh == 128 and N == 128 and D == Dm and B_u.shape == A_x.shape
    L = M + seg
    n_groups = D // GC
    n_chunks = S // T
    n_slots = 3
    n_it = GC // cb
    DC = Dm // n_groups

    def head_tiles(w):
        return w.reshape(Dm, H // 8, 8, Dh).transpose(0, 2, 1, 3).reshape(Dm * 8, H // 8 * Dh)

    any_spec = pl.BlockSpec(memory_space=pl.ANY)
    vmem_spec = pl.BlockSpec(memory_space=pltpu.VMEM)
    out = pl.pallas_call(
        functools.partial(_kernel, seg=seg, n_mem=M, n_heads=H, cb=cb, lag=lag, mode=mode, fill_n=fill_n, unroll=unroll, do_a=do_a, do_b=do_b),
        out_shape=jax.ShapeDtypeStruct((S, Dm + D), BF16),
        in_specs=[any_spec, vmem_spec] + [any_spec] * 11 + [vmem_spec, vmem_spec],
        out_specs=any_spec,
        scratch_shapes=[
            pltpu.VMEM((S, Dm), BF16),
            pltpu.VMEM((n_groups, S, GC), BF16),
            pltpu.VMEM((6, D, N), BF16),
            pltpu.VMEM((n_slots, 3 * H // 8, DC * 8, 128), BF16),
            pltpu.VMEM((n_slots, H * Dh // n_groups, Dm), BF16),
            pltpu.VMEM((3 * H, Dm // 2, Dh), U32),
            pltpu.VMEM((Dm // 128, H * Dh // 2, 128), U32),
            pltpu.VMEM((S, Dm), BF16),
            pltpu.VMEM((n_groups, S, GC), BF16),
            pltpu.VMEM((L, Dm), F32),
            pltpu.VMEM((L, H * Dh), F32),
            pltpu.VMEM((n_it, cb * BPITCH, N), F32),
            pltpu.VMEM((n_it, cb * BPITCH, N), F32),
            pltpu.VMEM((n_it, 8, cb, N), F32),
            pltpu.VMEM((n_it, cb, TC, 2 * N), BF16),
            pltpu.VMEM((n_it, cb * PITCH, T), F32),
            pltpu.VMEM((n_it, cb * PITCH, T), F32),
            pltpu.VMEM((n_it, cb * SPITCH, N), F32),
            pltpu.VMEM((n_it, cb * SPITCH, N), F32),
            pltpu.VMEM((n_it, cb * SPITCH, N), F32),
            pltpu.VMEM((n_it, cb * SPITCH, N), F32),
            pltpu.VMEM((n_it, cb * PITCH, T), F32),
            pltpu.VMEM((n_it, cb * 8, T), F32),
            pltpu.SemaphoreType.DMA(()),
            pltpu.SemaphoreType.DMA((n_groups,)),
            pltpu.SemaphoreType.DMA(()),
            pltpu.SemaphoreType.DMA((n_slots,)),
            pltpu.SemaphoreType.DMA(()),
            pltpu.SemaphoreType.DMA(()),
        ],
        compiler_params=pltpu.CompilerParams(vmem_limit_bytes=110 * 1024 * 1024),
    )(A_x.reshape(S, Dm), A_mem0.reshape(M, Dm), head_tiles(A_Wq), head_tiles(A_Wk), head_tiles(A_Wv),
      A_Wo.reshape(H * Dh, Dm), B_u.reshape(S, D), B_A_re, B_A_im, B_B_re, B_B_im, B_C_re, B_C_im,
      B_log_dt, B_Dskip)
    return out.reshape(Bsz, S, Dm + D)
```

```python
import functools

import jax
import jax.numpy as jnp
from jax import lax
import jax.experimental.pallas as pl
import jax.experimental.pallas.tpu as pltpu

F32 = jnp.float32
BF16 = jnp.bfloat16
U32 = jnp.uint32

NN = (((1,), (0,)), ((), ()))
NT = (((1,), (1,)), ((), ()))

T = 128
TC = T // 2
GC = 128
PITCH = 17
SPITCH = 33
BPITCH = 9
PRE = 8


def _dot(a, b, dims=NN):
    return lax.dot_general(a, b, dims, preferred_element_type=F32)


def _cmul(ar, ai, br, bi):
    return ar * br - ai * bi, ar * bi + ai * br


def _kernel(x_hbm, mem0_ref, wq_hbm, wk_hbm, wv_hbm, wo_hbm,
            u_hbm, are_hbm, aim_hbm, bre_hbm, bim_hbm, cre_hbm, cim_hbm, ldt_ref, dsk_ref,
            out_hbm,
            x_v, xt_v, xp_v, u_v, par_v, stage_w, w0_v, w1_v, w2_v, w3_v, wo_v, pre_v, outa_v, outb_v, h_v,
            dt_v, bre_v, bim_v, cf_v, p_v, uf_v, ur_v, sre_v, sim_v, gre_v, gim_v, y_v, taps_v,
            sem_x, sem_xt, sem_u, sem_par, sem_w, sem_wo, sem_oa, sem_ob,
            *, n_mem, n_heads, pb, lag, fill_n, unroll, units, RB, sb, n_q, do_a):
    n_seg, seg, Dm = x_v.shape
    S = n_seg * seg
    n_groups = Dm // GC
    n_blocks = S // T
    L = n_mem + seg
    Dh = 128
    n_slots = stage_w.shape[0]
    DC = 128
    n_pc = stage_w.shape[2] // (8 * DC)
    n_rb = n_seg * PRE // RB
    w_vs = (w0_v, w1_v, w2_v, w3_v)
    n_hg = len(w_vs)
    g_per_hg = n_groups // n_hg
    u_pre, u_uc, u_si, u_sc, u_so, u_ic, u_yc = units
    units_per_group = sum(units)
    assert units_per_group * g_per_hg % n_rb == 0
    n_pre = units_per_group * g_per_hg // n_rb
    assert n_pre <= pre_v.shape[1]

    def start_weights(hg, part, slot):
        for i, w in enumerate((wq_hbm, wk_hbm, wv_hbm)):
            rows = pl.ds(pl.multiple_of(part * (n_pc * DC * 8), DC * 8), n_pc * DC * 8)
            pltpu.make_async_copy(w.at[rows, pl.ds(hg * 128, 128)], stage_w.at[slot, i], sem_w.at[slot]).start()

    def wait_weights(slot):
        pltpu.make_async_copy(stage_w.at[slot], stage_w.at[slot], sem_w.at[slot]).wait()

    def wo_copy(j):
        return pltpu.make_async_copy(
            wo_hbm.at[:, pl.ds(pl.multiple_of(128 * j, 128), 128)], wo_v.at[j].bitcast(BF16), sem_wo)

    def x_copy(g):
        r = pl.ds(g * (n_seg // n_groups), n_seg // n_groups)
        return pltpu.make_async_copy(x_hbm.at[r], x_v.at[r], sem_x)

    def u_copy(g):
        return pltpu.make_async_copy(
            u_hbm.at[:, pl.ds(pl.multiple_of(g * GC, GC), GC)], u_v.at[g], sem_u.at[g])

    def par_copies():
        return [pltpu.make_async_copy(p, par_v.at[i], sem_par)
                for i, p in enumerate((are_hbm, aim_hbm, bre_hbm, bim_hbm, cre_hbm, cim_hbm))]

    def outb_copy(g):
        return pltpu.make_async_copy(outb_v.at[g], out_hbm.at[:, pl.ds(Dm + g * GC, GC)], sem_ob)

    def outa_copy(s):
        r = pl.ds(pl.multiple_of(s * seg, seg), seg)
        return pltpu.make_async_copy(outa_v.at[r, :], out_hbm.at[r, pl.ds(0, Dm)], sem_oa)

    xt_copy = pltpu.make_async_copy(x_hbm.at[:, pl.ds(seg - PRE, PRE), :], xt_v, sem_xt)

    for cp in par_copies():
        cp.start()
    u_copy(0).start()
    u_copy(1).start()

    def ahead(hg, unit):
        m = unit // n_rb
        rows = pl.ds(pl.multiple_of((unit - m * n_rb) * RB, RB), RB)
        pre_v[hg, m, rows, :] = _dot(xp_v[rows, :], pltpu.bitcast(w_vs[hg][m], BF16))

    def chan(k):
        return slice(k * PITCH, k * PITCH + n_blocks)

    def states(k):
        return slice(k * SPITCH, k * SPITCH + 2 * n_blocks)

    def group(part, carry, *, hg):
        g = hg * g_per_hg + part
        with_ahead = hg > 0
        next_unit = [part * units_per_group]

        def loop(n, n_units, body):
            assert n_units % n == 0
            per_iter = n_units // n
            first = next_unit[0]
            next_unit[0] = first + n_units

            def wrapped(i, c):
                todo = list(range(per_iter)) if with_ahead else []

                def fill(done, total):
                    while todo and todo[0] * total <= done * per_iter:
                        ahead(hg - 1, first + i * per_iter + todo.pop(0))

                body(i, fill)
                fill(1, 1)
                return c

            with jax.named_scope(body.__name__ + ("+" if with_ahead else "")):
                if n == 1:
                    @pl.when(g >= 0)
                    def _():
                        wrapped(0, 0)
                else:
                    lax.fori_loop(0, n, wrapped, 0)

        with jax.named_scope('wait_u'):
            u_copy(g).wait()

        @pl.when(g + 2 < n_groups)
        def _():
            u_copy(g + 2).start()

        sel = lax.broadcasted_iota(jnp.int32, (n_groups, GC), 0) == g
        ldt = jnp.sum(jnp.where(sel, carry[0], 0.0), axis=0, keepdims=True)
        dsk = jnp.sum(jnp.where(sel, carry[1], 0.0), axis=0, keepdims=True)
        dt_row = jnp.exp(ldt).astype(BF16).astype(F32)
        dt_v[...] = jnp.broadcast_to(dt_row, (GC, GC)).T

        def powers(_, fill):
            for it in range(GC // pb):
                fill(2 * it, 2 * GC // pb)
                rows = pl.ds(pl.multiple_of(g * GC + it * pb, pb), pb)
                k0 = it * pb
                dt = dt_v[k0:k0 + pb, :]
                zr = dt * par_v[0, rows, :].astype(F32)
                zi = dt * par_v[1, rows, :].astype(F32)
                c_re, c_im = _cmul(par_v[4, rows, :].astype(F32), par_v[5, rows, :].astype(F32),
                                   dt * par_v[2, rows, :].astype(F32), dt * par_v[3, rows, :].astype(F32))
                mag = jnp.exp(zr)
                l1 = (mag * jnp.cos(zi), mag * jnp.sin(zi))
                fill(2 * it + 1, 2 * GC // pb)
                l2 = _cmul(*l1, *l1)
                l3 = _cmul(*l2, *l1)
                l4 = _cmul(*l2, *l2)
                pw = [(jnp.ones_like(mag), jnp.zeros_like(mag)), l1, l2, l3, l4,
                      _cmul(*l4, *l1), _cmul(*l4, *l2), _cmul(*l4, *l3)]
                for r in range(8):
                    bre_v[pl.ds(k0 * BPITCH + r, pb, stride=BPITCH), :] = pw[r][0]
                    bim_v[pl.ds(k0 * BPITCH + r, pb, stride=BPITCH), :] = pw[r][1]
                l8 = _cmul(*l4, *l4)
                lt = l8
                for _ in range(3):
                    lt = _cmul(*lt, *lt)
                cl = _cmul(c_re, c_im, *l1)
                for i, val in enumerate((lt[0], -lt[1], cl[0], cl[1], c_re, -c_im, *l8)):
                    cf_v[i, k0:k0 + pb, :] = val

        loop(1, u_pre, powers)

        ri = lax.broadcasted_iota(jnp.int32, (T, T), 0)
        ci = lax.broadcasted_iota(jnp.int32, (T, T), 1)
        flip = jnp.where((ri ^ ci) == TC - 1, 1.0, 0.0).astype(BF16)

        def u_blocks(q, fill):
            uts = [u_v[g, pl.ds(pl.multiple_of((q * n_q + c) * T, T), T), :].astype(F32).T
                   for c in range(n_q)]
            fill(0, 4)
            urev = _dot(jnp.concatenate(uts, axis=0), flip)
            for c in range(n_q):
                idx = pl.ds(q * n_q + c, GC, stride=PITCH)
                uf_v[idx, :] = uts[c]
                ur_v[idx, :] = urev[c * GC:(c + 1) * GC]

        loop(n_blocks // n_q, u_uc, u_blocks)

        @pl.when(part + 1 < g_per_hg)
        def _():
            start_weights(hg, part + 1, part + 1)

        if hg + 1 < n_hg:
            @pl.when(part + 1 == g_per_hg)
            def _():
                start_weights(hg + 1, 0, 0)

        wo_copy(g).start()
        x_copy(g).start()

        even = lax.broadcasted_iota(jnp.int32, (n_blocks, T), 1) < TC

        def state_in(it, fill):
            for k in range(GC):
                pr = [bre_v[k * BPITCH:k * BPITCH + 8, :]]
                pi = [bim_v[k * BPITCH:k * BPITCH + 8, :]]
                mr = jnp.broadcast_to(cf_v[6, k:k + 1, :], (8, 128))
                mi = jnp.broadcast_to(cf_v[7, k:k + 1, :], (8, 128))
                for _ in range(TC // 8 - 1):
                    nr, ni = _cmul(pr[-1], pi[-1], mr, mi)
                    pr.append(nr)
                    pi.append(ni)
                p_v[k] = jnp.concatenate(
                    [jnp.concatenate(pr, axis=0), jnp.concatenate(pi, axis=0)], axis=1).astype(BF16)
                ur = ur_v[chan(k), :]
                ur = jnp.concatenate([jnp.where(even, ur, 0.0), jnp.where(even, 0.0, ur)], axis=0)
                if k % 2 == 0:
                    fill(k, GC)
                sre_v[states(k), :] = _dot(ur, jnp.concatenate(pr + pr, axis=0).astype(BF16))
                sim_v[states(k), :] = _dot(ur, jnp.concatenate(pi + pi, axis=0).astype(BF16))

        loop(1, u_si, state_in)

        def scan(_, fill):
            width = sb if with_ahead else 32
            last = None
            for k0 in range(0, GC, width):
                ltr, lti, clr, cli, gr, gi = (cf_v[i, k0:k0 + width, :] for i in range(6))
                if last is not None:
                    clr, cli = jnp.where(g < 0, last, clr), jnp.where(g < 0, last, cli)
                nclr = -clr
                for c in range(2 * n_blocks):
                    fill(k0 * 2 * n_blocks + c * width, GC * 2 * n_blocks)
                    idx = pl.ds(k0 * SPITCH + (c % 2) * n_blocks + c // 2, width, stride=SPITCH)
                    gre_v[idx, :] = gr
                    gim_v[idx, :] = gi
                    if c < 2 * n_blocks - 1:
                        xr, xi = sre_v[idx, :], sim_v[idx, :]
                        sr, si = clr * xr - cli * xi, nclr * xi - cli * xr
                        if c == 0:
                            gr, gi = sr, si
                        else:
                            gr, gi = _cmul(gr, gi, ltr, lti)
                            gr, gi = gr + sr, gi + si
                last = gr

        loop(1, u_sc, scan)

        slot = part
        with jax.named_scope('wait_w'):
            wait_weights(slot)

        def relayout(t):
            i, pc = divmod(t, n_pc)
            src = stage_w.at[slot, i].bitcast(U32)
            rows = pl.ds(pl.multiple_of((part * n_pc + pc) * (DC // 2), DC // 2), DC // 2)
            for pp in range(4):
                ev = src[pl.ds(pc * DC * 4 + pp, DC // 2, stride=8), :]
                od = src[pl.ds(pc * DC * 4 + pp + 4, DC // 2, stride=8), :]
                w_vs[hg][6 * pp + i, rows, :] = (ev & 0xFFFF) | (od << 16)
                w_vs[hg][6 * pp + 3 + i, rows, :] = (ev >> 16) | (od & jnp.uint32(0xFFFF0000))

        has_state = lax.broadcasted_iota(jnp.int32, (n_blocks, T), 0) > 0

        def state_out(it, fill):
            n_rl = 3 * n_pc
            for k in range(GC):
                if k * n_rl % GC < n_rl:
                    relayout(k * n_rl // GC)
                if k % 2 == 0:
                    fill(k, GC)
                gg = jnp.concatenate([gre_v[states(k), :], gim_v[states(k), :]], axis=1)
                p = p_v[k]
                y = _dot(gg, jnp.concatenate([p, jnp.zeros_like(p)], axis=0), NT)
                taps_v[8 * k:8 * k + 8, :] = y[0:8, :] + pltpu.roll(y[0:8, :], TC, 1)
                y_v[chan(k), :] = jnp.where(has_state, y[:n_blocks], 0.0) + pltpu.roll(y[n_blocks:], TC, 1)

        loop(1, u_so, state_out)

        ti = lax.broadcasted_iota(jnp.int32, (TC, T), 0)
        tj = lax.broadcasted_iota(jnp.int32, (TC, T), 1)
        causal_even = (tj >= ti) & (tj < TC)
        causal_odd = tj >= ti + TC

        def in_chunk(it, fill):
            for k in range(GC):
                if k % 4 == 0:
                    fill(k, GC)
                kb = jnp.broadcast_to(taps_v[8 * k:8 * k + 1, :], (TC, T))
                tz = pltpu.roll(kb, 0, 1, stride=1, stride_axis=0)
                tz = jnp.concatenate([jnp.where(causal_even, tz, 0.0),
                                      jnp.where(causal_odd, tz, 0.0)], axis=0)
                y_v[chan(k), :] += _dot(uf_v[chan(k), :], tz.astype(BF16))

        loop(1, u_ic, in_chunk)

        def y_blocks(q, fill):
            for c in range(n_q):
                fill(c, n_q)
                tt = pl.ds(pl.multiple_of((q * n_q + c) * T, T), T)
                yc = y_v[pl.ds(q * n_q + c, GC, stride=PITCH), :].T.astype(BF16).astype(F32)
                skip = (u_v[g, tt, :].astype(F32) * dsk).astype(BF16).astype(F32)
                outb_v[g, tt, :] = (yc + skip).astype(BF16)

        loop(n_blocks // n_q, u_yc, y_blocks)

        return carry

    vecs = (ldt_ref[...].astype(F32).reshape(n_groups, GC), dsk_ref[...].astype(F32).reshape(n_groups, GC))
    with jax.named_scope('wait_par'):
        for cp in par_copies():
            cp.wait()
    start_weights(0, 0, 0)
    xt_copy.start()

    lax.fori_loop(0, g_per_hg, functools.partial(group, hg=0), vecs)
    xt_copy.wait()

    def widen(q, carry):
        for c in range(8):
            s = q * 8 + c
            xp_v[pl.ds(pl.multiple_of(s * PRE, PRE), PRE), :] = xt_v[s].astype(F32)
        return carry

    lax.fori_loop(0, n_seg // 8, widen, 0)
    for hg in range(1, n_hg):
        lax.fori_loop(0, g_per_hg, functools.partial(group, hg=hg), vecs)
    for g in range(n_groups):
        outb_copy(g).start()
    with jax.named_scope('wait_x'):
        for g in range(n_groups):
            x_copy(g).wait()
            wo_copy(g).wait()

    scale = Dh ** -0.5
    qi = lax.broadcasted_iota(jnp.int32, (L, 128), 0)
    ki = lax.broadcasted_iota(jnp.int32, (L, 128), 1)
    keep = ((qi < n_mem) | (qi >= ki)) & (ki < L)
    masked = jnp.where(ki < L, -1000000000.0, -jnp.inf)
    zpad = jnp.zeros((128 - L, Dh), F32)
    HG = 8
    AG = 4
    n_og = n_heads // HG
    n_j = Dm // 128

    def step(s, carry):
        r = pl.ds(pl.multiple_of(s * seg, seg), seg)
        h_v[n_mem:, :] = x_v[s].astype(F32)
        qs, ks, vs, es, os_ = {}, {}, {}, {}, {}

        def proj(h, i):
            hg, m = divmod(h * 3 + i, 24)
            w = pltpu.bitcast(w_vs[hg][m], BF16)
            if hg + 1 < n_hg and m < n_pre:
                known = pre_v[hg, m, pl.ds(pl.multiple_of(s * PRE, PRE), PRE), :]
                return jnp.concatenate([_dot(h_v[:L - PRE, :], w), known], axis=0)
            return _dot(h_v[...], w)

        def scores(h):
            sc = _dot(qs.pop(h), ks.pop(h), NT)
            sc = jnp.where(keep, sc * scale, masked)
            e = jnp.exp(sc - jnp.max(sc, axis=1, keepdims=True))
            es[h] = (e, 1.0 / jnp.sum(e, axis=1, keepdims=True))

        def mix(h):
            e, inv = es.pop(h)
            os_[h] = _dot(e, vs.pop(h)) * inv

        def oproj(j, g):
            w = pltpu.bitcast(wo_v[j, g * HG * Dh // 2:(g + 1) * HG * Dh // 2, :], BF16)
            return _dot(jnp.concatenate([os_[h] for h in range(g * HG, (g + 1) * HG)], axis=1), w)

        def emit(j, res):
            h_v[:n_mem, 128 * j:128 * (j + 1)] = res[:n_mem]
            outa_v[r, 128 * j:128 * (j + 1)] = res[n_mem:].astype(BF16)

        for h0 in range(0, n_heads, AG):
            for i in range(AG):
                h = h0 + i
                qs[h] = proj(h, 0)
                if h0 and i == 0:
                    for hh in range(h0 - AG, h0):
                        scores(hh)
                ks[h] = jnp.concatenate([proj(h, 1), zpad], axis=0).astype(BF16)
                if h0 and i == lag:
                    for hh in range(h0 - AG, h0):
                        mix(hh)
                vs[h] = jnp.concatenate([proj(h, 2), zpad], axis=0).astype(BF16)

        acc = {}

        def early(t):
            j, g = divmod(t, n_og - 1)
            acc[j] = oproj(j, g) if g == 0 else acc[j] + oproj(j, g)

        t = 0
        early(t)
        t += 1
        for hh in range(n_heads - AG, n_heads):
            scores(hh)
        for _ in range(fill_n):
            early(t)
            t += 1
        for hh in range(n_heads - AG, n_heads):
            mix(hh)
        for _ in range(3):
            early(t)
            t += 1
        for j in range(n_j):
            while t < (j + 1) * (n_og - 1):
                early(t)
                t += 1
            emit(j, acc.pop(j) + oproj(j, n_og - 1))
        outa_copy(s).start()
        return carry

    h_v[:n_mem, :] = mem0_ref[...].astype(F32)
    if do_a:
        with jax.named_scope('steps'):
            lax.fori_loop(0, n_seg, step, 0, unroll=unroll)
    else:
        def dummy(s, carry):
            outa_v[pl.ds(pl.multiple_of(s * seg, seg), seg), :] = x_v[s]
            outa_copy(s).start()
            return carry
        lax.fori_loop(0, n_seg, dummy, 0)

    for g in range(n_groups):
        outb_copy(g).wait()

    def drain(s, carry):
        outa_copy(s).wait()
        return carry

    lax.fori_loop(0, n_seg, drain, 0)


@functools.partial(jax.jit, static_argnames=(
    "A_seg_len", "pb", "lag", "fill_n", "unroll", "units", "RB", "sb", "nq", "flags", "do_a"))
def pallas_concat_heads__memory_aug_recurrent_mem_tr__ssm_conv_s4__prompt_kernel(A_x, A_mem0, A_Wq, A_Wk, A_Wv, A_Wo, A_seg_len, B_u, B_A_re, B_A_im, B_B_re, B_B_im,
           B_C_re, B_C_im, B_log_dt, B_Dskip, pb=32, lag=3, fill_n=5, unroll=1,
           units="11,14,2,23,8,14,12", RB=64, sb=8, nq=8, flags="", do_a=True):
    Bsz, S, Dm = A_x.shape
    H, Dh = A_Wq.shape[1], A_Wq.shape[2]
    M = A_mem0.shape[1]
    D, N = B_A_re.shape
    seg = int(A_seg_len)
    assert Bsz == 1 and Dh == 128 and N == 128 and D == Dm and B_u.shape == A_x.shape
    L = M + seg
    n_seg = S // seg
    n_groups = D // GC
    n_slots = n_groups // (H // 8)
    if isinstance(units, str):
        units = tuple(int(c) for c in units.split(','))

    def head_tiles(w):
        return w.reshape(Dm, H // 8, 8, Dh).transpose(0, 2, 1, 3).reshape(Dm * 8, H // 8 * Dh)

    any_spec = pl.BlockSpec(memory_space=pl.ANY)
    vmem_spec = pl.BlockSpec(memory_space=pltpu.VMEM)
    out = pl.pallas_call(
        functools.partial(_kernel, n_mem=M, n_heads=H, pb=pb, lag=lag, fill_n=fill_n, unroll=unroll,
                          units=units, RB=RB, sb=sb, n_q=nq, do_a=do_a),
        out_shape=jax.ShapeDtypeStruct((S, Dm + D), BF16),
        in_specs=[any_spec, vmem_spec] + [any_spec] * 11 + [vmem_spec, vmem_spec],
        out_specs=any_spec,
        scratch_shapes=[
            pltpu.VMEM((n_seg, seg, Dm), BF16),
            pltpu.VMEM((n_seg, PRE, Dm), BF16),
            pltpu.VMEM((n_seg * PRE, Dm), F32),
            pltpu.VMEM((n_groups, S, GC), BF16),
            pltpu.VMEM((6, D, N), BF16),
            pltpu.VMEM((n_slots, 3, Dm * 8 // n_slots, 128), BF16),
            *[pltpu.VMEM((24, Dm // 2, Dh), U32)] * (H // 8),
            pltpu.VMEM((Dm // 128, H * Dh // 2, 128), U32),
            pltpu.VMEM((H // 8 - 1, 24, n_seg * PRE, Dh), F32),
            pltpu.VMEM((S, Dm), BF16),
            pltpu.VMEM((n_groups, S, GC), BF16),
            pltpu.VMEM((L, Dm), F32),
            pltpu.VMEM((GC, N), F32),
            pltpu.VMEM((GC * BPITCH, N), F32),
            pltpu.VMEM((GC * BPITCH, N), F32),
            pltpu.VMEM((8, GC, N), F32),
            pltpu.VMEM((GC, TC, 2 * N), BF16),
            pltpu.VMEM((GC * PITCH, T), F32),
            pltpu.VMEM((GC * PITCH, T), F32),
            pltpu.VMEM((GC * SPITCH, N), F32),
            pltpu.VMEM((GC * SPITCH, N), F32),
            pltpu.VMEM((GC * SPITCH, N), F32),
            pltpu.VMEM((GC * SPITCH, N), F32),
            pltpu.VMEM((GC * PITCH, T), F32),
            pltpu.VMEM((GC * 8, T), F32),
            pltpu.SemaphoreType.DMA(()),
            pltpu.SemaphoreType.DMA(()),
            pltpu.SemaphoreType.DMA((n_groups,)),
            pltpu.SemaphoreType.DMA(()),
            pltpu.SemaphoreType.DMA((n_slots,)),
            pltpu.SemaphoreType.DMA(()),
            pltpu.SemaphoreType.DMA(()),
            pltpu.SemaphoreType.DMA(()),
        ],
        compiler_params=pltpu.CompilerParams(vmem_limit_bytes=120 * 1024 * 1024, flags={f: True for f in flags.split(',') if f} or None),
    )(A_x.reshape(n_seg, seg, Dm), A_mem0.reshape(M, Dm),
      head_tiles(A_Wq), head_tiles(A_Wk), head_tiles(A_Wv), A_Wo.reshape(H * Dh, Dm),
      B_u.reshape(S, D), B_A_re, B_A_im, B_B_re, B_B_im, B_C_re, B_C_im, B_log_dt, B_Dskip)
    return out.reshape(Bsz, S, Dm + D)
```

```python
import functools
import math

import jax
import jax.numpy as jnp
from jax import lax
import jax.experimental.pallas as pl
import jax.experimental.pallas.tpu as pltpu

F32 = jnp.float32
BF16 = jnp.bfloat16
U32 = jnp.uint32

NN = (((1,), (0,)), ((), ()))
NT = (((1,), (1,)), ((), ()))

T = 128
TC = T // 2
GC = 128
PITCH = 17
SPITCH = 33
BPITCH = 9
LOG2E = math.log2(math.e)
PRE = 8


def _dot(a, b, dims=NN):
    return lax.dot_general(a, b, dims, preferred_element_type=F32)


def _cmul(ar, ai, br, bi):
    return ar * br - ai * bi, ar * bi + ai * br


def _kernel(x_hbm, mem0_ref, wq_hbm, wk_hbm, wv_hbm, wo_hbm,
            u_hbm, are_hbm, aim_hbm, bre_hbm, bim_hbm, cre_hbm, cim_hbm, ldt_ref, dsk_ref,
            out_hbm,
            x_v, xt_v, xp_v, u_v, par_v, stage_w, w0_v, w1_v, w2_v, w3_v, wo_v, pre_v, outa_v, outb_v, h_v,
            dt_v, bre_v, bim_v, cf_v, p_v, uf_v, ur_v, sre_v, sim_v, gre_v, gim_v, y_v, taps_v,
            sem_x, sem_xt, sem_u, sem_par, sem_w, sem_wo, sem_oa, sem_ob,
            *, n_mem, n_heads, pb, lag, fill_n, unroll, units, RB, sb, n_q, split, order, perm, lag0, pre_n, do_b):
    n_seg, seg, Dm = x_v.shape
    S = n_seg * seg
    n_groups = Dm // GC
    n_blocks = S // T
    L = n_mem + seg
    Dh = 128
    n_slots = stage_w.shape[0]
    DC = 128
    n_pc = stage_w.shape[2] // (8 * DC)
    n_rb = n_seg * PRE // RB
    w_vs = (w0_v, w1_v, w2_v, w3_v)
    n_hg = len(w_vs)
    g_per_hg = n_groups // n_hg
    u_pre, u_uc, u_si, u_sc, u_so, u_ic, u_yc = units
    units_per_group = sum(units)
    assert units_per_group * g_per_hg % n_rb == 0
    n_pre = units_per_group * g_per_hg // n_rb
    assert n_pre <= pre_v.shape[1]

    def start_weights(hg, part, slot):
        for c in range(3):
            if order:
                i, tile = divmod(3 * hg + c, n_hg)
            else:
                tile, i = divmod(3 * hg + c, 3)
            rows = pl.ds(pl.multiple_of(part * (n_pc * DC * 8), DC * 8), n_pc * DC * 8)
            pltpu.make_async_copy((wq_hbm, wk_hbm, wv_hbm)[i].at[rows, pl.ds(tile * 128, 128)],
                                  stage_w.at[slot, c], sem_w.at[slot]).start()

    def wait_weights(slot):
        pltpu.make_async_copy(stage_w.at[slot], stage_w.at[slot], sem_w.at[slot]).wait()

    def wo_copy(j):
        return pltpu.make_async_copy(
            wo_hbm.at[:, pl.ds(pl.multiple_of(128 * j, 128), 128)], wo_v.at[j].bitcast(BF16), sem_wo)

    def x_copy(g):
        r = pl.ds(g * (n_seg // n_groups), n_seg // n_groups)
        return pltpu.make_async_copy(x_hbm.at[r], x_v.at[r], sem_x)

    def u_copy(g):
        return pltpu.make_async_copy(
            u_hbm.at[:, pl.ds(pl.multiple_of(g * GC, GC), GC)], u_v.at[g], sem_u.at[g])

    def par_copies():
        return [pltpu.make_async_copy(p, par_v.at[i], sem_par)
                for i, p in enumerate((are_hbm, aim_hbm, bre_hbm, bim_hbm, cre_hbm, cim_hbm))]

    def outb_copy(g):
        return pltpu.make_async_copy(outb_v.at[g], out_hbm.at[:, pl.ds(Dm + g * GC, GC)], sem_ob)

    def outa_copy(it):
        r = pl.ds(pl.multiple_of(it * unroll * seg, seg), unroll * seg)
        return pltpu.make_async_copy(outa_v.at[r, :], out_hbm.at[r, pl.ds(0, Dm)], sem_oa)

    xt_copy = pltpu.make_async_copy(x_hbm.at[:, pl.ds(seg - PRE, PRE), :], xt_v, sem_xt)

    for cp in par_copies():
        cp.start()
    u_copy(0).start()
    u_copy(1).start()

    def ahead(hg, unit):
        m = unit // n_rb
        rows = pl.ds(pl.multiple_of((unit - m * n_rb) * RB, RB), RB)
        pre_v[hg, m, rows, :] = _dot(xp_v[rows, :], pltpu.bitcast(w_vs[hg][m], BF16))

    def chan(k):
        return slice(k * PITCH, k * PITCH + n_blocks)

    def states(k):
        return slice(k * SPITCH, k * SPITCH + 2 * n_blocks)

    def group(part, carry, *, hg):
        g = hg * g_per_hg + part
        with_ahead = hg > 0
        next_unit = [part * units_per_group]

        def loop(n, n_units, body):
            assert n_units % n == 0
            per_iter = n_units // n
            first = next_unit[0]
            next_unit[0] = first + n_units

            def wrapped(i, c):
                todo = list(range(per_iter)) if with_ahead else []

                def fill(done, total):
                    while todo and todo[0] * total <= done * per_iter:
                        ahead(hg - 1, first + i * per_iter + todo.pop(0))

                body(i, fill)
                fill(1, 1)
                return c

            if not do_b:
                return
            with jax.named_scope(body.__name__ + ("+" if with_ahead else "")):
                if n == 1:
                    @pl.when(g >= 0)
                    def _():
                        wrapped(0, 0)
                else:
                    lax.fori_loop(0, n, wrapped, 0)

        with jax.named_scope('wait_u'):
            u_copy(g).wait()

        @pl.when(g + 2 < n_groups)
        def _():
            u_copy(g + 2).start()

        sel = lax.broadcasted_iota(jnp.int32, (n_groups, GC), 0) == g
        ldt = jnp.sum(jnp.where(sel, carry[0], 0.0), axis=0, keepdims=True)
        dsk = jnp.sum(jnp.where(sel, carry[1], 0.0), axis=0, keepdims=True)
        dt_row = jnp.exp(ldt).astype(BF16).astype(F32)
        dt_v[...] = jnp.broadcast_to(dt_row, (GC, GC)).T

        def powers(_, fill):
            for it in range(GC // pb):
                fill(2 * it, 2 * GC // pb)
                rows = pl.ds(pl.multiple_of(g * GC + it * pb, pb), pb)
                k0 = it * pb
                dt = dt_v[k0:k0 + pb, :]
                zr = dt * par_v[0, rows, :].astype(F32)
                zi = dt * par_v[1, rows, :].astype(F32)
                c_re, c_im = _cmul(par_v[4, rows, :].astype(F32), par_v[5, rows, :].astype(F32),
                                   dt * par_v[2, rows, :].astype(F32), dt * par_v[3, rows, :].astype(F32))
                mag = jnp.exp(zr)
                l1 = (mag * jnp.cos(zi), mag * jnp.sin(zi))
                fill(2 * it + 1, 2 * GC // pb)
                l2 = _cmul(*l1, *l1)
                l3 = _cmul(*l2, *l1)
                l4 = _cmul(*l2, *l2)
                pw = [(jnp.ones_like(mag), jnp.zeros_like(mag)), l1, l2, l3, l4,
                      _cmul(*l4, *l1), _cmul(*l4, *l2), _cmul(*l4, *l3)]
                for r in range(8):
                    bre_v[pl.ds(k0 * BPITCH + r, pb, stride=BPITCH), :] = pw[r][0]
                    bim_v[pl.ds(k0 * BPITCH + r, pb, stride=BPITCH), :] = pw[r][1]
                l8 = _cmul(*l4, *l4)
                lt = l8
                for _ in range(3):
                    lt = _cmul(*lt, *lt)
                cl = _cmul(c_re, c_im, *l1)
                for i, val in enumerate((lt[0], -lt[1], cl[0], cl[1], c_re, -c_im, *l8)):
                    cf_v[i, k0:k0 + pb, :] = val

        loop(1, u_pre, powers)

        ri = lax.broadcasted_iota(jnp.int32, (T, T), 0)
        ci = lax.broadcasted_iota(jnp.int32, (T, T), 1)
        flip = jnp.where((ri ^ ci) == TC - 1, 1.0, 0.0).astype(BF16)

        def u_blocks(q, fill):
            uts = [u_v[g, pl.ds(pl.multiple_of((q * n_q + c) * T, T), T), :].astype(F32).T
                   for c in range(n_q)]
            fill(0, 4)
            urev = _dot(jnp.concatenate(uts, axis=0), flip)
            for c in range(n_q):
                idx = pl.ds(q * n_q + c, GC, stride=PITCH)
                uf_v[idx, :] = uts[c]
                ur_v[idx, :] = urev[c * GC:(c + 1) * GC]

        loop(n_blocks // n_q, u_uc, u_blocks)

        @pl.when(part + 1 < g_per_hg)
        def _():
            start_weights(hg, part + 1, part + 1)

        if hg + 1 < n_hg:
            @pl.when(part + 1 == g_per_hg)
            def _():
                start_weights(hg + 1, 0, 0)

        wo_copy(g).start()
        x_copy(g).start()

        even = lax.broadcasted_iota(jnp.int32, (n_blocks, T), 1) < TC

        def state_in(it, fill):
            for k in range(GC):
                pr = [bre_v[k * BPITCH:k * BPITCH + 8, :]]
                pi = [bim_v[k * BPITCH:k * BPITCH + 8, :]]
                mr = jnp.broadcast_to(cf_v[6, k:k + 1, :], (8, 128))
                mi = jnp.broadcast_to(cf_v[7, k:k + 1, :], (8, 128))
                for _ in range(TC // 8 - 1):
                    nr, ni = _cmul(pr[-1], pi[-1], mr, mi)
                    pr.append(nr)
                    pi.append(ni)
                p_v[k] = jnp.concatenate(
                    [jnp.concatenate(pr, axis=0), jnp.concatenate(pi, axis=0)], axis=1).astype(BF16)
                ur = ur_v[chan(k), :]
                ur = jnp.concatenate([jnp.where(even, ur, 0.0), jnp.where(even, 0.0, ur)], axis=0)
                if k % 2 == 0:
                    fill(k, GC)
                sre_v[states(k), :] = _dot(ur, jnp.concatenate(pr + pr, axis=0).astype(BF16))
                sim_v[states(k), :] = _dot(ur, jnp.concatenate(pi + pi, axis=0).astype(BF16))

        loop(1, u_si, state_in)

        def scan(_, fill):
            width = sb if with_ahead else 32
            last = None
            for k0 in range(0, GC, width):
                ltr, lti, clr, cli, gr, gi = (cf_v[i, k0:k0 + width, :] for i in range(6))
                if last is not None:
                    clr, cli = jnp.where(g < 0, last, clr), jnp.where(g < 0, last, cli)
                nclr = -clr
                for c in range(2 * n_blocks):
                    fill(k0 * 2 * n_blocks + c * width, GC * 2 * n_blocks)
                    idx = pl.ds(k0 * SPITCH + (c % 2) * n_blocks + c // 2, width, stride=SPITCH)
                    gre_v[idx, :] = gr
                    gim_v[idx, :] = gi
                    if c < 2 * n_blocks - 1:
                        xr, xi = sre_v[idx, :], sim_v[idx, :]
                        sr, si = clr * xr - cli * xi, nclr * xi - cli * xr
                        if c == 0:
                            gr, gi = sr, si
                        else:
                            gr, gi = _cmul(gr, gi, ltr, lti)
                            gr, gi = gr + sr, gi + si
                last = gr

        loop(1, u_sc, scan)

        slot = part
        with jax.named_scope('wait_w'):
            wait_weights(slot)

        def relayout(t):
            i, pc = divmod(t, n_pc)
            src = stage_w.at[slot, i].bitcast(U32)
            rows = pl.ds(pl.multiple_of((part * n_pc + pc) * (DC // 2), DC // 2), DC // 2)
            for pp in range(4):
                ev = src[pl.ds(pc * DC * 4 + pp, DC // 2, stride=8), :]
                od = src[pl.ds(pc * DC * 4 + pp + 4, DC // 2, stride=8), :]
                w_vs[hg][8 * i + 2 * pp, rows, :] = (ev & 0xFFFF) | (od << 16)
                w_vs[hg][8 * i + 2 * pp + 1, rows, :] = (ev >> 16) | (od & jnp.uint32(0xFFFF0000))

        has_state = lax.broadcasted_iota(jnp.int32, (n_blocks, T), 0) > 0

        def state_out(it, fill):
            n_rl = 3 * n_pc
            for k in range(GC):
                if k * n_rl % GC < n_rl:
                    relayout(k * n_rl // GC)
                if k % 2 == 0:
                    fill(k, GC)
                gg = jnp.concatenate([gre_v[states(k), :], gim_v[states(k), :]], axis=1)
                p = p_v[k]
                y = _dot(gg, jnp.concatenate([p, jnp.zeros_like(p)], axis=0), NT)
                taps_v[8 * k:8 * k + 8, :] = y[0:8, :] + pltpu.roll(y[0:8, :], TC, 1)
                y_v[chan(k), :] = jnp.where(has_state, y[:n_blocks], 0.0) + pltpu.roll(y[n_blocks:], TC, 1)

        loop(1, u_so, state_out)

        ti = lax.broadcasted_iota(jnp.int32, (TC, T), 0)
        tj = lax.broadcasted_iota(jnp.int32, (TC, T), 1)
        causal_even = (tj >= ti) & (tj < TC)
        causal_odd = tj >= ti + TC

        def in_chunk(it, fill):
            for k in range(GC):
                if k % 4 == 0:
                    fill(k, GC)
                kb = jnp.broadcast_to(taps_v[8 * k:8 * k + 1, :], (TC, T))
                tz = pltpu.roll(kb, 0, 1, stride=1, stride_axis=0)
                tz = jnp.concatenate([jnp.where(causal_even, tz, 0.0),
                                      jnp.where(causal_odd, tz, 0.0)], axis=0)
                y_v[chan(k), :] += _dot(uf_v[chan(k), :], tz.astype(BF16))

        loop(1, u_ic, in_chunk)

        def y_blocks(q, fill):
            for c in range(n_q):
                fill(c, n_q)
                tt = pl.ds(pl.multiple_of((q * n_q + c) * T, T), T)
                yc = y_v[pl.ds(q * n_q + c, GC, stride=PITCH), :].T.astype(BF16).astype(F32)
                skip = (u_v[g, tt, :].astype(F32) * dsk).astype(BF16).astype(F32)
                outb_v[g, tt, :] = (yc + skip).astype(BF16)

        loop(n_blocks // n_q, u_yc, y_blocks)

        return carry

    vecs = (ldt_ref[...].astype(F32).reshape(n_groups, GC), dsk_ref[...].astype(F32).reshape(n_groups, GC))
    with jax.named_scope('wait_par'):
        for cp in par_copies():
            cp.wait()
    start_weights(0, 0, 0)
    xt_copy.start()

    lax.fori_loop(0, g_per_hg, functools.partial(group, hg=0), vecs)
    xt_copy.wait()

    def widen(q, carry):
        for c in range(8):
            s = q * 8 + c
            xp_v[pl.ds(pl.multiple_of(s * PRE, PRE), PRE), :] = xt_v[s].astype(F32)
        return carry

    lax.fori_loop(0, n_seg // 8, widen, 0)
    for hg in range(1, n_hg):
        lax.fori_loop(0, g_per_hg, functools.partial(group, hg=hg), vecs)
    for g in range(n_groups):
        outb_copy(g).start()
    with jax.named_scope('wait_x'):
        for g in range(n_groups):
            x_copy(g).wait()
            wo_copy(g).wait()

    scale = Dh ** -0.5
    qi = lax.broadcasted_iota(jnp.int32, (L, 128), 0)
    ki = lax.broadcasted_iota(jnp.int32, (L, 128), 1)
    keep = ((qi < n_mem) | (qi >= ki)) & (ki < L)
    masked = jnp.where(ki < L, -1000000000.0 / scale, -jnp.inf)
    zpad = jnp.zeros((128 - L, Dh), F32)
    HG = 8
    AG = 4
    n_og = n_heads // HG
    n_j = Dm // 128
    heads = [h % 4 * 8 + h // 4 for h in range(n_heads)] if perm else list(range(n_heads))

    def where(h, i):
        if order:
            return divmod(i * n_heads + h, 24)
        return h // 8, 8 * i + h % 8

    def step(s, cur, nxt, split):
        r = pl.ds(pl.multiple_of(s * seg, seg), seg)
        qs, ks, vs, es, os_ = {}, {}, {}, {}, {}

        def part(h, i, k0, k1):
            hg, m = where(h, i)
            rows = L - PRE if hg + 1 < n_hg and m < n_pre else L
            return _dot(h_v[cur, :rows, k0:k1], pltpu.bitcast(w_vs[hg][m, k0 // 2:k1 // 2, :], BF16))

        head_start = {divmod(t, 3): part(*divmod(t, 3), 0, Dm // 2) for t in range(split)}

        def proj(h, i):
            if (h, i) in head_start:
                res = head_start.pop((h, i)) + part(h, i, Dm // 2, Dm)
            else:
                res = part(h, i, 0, Dm)
            if res.shape[0] < L:
                hg, m = where(h, i)
                known = pre_v[hg, m, pl.ds(pl.multiple_of(s * PRE, PRE), PRE), :]
                res = jnp.concatenate([res, known], axis=0)
            return res

        def scores(h):
            sc = jnp.where(keep, _dot(qs.pop(h), ks.pop(h), NT), masked)
            e = jnp.exp2((sc - jnp.max(sc, axis=1, keepdims=True)) * (scale * LOG2E))
            total = jnp.sum(e, axis=1, keepdims=True)
            inv = pl.reciprocal(total, approx=True)
            es[h] = (e, inv * (2.0 - total * inv))

        def mix(h):
            e, inv = es.pop(h)
            os_[h] = _dot(e, vs.pop(h)) * inv

        def oproj(j, g):
            hs = heads[g * HG:(g + 1) * HG]
            w = jnp.concatenate([wo_v[j, h * Dh // 2:(h + 1) * Dh // 2, :] for h in hs], axis=0)
            return _dot(jnp.concatenate([os_[h] for h in hs], axis=1), pltpu.bitcast(w, BF16))

        def emit(j, res):
            h_v[nxt, :n_mem, 128 * j:128 * (j + 1)] = res[:n_mem]
            outa_v[r, 128 * j:128 * (j + 1)] = res[n_mem:].astype(BF16)

        for h0 in range(0, n_heads, AG):
            for i in range(AG):
                h = heads[h0 + i]
                qs[h] = proj(h, 0)
                if h0 and i == lag0:
                    for hh in heads[h0 - AG:h0]:
                        scores(hh)
                ks[h] = jnp.concatenate([proj(h, 1), zpad], axis=0).astype(BF16)
                if h0 and i == lag:
                    for hh in heads[h0 - AG:h0]:
                        mix(hh)
                vs[h] = jnp.concatenate([proj(h, 2), zpad], axis=0).astype(BF16)

        h_v[nxt, n_mem:, :] = x_v[jnp.minimum(s + 1, n_seg - 1)].astype(F32)

        acc = {}

        def early(t):
            j, g = divmod(t, n_og - 1)
            acc[j] = oproj(j, g) if g == 0 else acc[j] + oproj(j, g)

        t = 0
        for _ in range(pre_n):
            early(t)
            t += 1
        for hh in heads[n_heads - AG:]:
            scores(hh)
        for _ in range(fill_n):
            early(t)
            t += 1
        for hh in heads[n_heads - AG:]:
            mix(hh)
        for _ in range(3):
            early(t)
            t += 1
        for j in range(n_j):
            while t < (j + 1) * (n_og - 1):
                early(t)
                t += 1
            emit(j, acc.pop(j) + oproj(j, n_og - 1))

    def steps(it, carry):
        for c in range(unroll):
            step(it * unroll + c, c % 2, (c + 1) % 2, split if c else 0)
        outa_copy(it).start()
        return carry

    h_v[0, :n_mem, :] = mem0_ref[...].astype(F32)
    h_v[0, n_mem:, :] = x_v[0].astype(F32)
    with jax.named_scope('steps'):
        lax.fori_loop(0, n_seg // unroll, steps, 0)

    for g in range(n_groups):
        outb_copy(g).wait()

    def drain(s, carry):
        outa_copy(s).wait()
        return carry

    lax.fori_loop(0, n_seg // unroll, drain, 0)


@functools.partial(jax.jit, static_argnames=(
    "A_seg_len", "pb", "lag", "fill_n", "unroll", "units", "RB", "sb", "nq", "flags", "order", "perm", "lag0", "pre_n", "split", "do_b"))
def pallas_concat_heads__memory_aug_recurrent_mem_tr__ssm_conv_s4__prompt_kernel(A_x, A_mem0, A_Wq, A_Wk, A_Wv, A_Wo, A_seg_len, B_u, B_A_re, B_A_im, B_B_re, B_B_im,
           B_C_re, B_C_im, B_log_dt, B_Dskip, pb=32, lag=3, fill_n=7, unroll=4,
           units="12,16,4,24,12,16,12", RB=64, sb=8, nq=8, flags="", split=0, order=1, perm=1, lag0=1, pre_n=3, do_b=True):
    Bsz, S, Dm = A_x.shape
    H, Dh = A_Wq.shape[1], A_Wq.shape[2]
    M = A_mem0.shape[1]
    D, N = B_A_re.shape
    seg = int(A_seg_len)
    assert Bsz == 1 and Dh == 128 and N == 128 and D == Dm and B_u.shape == A_x.shape
    L = M + seg
    n_seg = S // seg
    n_groups = D // GC
    n_slots = n_groups // (H // 8)
    if isinstance(units, str):
        units = tuple(int(c) for c in units.split(','))

    def head_tiles(w):
        return w.reshape(Dm, H // 8, 8, Dh).transpose(0, 2, 1, 3).reshape(Dm * 8, H // 8 * Dh)

    any_spec = pl.BlockSpec(memory_space=pl.ANY)
    vmem_spec = pl.BlockSpec(memory_space=pltpu.VMEM)
    out = pl.pallas_call(
        functools.partial(_kernel, n_mem=M, n_heads=H, pb=pb, lag=lag, fill_n=fill_n, unroll=unroll,
                          units=units, RB=RB, sb=sb, n_q=nq, split=split, order=order, perm=perm, lag0=lag0, pre_n=pre_n, do_b=do_b),
        out_shape=jax.ShapeDtypeStruct((S, Dm + D), BF16),
        in_specs=[any_spec, vmem_spec] + [any_spec] * 11 + [vmem_spec, vmem_spec],
        out_specs=any_spec,
        scratch_shapes=[
            pltpu.VMEM((n_seg, seg, Dm), BF16),
            pltpu.VMEM((n_seg, PRE, Dm), BF16),
            pltpu.VMEM((n_seg * PRE, Dm), F32),
            pltpu.VMEM((n_groups, S, GC), BF16),
            pltpu.VMEM((6, D, N), BF16),
            pltpu.VMEM((n_slots, 3, Dm * 8 // n_slots, 128), BF16),
            *[pltpu.VMEM((24, Dm // 2, Dh), U32)] * (H // 8),
            pltpu.VMEM((Dm // 128, H * Dh // 2, 128), U32),
            pltpu.VMEM((H // 8 - 1, 24, n_seg * PRE, Dh), F32),
            pltpu.VMEM((S, Dm), BF16),
            pltpu.VMEM((n_groups, S, GC), BF16),
            pltpu.VMEM((2, L, Dm), F32),
            pltpu.VMEM((GC, N), F32),
            pltpu.VMEM((GC * BPITCH, N), F32),
            pltpu.VMEM((GC * BPITCH, N), F32),
            pltpu.VMEM((8, GC, N), F32),
            pltpu.VMEM((GC, TC, 2 * N), BF16),
            pltpu.VMEM((GC * PITCH, T), F32),
            pltpu.VMEM((GC * PITCH, T), F32),
            pltpu.VMEM((GC * SPITCH, N), F32),
            pltpu.VMEM((GC * SPITCH, N), F32),
            pltpu.VMEM((GC * SPITCH, N), F32),
            pltpu.VMEM((GC * SPITCH, N), F32),
            pltpu.VMEM((GC * PITCH, T), F32),
            pltpu.VMEM((GC * 8, T), F32),
            pltpu.SemaphoreType.DMA(()),
            pltpu.SemaphoreType.DMA(()),
            pltpu.SemaphoreType.DMA((n_groups,)),
            pltpu.SemaphoreType.DMA(()),
            pltpu.SemaphoreType.DMA((n_slots,)),
            pltpu.SemaphoreType.DMA(()),
            pltpu.SemaphoreType.DMA(()),
            pltpu.SemaphoreType.DMA(()),
        ],
        compiler_params=pltpu.CompilerParams(vmem_limit_bytes=120 * 1024 * 1024, flags={f: True for f in flags.split(',') if f} or None),
    )(A_x.reshape(n_seg, seg, Dm), A_mem0.reshape(M, Dm),
      head_tiles(A_Wq), head_tiles(A_Wk), head_tiles(A_Wv), A_Wo.reshape(H * Dh, Dm),
      B_u.reshape(S, D), B_A_re, B_A_im, B_B_re, B_B_im, B_C_re, B_C_im, B_log_dt, B_Dskip)
    return out.reshape(Bsz, S, Dm + D)
```

```python
import functools
import math

import jax
import jax.numpy as jnp
from jax import lax
import jax.experimental.pallas as pl
import jax.experimental.pallas.tpu as pltpu

F32 = jnp.float32
BF16 = jnp.bfloat16
U32 = jnp.uint32

NN = (((1,), (0,)), ((), ()))
NT = (((1,), (1,)), ((), ()))

T = 128
TC = T // 2
GC = 128
PITCH = 17
SPITCH = 33
BPITCH = 9
LOG2E = math.log2(math.e)
PRE = 8


PLANS = {
    0: (("in", {"in": 0}), ("scan_out", {"scan": 0, "out": 2}), ("chunk", {"chunk": 0})),
    1: (("in", {"in": 0}), ("rest", {"scan": 0, "out": 2, "chunk": 4})),
    2: (("all", {"in": 0, "scan": 2, "out": 4, "chunk": 6}),),
    3: (("in_scan", {"in": 0, "scan": 2}), ("out_chunk", {"out": 0, "chunk": 2})),
    4: (("in", {"in": 0}), ("rest", {"scan": 0, "out": 1, "chunk": 3})),
}


def _dot(a, b, dims=NN):
    return lax.dot_general(a, b, dims, preferred_element_type=F32)


def _cmul(ar, ai, br, bi):
    return ar * br - ai * bi, ar * bi + ai * br


def _kernel(x_hbm, mem0_hbm, wq_hbm, wk_hbm, wv_hbm, wo_hbm,
            u_hbm, are_hbm, aim_hbm, bre_hbm, bim_hbm, cre_hbm, cim_hbm, ldt_hbm, dsk_hbm,
            out_hbm,
            x_v, xt_v, xp_v, u_v, par_v, stage_w, w0_v, w1_v, w2_v, w3_v, wo_v, pre_v, outa_v, outb_v, h_v,
            bre_v, bim_v, cf_v, p_v, uf_v, ur_v, sre_v, sim_v, gre_v, gim_v, y_v, taps_v,
            mem0_v, ldt_v, dsk_v, sem_s, sem_x, sem_xt, sem_u, sem_par, sem_w, sem_wo, sem_oa, sem_ob,
            *, n_mem, n_heads, pb, lag, fill_n, unroll, units, RB, sbs, n_q, split, order, perm, lag0, pre_n, mlag, do_b):
    n_seg, seg, Dm = x_v.shape
    S = n_seg * seg
    n_groups = Dm // GC
    n_blocks = S // T
    L = n_mem + seg
    Dh = 128
    n_slots = stage_w.shape[0]
    DC = 128
    n_pc = stage_w.shape[2] // (8 * DC)
    n_rb = n_seg * PRE // RB
    w_vs = (w0_v, w1_v, w2_v, w3_v)
    n_hg = len(w_vs)
    g_per_hg = n_groups // n_hg
    u_pre, u_yc = units[0], units[-1]
    plan = PLANS[mlag]
    units_per_group = sum(units)
    assert units_per_group * g_per_hg % n_rb == 0
    n_pre = units_per_group * g_per_hg // n_rb
    assert n_pre <= pre_v.shape[1]

    def start_weights(hg, part, slot):
        for c in range(3):
            if order:
                i, tile = divmod(3 * hg + c, n_hg)
            else:
                tile, i = divmod(3 * hg + c, 3)
            rows = pl.ds(pl.multiple_of(part * (n_pc * DC * 8), DC * 8), n_pc * DC * 8)
            pltpu.make_async_copy((wq_hbm, wk_hbm, wv_hbm)[i].at[rows, pl.ds(tile * 128, 128)],
                                  stage_w.at[slot, c], sem_w.at[slot]).start()

    def wait_weights(slot):
        pltpu.make_async_copy(stage_w.at[slot], stage_w.at[slot], sem_w.at[slot]).wait()

    def wo_copy(j):
        return pltpu.make_async_copy(
            wo_hbm.at[:, pl.ds(pl.multiple_of(128 * j, 128), 128)], wo_v.at[j].bitcast(BF16), sem_wo)

    def x_copy(g):
        r = pl.ds(g * (n_seg // n_groups), n_seg // n_groups)
        return pltpu.make_async_copy(x_hbm.at[r], x_v.at[r], sem_x)

    def u_copy(g):
        return pltpu.make_async_copy(
            u_hbm.at[:, pl.ds(pl.multiple_of(g * GC, GC), GC)], u_v.at[g], sem_u.at[g])

    def par_copies(g):
        rows = pl.ds(pl.multiple_of(g * GC, GC), GC)
        return [pltpu.make_async_copy(p.at[rows, :], par_v.at[i, rows, :], sem_par.at[g])
                for i, p in enumerate((are_hbm, aim_hbm, bre_hbm, bim_hbm, cre_hbm, cim_hbm))]

    def outb_copy(g):
        return pltpu.make_async_copy(outb_v.at[g], out_hbm.at[:, pl.ds(Dm + g * GC, GC)], sem_ob)

    def outa_copy(it):
        r = pl.ds(pl.multiple_of(it * unroll * seg, seg), unroll * seg)
        return pltpu.make_async_copy(outa_v.at[r, :], out_hbm.at[r, pl.ds(0, Dm)], sem_oa)

    xt_copy = pltpu.make_async_copy(x_hbm.at[:, pl.ds(seg - PRE, PRE), :], xt_v, sem_xt)

    for cp in par_copies(0):
        cp.start()
    u_copy(0).start()
    small = [pltpu.make_async_copy(src, dst, sem_s.at[i]) for i, (src, dst) in
             enumerate(((ldt_hbm, ldt_v), (dsk_hbm, dsk_v), (mem0_hbm, mem0_v)))]
    for cp in small:
        cp.start()

    def ahead(hg, unit, never, after):
        m = unit // n_rb
        rows = pl.ds(pl.multiple_of((unit - m * n_rb) * RB, RB), RB)
        lhs = xp_v[rows, :]
        if after is not None:
            corner = jnp.where(never, after, lhs[:8, :128])
            lhs = jnp.concatenate([jnp.concatenate([corner, lhs[:8, 128:]], axis=1), lhs[8:]], axis=0)
        pre_v[hg, m, rows, :] = _dot(lhs, pltpu.bitcast(w_vs[hg][m], BF16))

    def chan(k):
        return slice(k * PITCH, k * PITCH + n_blocks)

    def states(k):
        return slice(k * SPITCH, k * SPITCH + 2 * n_blocks)

    def group(part, carry, *, hg):
        g = hg * g_per_hg + part
        ldt_all, dsk_all = carry
        with_ahead = hg > 0
        next_unit = [part * units_per_group]

        def loop(n, n_units, body):
            assert n_units % n == 0
            per_iter = n_units // n
            first = next_unit[0]
            next_unit[0] = first + n_units

            def wrapped(i, c):
                todo = list(range(per_iter)) if with_ahead else []

                def fill(done, total, after=()):
                    while todo and todo[0] * total <= done * per_iter:
                        rows = [v[r:r + 8] for v in after for r in range(0, v.shape[0], 8)]
                        ahead(hg - 1, first + i * per_iter + todo.pop(0), g < 0,
                              functools.reduce(jnp.add, rows) if rows else None)
                        after = ()

                body(i, fill)
                fill(1, 1)
                return c

            if not do_b:
                return
            with jax.named_scope(body.__name__ + ("+" if with_ahead else "")):
                if n == 1:
                    @pl.when(g >= 0)
                    def _():
                        wrapped(0, 0)
                else:
                    lax.fori_loop(0, n, wrapped, 0)

        with jax.named_scope('wait_par'):
            for cp in par_copies(g):
                cp.wait()

        if hg == 0:
            @pl.when(part == 0)
            def _():
                start_weights(0, 0, 0)

        @pl.when(g + 1 < n_groups)
        def _():
            for cp in par_copies(g + 1):
                cp.start()
            u_copy(g + 1).start()

        sel = lax.broadcasted_iota(jnp.int32, (n_groups, GC), 0) == g

        def prepare(_, fill):
            fill(0, 1)
            ldt = jnp.sum(jnp.where(sel, ldt_all, 0.0), axis=0, keepdims=True)
            dt_row = jnp.exp(ldt).astype(BF16).astype(F32)
            dt_all = jnp.broadcast_to(dt_row, (GC, GC)).T
            n_part = 2 * GC // pb
            done = ()
            for it in range(GC // pb):
                fill(2 * it, n_part)
                rows = pl.ds(pl.multiple_of(g * GC + it * pb, pb), pb)
                k0 = it * pb
                dt = dt_all[k0:k0 + pb]
                zr = dt * par_v[0, rows, :].astype(F32)
                zi = dt * par_v[1, rows, :].astype(F32)
                c_re, c_im = _cmul(par_v[4, rows, :].astype(F32), par_v[5, rows, :].astype(F32),
                                   dt * par_v[2, rows, :].astype(F32), dt * par_v[3, rows, :].astype(F32))
                mag = jnp.exp(zr)
                l1 = (mag * jnp.cos(zi), mag * jnp.sin(zi))
                u_blocks(it * n_blocks * pb // GC, n_blocks * pb // GC)
                fill(2 * it + 1, n_part, done)
                l2 = _cmul(*l1, *l1)
                l3 = _cmul(*l2, *l1)
                l4 = _cmul(*l2, *l2)
                pw = [(jnp.ones_like(mag), jnp.zeros_like(mag)), l1, l2, l3, l4,
                      _cmul(*l4, *l1), _cmul(*l4, *l2), _cmul(*l4, *l3)]
                for r in range(8):
                    bre_v[pl.ds(k0 * BPITCH + r, pb, stride=BPITCH), :] = pw[r][0]
                    bim_v[pl.ds(k0 * BPITCH + r, pb, stride=BPITCH), :] = pw[r][1]
                l8 = _cmul(*l4, *l4)
                lt = l8
                for _ in range(3):
                    lt = _cmul(*lt, *lt)
                cl = _cmul(c_re, c_im, *l1)
                for i, val in enumerate((lt[0], -lt[1], cl[0], cl[1], c_re, -c_im, *l8)):
                    cf_v[i, k0:k0 + pb, :] = val
                done = (*pw[5], *pw[6], *pw[7], *lt, *cl)

        ri = lax.broadcasted_iota(jnp.int32, (T, T), 0)
        ci = lax.broadcasted_iota(jnp.int32, (T, T), 1)
        flip = jnp.where((ri ^ ci) == TC - 1, 1.0, 0.0).astype(BF16)

        def u_blocks(c0, count):
            uts = [u_v[g, c * T:(c + 1) * T, :].astype(F32).T for c in range(c0, c0 + count)]
            urev = _dot(jnp.concatenate(uts, axis=0), flip)
            for c in range(count):
                idx = pl.ds(c0 + c, GC, stride=PITCH)
                uf_v[idx, :] = uts[c]
                ur_v[idx, :] = urev[c * GC:(c + 1) * GC]

        u_copy(g).wait()
        loop(1, u_pre, prepare)

        even = lax.broadcasted_iota(jnp.int32, (n_blocks, T), 1) < TC

        def read_in(k):
            if True:
                pr = [bre_v[k * BPITCH:k * BPITCH + 8, :]]
                pi = [bim_v[k * BPITCH:k * BPITCH + 8, :]]
                mr = jnp.broadcast_to(cf_v[6, k:k + 1, :], (8, 128))
                mi = jnp.broadcast_to(cf_v[7, k:k + 1, :], (8, 128))
                for _ in range(TC // 8 - 1):
                    nr, ni = _cmul(pr[-1], pi[-1], mr, mi)
                    pr.append(nr)
                    pi.append(ni)
                p_v[k] = jnp.concatenate(
                    [jnp.concatenate(pr, axis=0), jnp.concatenate(pi, axis=0)], axis=1).astype(BF16)
                ur = ur_v[chan(k), :]
                ur = jnp.concatenate([jnp.where(even, ur, 0.0), jnp.where(even, 0.0, ur)], axis=0)
                sre_v[states(k), :] = _dot(ur, jnp.concatenate(pr + pr, axis=0).astype(BF16))
                sim_v[states(k), :] = _dot(ur, jnp.concatenate(pi + pi, axis=0).astype(BF16))


        has_state = lax.broadcasted_iota(jnp.int32, (n_blocks, T), 0) > 0

        def scan_batch(k0, width, last, fill):
            ltr, lti, clr, cli, gr, gi = (cf_v[i, k0:k0 + width, :] for i in range(6))
            if last is not None:
                clr, cli = jnp.where(g < 0, last, clr), jnp.where(g < 0, last, cli)
            nclr = -clr
            for c in range(2 * n_blocks):
                fill(k0 * 2 * n_blocks + c * width, GC * 2 * n_blocks)
                idx = pl.ds(k0 * SPITCH + (c % 2) * n_blocks + c // 2, width, stride=SPITCH)
                gre_v[idx, :] = gr
                gim_v[idx, :] = gi
                if c < 2 * n_blocks - 1:
                    xr, xi = sre_v[idx, :], sim_v[idx, :]
                    sr, si = clr * xr - cli * xi, nclr * xi - cli * xr
                    if c == 0:
                        gr, gi = sr, si
                    else:
                        gr, gi = _cmul(gr, gi, ltr, lti)
                        gr, gi = gr + sr, gi + si
            return gr

        def read_out(k):
            gg = jnp.concatenate([gre_v[states(k), :], gim_v[states(k), :]], axis=1)
            p = p_v[k]
            y = _dot(gg, jnp.concatenate([p, jnp.zeros_like(p)], axis=0), NT)
            taps_v[8 * k:8 * k + 8, :] = y[0:8, :] + pltpu.roll(y[0:8, :], TC, 1)
            y_v[chan(k), :] = jnp.where(has_state, y[:n_blocks], 0.0) + pltpu.roll(y[n_blocks:], TC, 1)

        slot = part
        def weights_ready():
            with jax.named_scope('wait_w'):
                wait_weights(slot)

            @pl.when(part + 1 < g_per_hg)
            def _():
                start_weights(hg, part + 1, part + 1)

            if hg + 1 < n_hg:
                @pl.when(part + 1 == g_per_hg)
                def _():
                    start_weights(hg + 1, 0, 0)

            if hg == 0:
                @pl.when(part == 0)
                def _():
                    xt_copy.start()

            wo_copy(g).start()
            x_copy(g).start()

        def relayout(t):
            i, pc = divmod(t, n_pc)
            src = stage_w.at[slot, i].bitcast(U32)
            rows = pl.ds(pl.multiple_of((part * n_pc + pc) * (DC // 2), DC // 2), DC // 2)
            for pp in range(4):
                ev = src[pl.ds(pc * DC * 4 + pp, DC // 2, stride=8), :]
                od = src[pl.ds(pc * DC * 4 + pp + 4, DC // 2, stride=8), :]
                w_vs[hg][8 * i + 2 * pp, rows, :] = (ev & 0xFFFF) | (od << 16)
                w_vs[hg][8 * i + 2 * pp + 1, rows, :] = (ev >> 16) | (od & jnp.uint32(0xFFFF0000))

        ti = lax.broadcasted_iota(jnp.int32, (TC, T), 0)
        tj = lax.broadcasted_iota(jnp.int32, (TC, T), 1)
        causal_even = (tj >= ti) & (tj < TC)
        causal_odd = tj >= ti + TC

        def in_chunk(k):
            kb = jnp.broadcast_to(taps_v[8 * k:8 * k + 1, :], (TC, T))
            tz = pltpu.roll(kb, 0, 1, stride=1, stride_axis=0)
            tz = jnp.concatenate([jnp.where(causal_even, tz, 0.0),
                                  jnp.where(causal_odd, tz, 0.0)], axis=0)
            y_v[chan(k), :] += _dot(uf_v[chan(k), :], tz.astype(BF16))

        def stage(name, n_units, lags):
            sb = sbs[with_ahead]
            n_slot = GC // sb + max(lags.values())
            n_rl = 3 * n_pc if "chunk" in lags else 0

            def body(_, fill):
                last = None
                for j in range(n_slot):
                    if 0 <= j - lags.get("scan", n_slot) < GC // sb:
                        last = scan_batch((j - lags["scan"]) * sb, sb, last, lambda *_: None)
                    for t in range(j * n_rl // n_slot, (j + 1) * n_rl // n_slot):
                        relayout(t)
                    for c in range(sb):
                        if c % 2 == 0:
                            fill(j * sb + c, n_slot * sb)
                        for work, fn in (("in", read_in), ("out", read_out), ("chunk", in_chunk)):
                            if 0 <= j - lags.get(work, n_slot) < GC // sb:
                                fn((j - lags[work]) * sb + c)

            body.__name__ = name
            loop(1, n_units, body)

        for (name, lags), n_units in zip(plan, units[1:-1]):
            if "chunk" in dict(lags):
                weights_ready()
            stage(name, n_units, dict(lags))

        def y_blocks(q, fill):
            dsk = jnp.sum(jnp.where(sel, dsk_all, 0.0), axis=0, keepdims=True)
            done = [(), ()]
            for c in range(n_q):
                fill(c, n_q, done.pop(0))
                tt = pl.ds(pl.multiple_of((q * n_q + c) * T, T), T)
                yc = y_v[pl.ds(q * n_q + c, GC, stride=PITCH), :].T.astype(BF16).astype(F32)
                skip = (u_v[g, tt, :].astype(F32) * dsk).astype(BF16).astype(F32)
                outb_v[g, tt, :] = (yc + skip).astype(BF16)
                done.append((yc + skip,))

        loop(n_blocks // n_q, u_yc, y_blocks)

        return carry

    for cp in small:
        cp.wait()
    vecs = (ldt_v[...].astype(F32).reshape(n_groups, GC), dsk_v[...].astype(F32).reshape(n_groups, GC))

    lax.fori_loop(0, g_per_hg, functools.partial(group, hg=0), vecs)
    xt_copy.wait()

    def widen(q, carry):
        for c in range(8):
            s = q * 8 + c
            xp_v[pl.ds(pl.multiple_of(s * PRE, PRE), PRE), :] = xt_v[s].astype(F32)
        return carry

    with jax.named_scope('widen'):
        lax.fori_loop(0, n_seg // 8, widen, 0)
    for hg in range(1, n_hg):
        lax.fori_loop(0, g_per_hg, functools.partial(group, hg=hg), vecs)
    for g in range(n_groups):
        outb_copy(g).start()
    with jax.named_scope('wait_x'):
        for g in range(n_groups):
            x_copy(g).wait()
            wo_copy(g).wait()

    scale = Dh ** -0.5
    qi = lax.broadcasted_iota(jnp.int32, (L, 128), 0)
    ki = lax.broadcasted_iota(jnp.int32, (L, 128), 1)
    keep = ((qi < n_mem) | (qi >= ki)) & (ki < L)
    masked = jnp.where(ki < L, -1000000000.0 / scale, -jnp.inf)
    zpad = jnp.zeros((128 - L, Dh), F32)
    HG = 8
    AG = 4
    n_og = n_heads // HG
    n_j = Dm // 128
    heads = [h % 4 * 8 + h // 4 for h in range(n_heads)] if perm else list(range(n_heads))

    def where(h, i):
        if order:
            return divmod(i * n_heads + h, 24)
        return h // 8, 8 * i + h % 8

    def step(s, cur, nxt, split):
        r = pl.ds(pl.multiple_of(s * seg, seg), seg)
        qs, ks, vs, es, os_ = {}, {}, {}, {}, {}

        def part(h, i, k0, k1):
            hg, m = where(h, i)
            rows = L - PRE if hg + 1 < n_hg and m < n_pre else L
            return _dot(h_v[cur, :rows, k0:k1], pltpu.bitcast(w_vs[hg][m, k0 // 2:k1 // 2, :], BF16))

        head_start = {divmod(t, 3): part(*divmod(t, 3), 0, Dm // 2) for t in range(split)}

        def proj(h, i):
            if (h, i) in head_start:
                res = head_start.pop((h, i)) + part(h, i, Dm // 2, Dm)
            else:
                res = part(h, i, 0, Dm)
            if res.shape[0] < L:
                hg, m = where(h, i)
                known = pre_v[hg, m, pl.ds(pl.multiple_of(s * PRE, PRE), PRE), :]
                res = jnp.concatenate([res, known], axis=0)
            return res

        def scores(h):
            sc = jnp.where(keep, _dot(qs.pop(h), ks.pop(h), NT), masked)
            e = jnp.exp2((sc - jnp.max(sc, axis=1, keepdims=True)) * (scale * LOG2E))
            total = jnp.sum(e, axis=1, keepdims=True)
            inv = pl.reciprocal(total, approx=True)
            es[h] = (e, inv * (2.0 - total * inv))

        def mix(h):
            e, inv = es.pop(h)
            os_[h] = _dot(e, vs.pop(h)) * inv

        def oproj(j, g):
            hs = heads[g * HG:(g + 1) * HG]
            w = jnp.concatenate([wo_v[j, h * Dh // 2:(h + 1) * Dh // 2, :] for h in hs], axis=0)
            return _dot(jnp.concatenate([os_[h] for h in hs], axis=1), pltpu.bitcast(w, BF16))

        def emit(j, res):
            h_v[nxt, :n_mem, 128 * j:128 * (j + 1)] = res[:n_mem]
            outa_v[r, 128 * j:128 * (j + 1)] = res[n_mem:].astype(BF16)

        for h0 in range(0, n_heads, AG):
            for i in range(AG):
                h = heads[h0 + i]
                qs[h] = proj(h, 0)
                if h0 and i == lag0:
                    for hh in heads[h0 - AG:h0]:
                        scores(hh)
                ks[h] = jnp.concatenate([proj(h, 1), zpad], axis=0).astype(BF16)
                if h0 and i == lag:
                    for hh in heads[h0 - AG:h0]:
                        mix(hh)
                vs[h] = jnp.concatenate([proj(h, 2), zpad], axis=0).astype(BF16)

        h_v[nxt, n_mem:, :] = x_v[jnp.minimum(s + 1, n_seg - 1)].astype(F32)

        acc = {}

        def early(t):
            j, g = divmod(t, n_og - 1)
            acc[j] = oproj(j, g) if g == 0 else acc[j] + oproj(j, g)

        t = 0
        for _ in range(pre_n):
            early(t)
            t += 1
        for hh in heads[n_heads - AG:]:
            scores(hh)
        for _ in range(fill_n):
            early(t)
            t += 1
        for hh in heads[n_heads - AG:]:
            mix(hh)
        for _ in range(3):
            early(t)
            t += 1
        for j in range(n_j):
            while t < (j + 1) * (n_og - 1):
                early(t)
                t += 1
            emit(j, acc.pop(j) + oproj(j, n_og - 1))

    def steps(it, carry):
        for c in range(unroll):
            step(it * unroll + c, c % 2, (c + 1) % 2, split if c else 0)
        outa_copy(it).start()
        return carry

    h_v[0, :n_mem, :] = mem0_v[...].astype(F32)
    h_v[0, n_mem:, :] = x_v[0].astype(F32)
    with jax.named_scope('steps'):
        lax.fori_loop(0, n_seg // unroll, steps, 0)

    for g in range(n_groups):
        outb_copy(g).wait()

    def drain(s, carry):
        outa_copy(s).wait()
        return carry

    with jax.named_scope('drain'):
        lax.fori_loop(0, n_seg // unroll, drain, 0)


@functools.partial(jax.jit, static_argnames=(
    "A_seg_len", "pb", "lag", "fill_n", "unroll", "units", "RB", "sb", "sb0", "nq", "flags", "order", "perm", "lag0", "pre_n", "mlag", "split", "nochk", "do_b"))
def pallas_concat_heads__memory_aug_recurrent_mem_tr__ssm_conv_s4__prompt_kernel(A_x, A_mem0, A_Wq, A_Wk, A_Wv, A_Wo, A_seg_len, B_u, B_A_re, B_A_im, B_B_re, B_B_im,
           B_C_re, B_C_im, B_log_dt, B_Dskip, pb=32, lag=3, fill_n=7, unroll=4,
           units="12,6,10,14,6", RB=128, sb=8, sb0=16, nq=16, flags="", split=0, order=1, perm=1, lag0=1, pre_n=3, mlag=0, nochk=1, do_b=True):
    Bsz, S, Dm = A_x.shape
    H, Dh = A_Wq.shape[1], A_Wq.shape[2]
    M = A_mem0.shape[1]
    D, N = B_A_re.shape
    seg = int(A_seg_len)
    assert Bsz == 1 and Dh == 128 and N == 128 and D == Dm and B_u.shape == A_x.shape
    L = M + seg
    n_seg = S // seg
    n_groups = D // GC
    n_slots = n_groups // (H // 8)
    if isinstance(units, str):
        units = tuple(int(c) for c in units.split(','))

    def head_tiles(w):
        return w.reshape(Dm, H // 8, 8, Dh).transpose(0, 2, 1, 3).reshape(Dm * 8, H // 8 * Dh)

    any_spec = pl.BlockSpec(memory_space=pl.ANY)
    vmem_spec = pl.BlockSpec(memory_space=pltpu.VMEM)
    out = pl.pallas_call(
        functools.partial(_kernel, n_mem=M, n_heads=H, pb=pb, lag=lag, fill_n=fill_n, unroll=unroll,
                          units=units, RB=RB, sbs=(sb0, sb), n_q=nq, split=split, order=order, perm=perm, lag0=lag0, pre_n=pre_n, mlag=mlag, do_b=do_b),
        out_shape=jax.ShapeDtypeStruct((S, Dm + D), BF16),
        in_specs=[any_spec] * 15,
        out_specs=any_spec,
        scratch_shapes=[
            pltpu.VMEM((n_seg, seg, Dm), BF16),
            pltpu.VMEM((n_seg, PRE, Dm), BF16),
            pltpu.VMEM((n_seg * PRE, Dm), F32),
            pltpu.VMEM((n_groups, S, GC), BF16),
            pltpu.VMEM((6, D, N), BF16),
            pltpu.VMEM((n_slots, 3, Dm * 8 // n_slots, 128), BF16),
            *[pltpu.VMEM((24, Dm // 2, Dh), U32)] * (H // 8),
            pltpu.VMEM((Dm // 128, H * Dh // 2, 128), U32),
            pltpu.VMEM((H // 8 - 1, 24, n_seg * PRE, Dh), F32),
            pltpu.VMEM((S, Dm), BF16),
            pltpu.VMEM((n_groups, S, GC), BF16),
            pltpu.VMEM((2, L, Dm), F32),
            pltpu.VMEM((GC * BPITCH, N), F32),
            pltpu.VMEM((GC * BPITCH, N), F32),
            pltpu.VMEM((8, GC, N), F32),
            pltpu.VMEM((GC, TC, 2 * N), BF16),
            pltpu.VMEM((GC * PITCH, T), F32),
            pltpu.VMEM((GC * PITCH, T), F32),
            pltpu.VMEM((GC * SPITCH, N), F32),
            pltpu.VMEM((GC * SPITCH, N), F32),
            pltpu.VMEM((GC * SPITCH, N), F32),
            pltpu.VMEM((GC * SPITCH, N), F32),
            pltpu.VMEM((GC * PITCH, T), F32),
            pltpu.VMEM((GC * 8, T), F32),
            pltpu.VMEM((M, Dm), BF16),
            pltpu.VMEM((D,), BF16),
            pltpu.VMEM((D,), BF16),
            pltpu.SemaphoreType.DMA((3,)),
            pltpu.SemaphoreType.DMA(()),
            pltpu.SemaphoreType.DMA(()),
            pltpu.SemaphoreType.DMA((n_groups,)),
            pltpu.SemaphoreType.DMA((n_groups,)),
            pltpu.SemaphoreType.DMA((n_slots,)),
            pltpu.SemaphoreType.DMA(()),
            pltpu.SemaphoreType.DMA(()),
            pltpu.SemaphoreType.DMA(()),
        ],
        compiler_params=pltpu.CompilerParams(vmem_limit_bytes=120 * 1024 * 1024, disable_bounds_checks=bool(nochk), flags={f: True for f in flags.split(',') if f} or None),
    )(A_x.reshape(n_seg, seg, Dm), A_mem0.reshape(M, Dm),
      head_tiles(A_Wq), head_tiles(A_Wk), head_tiles(A_Wv), A_Wo.reshape(H * Dh, Dm),
      B_u.reshape(S, D), B_A_re, B_A_im, B_B_re, B_B_im, B_C_re, B_C_im, B_log_dt, B_Dskip)
    return out.reshape(Bsz, S, Dm + D)
```

```python
import functools
import math

import jax
import jax.numpy as jnp
import numpy as np
from jax import lax
import jax.experimental.pallas as pl
import jax.experimental.pallas.tpu as pltpu

F32 = jnp.float32
BF16 = jnp.bfloat16
U32 = jnp.uint32

NN = (((1,), (0,)), ((), ()))
NT = (((1,), (1,)), ((), ()))
LOG2E = math.log2(math.e)

T = 128
TC = T // 2
GC = 128
PB = 32
PITCH = 17
SPITCH = 33
BPITCH = 9
HT = 8
DC = 128
PRE = 8
HG = 8
AG = 4


def _dot(a, b, dims=NN):
    return lax.dot_general(a, b, dims, preferred_element_type=F32)


def _cmul(ar, ai, br, bi):
    return ar * br - ai * bi, ar * bi + ai * br


def _kernel(zero_ref, x_hbm, mem0_hbm, wq_hbm, wk_hbm, wv_hbm, wo_hbm,
            u_hbm, are_hbm, aim_hbm, bre_hbm, bim_hbm, cre_hbm, cim_hbm, ldt_hbm, dsk_hbm,
            out_hbm,
            x_v, xt_v, xp_v, u_v, par_v, stage_v, w_v, wo_v, pre_v, outa_v, outb_v, h_v,
            bre_v, bim_v, cf_v, p_v, uf_v, ur_v, sre_v, sim_v, gre_v, gim_v, y_v, taps_v,
            mem0_v, ldt_v, dsk_v,
            sem_s, sem_x, sem_xt, sem_u, sem_par, sem_w, sem_wo, sem_oa, sem_ob,
            *, unroll, quota, pieces, RB, sizes, do_b):
    n_seg, seg, Dm = x_v.shape
    n_mem = mem0_v.shape[0]
    Dh = w_v.shape[2]
    n_heads = w_v.shape[0] // 3
    n_groups = Dm // GC
    n_blocks = n_seg * seg // T
    L = n_mem + seg
    n_slots = stage_v.shape[0]
    n_tiles = 3 * n_heads // HT
    n_dc = Dm // DC
    n_rb = n_seg * PRE // RB
    n_pre = pre_v.shape[0]

    always = zero_ref[0] == 0
    never = zero_ref[0] != 0

    def w_copy(c):
        i, tile = divmod(c, n_heads // HT)
        return pltpu.make_async_copy((wq_hbm, wk_hbm, wv_hbm)[i].at[:, pl.ds(tile * Dh, Dh)],
                                     stage_v.at[c % n_slots, pl.ds(0, Dm * HT), :], sem_w.at[c % n_slots])

    def wo_copy(j):
        return pltpu.make_async_copy(wo_hbm.at[:, pl.ds(128 * j, 128)], wo_v.at[j].bitcast(BF16), sem_wo)

    def x_copy(g):
        r = pl.ds(g * (n_seg // n_groups), n_seg // n_groups)
        return pltpu.make_async_copy(x_hbm.at[r], x_v.at[r], sem_x)

    def group_copies(g):
        ch = pl.ds(g * GC, GC)
        return [pltpu.make_async_copy(p.at[ch, :], par_v.at[i, ch, :], sem_par.at[g])
                for i, p in enumerate((are_hbm, aim_hbm, bre_hbm, bim_hbm, cre_hbm, cim_hbm))] + [
                    pltpu.make_async_copy(u_hbm.at[:, ch], u_v.at[g], sem_u.at[g])]

    def outb_copy(g):
        return pltpu.make_async_copy(outb_v.at[g], out_hbm.at[:, pl.ds(Dm + g * GC, GC)], sem_ob)

    def outa_copy(it):
        r = pl.ds(pl.multiple_of(it * unroll * seg, seg), unroll * seg)
        return pltpu.make_async_copy(outa_v.at[r, :], out_hbm.at[r, pl.ds(0, Dm)], sem_oa)

    xt_copy = pltpu.make_async_copy(x_hbm.at[:, pl.ds(seg - PRE, PRE), :], xt_v, sem_xt)
    small = [pltpu.make_async_copy(src, dst, sem_s.at[i]) for i, (src, dst) in
             enumerate(((ldt_hbm, ldt_v), (dsk_hbm, dsk_v), (mem0_hbm, mem0_v)))]

    def relayout(piece):
        c, pc = divmod(piece, n_dc)
        src = stage_v.at[c % n_slots].bitcast(U32)
        rows = slice(pc * DC // 2, (pc + 1) * DC // 2)
        done = []
        for pp in range(HT // 2):
            ev = src[pl.ds(pc * DC * HT // 2 + pp, DC // 2, stride=HT), :]
            od = src[pl.ds(pc * DC * HT // 2 + pp + HT // 2, DC // 2, stride=HT), :]
            done += [(ev & 0xFFFF) | (od << 16), (ev >> 16) | (od & jnp.uint32(0xFFFF0000))]
            w_v[c * HT + 2 * pp, rows, :] = done[-2]
            w_v[c * HT + 2 * pp + 1, rows, :] = done[-1]
        return [lax.bitcast_convert_type(v, F32) for v in done]

    def ahead(unit, size, after):
        m, rb = divmod(unit, n_rb)
        rows = slice(rb * RB, (rb + size) * RB)
        lhs = xp_v[rows, :]
        if after is not None:
            corner = jnp.where(never, after, lhs[:8, :128])
            lhs = jnp.concatenate([jnp.concatenate([corner, lhs[:8, 128:]], axis=1), lhs[8:]], axis=0)
        pre_v[m, rows, :] = _dot(lhs, pltpu.bitcast(w_v[m], BF16))

    progress = {"piece": 0, "unit": 0}

    def stage(body, n_units=0, n_pieces=0, size=2):
        p0 = progress["piece"]
        p1 = min(p0 + n_pieces, n_tiles * n_dc)
        u0 = progress["unit"]
        u1 = min(u0 + n_units, p0 // n_dc * HT * n_rb, n_pre * n_rb)
        progress.update(piece=p1, unit=u1)
        for c in range(-(-p0 // n_dc), -(-p1 // n_dc)):
            with jax.named_scope(f"wait_w{c}"):
                w_copy(c).wait()
        todo_p, todo_u, pending = list(range(p0, p1)), list(range(u0, u1, size)), []
        assert u0 % 2 == 0 and u1 % 2 == 0

        def fill(done, total, after=()):
            while todo_u and (todo_u[0] - u0) * total <= done * (u1 - u0):
                rows = [v[r:r + 8] for v in (*after, *pending) for r in range(0, v.shape[0], 8)]
                ahead(todo_u.pop(0), size, functools.reduce(jnp.add, rows) if rows else None)
                after = ()
                pending.clear()
            while todo_p and (todo_p[0] - p0) * total <= done * (p1 - p0 + 1):
                pending.extend(relayout(todo_p.pop(0)))

        with jax.named_scope(body.__name__ + ("+" if u1 > u0 else "")):
            @pl.when(always)
            def _():
                if do_b:
                    body(fill)
                fill(1, 1)

        for c in range(p0 // n_dc, p1 // n_dc):
            if c + n_slots < n_tiles:
                w_copy(c + n_slots).start()

    def chan(k):
        return slice(k * PITCH, k * PITCH + n_blocks)

    def states(k):
        return slice(k * SPITCH, k * SPITCH + 2 * n_blocks)

    def ssm_group(g):
        ch = slice(g * GC, (g + 1) * GC)

        def prepare(fill):
            fill(0, 1)
            dt = jnp.exp(ldt_v[ch].astype(F32).reshape(1, GC)).astype(BF16).astype(F32)
            dt = jnp.broadcast_to(dt, (GC, GC)).T
            ri = lax.broadcasted_iota(jnp.int32, (T, T), 0)
            ci = lax.broadcasted_iota(jnp.int32, (T, T), 1)
            flip = jnp.where((ri ^ ci) == TC - 1, 1.0, 0.0).astype(BF16)
            n_part = 2 * GC // PB
            done = ()
            for k0 in range(0, GC, PB):
                fill(2 * k0 // PB, n_part)
                a_re, a_im, b_re, b_im, c_re, c_im = (
                    par_v[i, g * GC + k0:g * GC + k0 + PB, :].astype(F32) for i in range(6))
                step = dt[k0:k0 + PB]
                w_re, w_im = _cmul(c_re, c_im, step * b_re, step * b_im)
                mag = jnp.exp(step * a_re)
                l1 = (mag * jnp.cos(step * a_im), mag * jnp.sin(step * a_im))
                blocks = range(k0 * n_blocks // GC, (k0 + PB) * n_blocks // GC)
                uts = [u_v[g, c * T:(c + 1) * T, :].astype(F32).T for c in blocks]
                urev = _dot(jnp.concatenate(uts, axis=0), flip)
                for i, c in enumerate(blocks):
                    uf_v[pl.ds(c, GC, stride=PITCH), :] = uts[i]
                    ur_v[pl.ds(c, GC, stride=PITCH), :] = urev[i * GC:(i + 1) * GC]
                fill(2 * k0 // PB + 1, n_part, done)
                l2 = _cmul(*l1, *l1)
                l3 = _cmul(*l2, *l1)
                l4 = _cmul(*l2, *l2)
                pw = [(jnp.ones_like(mag), jnp.zeros_like(mag)), l1, l2, l3, l4,
                      _cmul(*l4, *l1), _cmul(*l4, *l2), _cmul(*l4, *l3)]
                for r in range(8):
                    bre_v[pl.ds(k0 * BPITCH + r, PB, stride=BPITCH), :] = pw[r][0]
                    bim_v[pl.ds(k0 * BPITCH + r, PB, stride=BPITCH), :] = pw[r][1]
                l8 = _cmul(*l4, *l4)
                lt = l8
                for _ in range(3):
                    lt = _cmul(*lt, *lt)
                wl = _cmul(w_re, w_im, *l1)
                for i, val in enumerate((lt[0], -lt[1], wl[0], wl[1], w_re, -w_im, *l8)):
                    cf_v[i, k0:k0 + PB, :] = val
                done = (*pw[5], *pw[6], *pw[7], *lt, *wl)

        def read_in(fill):
            even = lax.broadcasted_iota(jnp.int32, (n_blocks, T), 1) < TC
            for k in range(GC):
                if k % 2 == 0:
                    fill(k, GC)
                pr = [bre_v[k * BPITCH:k * BPITCH + 8, :]]
                pi = [bim_v[k * BPITCH:k * BPITCH + 8, :]]
                mr = jnp.broadcast_to(cf_v[6, k:k + 1, :], (8, 128))
                mi = jnp.broadcast_to(cf_v[7, k:k + 1, :], (8, 128))
                for _ in range(TC // 8 - 1):
                    nr, ni = _cmul(pr[-1], pi[-1], mr, mi)
                    pr.append(nr)
                    pi.append(ni)
                p_v[k] = jnp.concatenate(
                    [jnp.concatenate(pr, axis=0), jnp.concatenate(pi, axis=0)], axis=1).astype(BF16)
                ur = ur_v[chan(k), :]
                ur = jnp.concatenate([jnp.where(even, ur, 0.0), jnp.where(even, 0.0, ur)], axis=0)
                sre_v[states(k), :] = _dot(ur, jnp.concatenate(pr + pr, axis=0).astype(BF16))
                sim_v[states(k), :] = _dot(ur, jnp.concatenate(pi + pi, axis=0).astype(BF16))

        def scan(k0, width, last):
            ltr, lti, wlr, wli, gr, gi = (cf_v[i, k0:k0 + width, :] for i in range(6))
            if last is not None:
                wlr, wli = jnp.where(never, last, wlr), jnp.where(never, last, wli)
            nwlr = -wlr
            for c in range(2 * n_blocks):
                idx = pl.ds(k0 * SPITCH + (c % 2) * n_blocks + c // 2, width, stride=SPITCH)
                gre_v[idx, :] = gr
                gim_v[idx, :] = gi
                if c < 2 * n_blocks - 1:
                    xr, xi = sre_v[idx, :], sim_v[idx, :]
                    sr, si = wlr * xr - wli * xi, nwlr * xi - wli * xr
                    if c == 0:
                        gr, gi = sr, si
                    else:
                        gr, gi = _cmul(gr, gi, ltr, lti)
                        gr, gi = gr + sr, gi + si
            return gr

        def read_out(fill):
            has_state = lax.broadcasted_iota(jnp.int32, (n_blocks, T), 0) > 0
            width, lag = (8 if g else 16), 2
            last = None
            for k0 in range(0, GC + lag * width, width):
                if k0 < GC:
                    last = scan(k0, width, last)
                for k in range(k0 - lag * width, k0 - (lag - 1) * width):
                    if k % 2 == 0:
                        fill(k + lag * width, GC + lag * width)
                    if k < 0:
                        continue
                    gg = jnp.concatenate([gre_v[states(k), :], gim_v[states(k), :]], axis=1)
                    p = p_v[k]
                    y = _dot(gg, jnp.concatenate([p, jnp.zeros_like(p)], axis=0), NT)
                    taps_v[8 * k:8 * k + 8, :] = y[0:8, :] + pltpu.roll(y[0:8, :], TC, 1)
                    y_v[chan(k), :] = (jnp.where(has_state, y[:n_blocks], 0.0)
                                       + pltpu.roll(y[n_blocks:], TC, 1))

        def in_chunk(fill):
            ti = lax.broadcasted_iota(jnp.int32, (TC, T), 0)
            tj = lax.broadcasted_iota(jnp.int32, (TC, T), 1)
            causal_even = (tj >= ti) & (tj < TC)
            causal_odd = tj >= ti + TC
            for k in range(GC):
                if k % 2 == 0:
                    fill(k, GC)
                kb = jnp.broadcast_to(taps_v[8 * k:8 * k + 1, :], (TC, T))
                tz = pltpu.roll(kb, 0, 1, stride=1, stride_axis=0)
                tz = jnp.concatenate([jnp.where(causal_even, tz, 0.0),
                                      jnp.where(causal_odd, tz, 0.0)], axis=0)
                y_v[chan(k), :] += _dot(uf_v[chan(k), :], tz.astype(BF16))

        def finish(fill):
            dsk = dsk_v[ch].astype(F32).reshape(1, GC)
            done = [(), ()]
            for c in range(n_blocks):
                fill(c, n_blocks, done.pop(0))
                rows = slice(c * T, (c + 1) * T)
                yc = y_v[pl.ds(c, GC, stride=PITCH), :].T.astype(BF16).astype(F32)
                yc = yc + (u_v[g, rows, :].astype(F32) * dsk).astype(BF16).astype(F32)
                outb_v[g, rows, :] = yc.astype(BF16)
                done.append((yc,))

        def first_weights(fill):
            for s in range(n_seg):
                xp_v[s * PRE:(s + 1) * PRE, :] = xt_v[s].astype(F32)

        with jax.named_scope(f"wait_g{g}"):
            for cp in group_copies(g):
                cp.wait()
        if g == 0:
            w_copy(0).start()
            xt_copy.start()
        elif g + 1 < n_groups:
            for cp in group_copies(g + 1):
                cp.start()
        if 1 <= g <= n_groups // 2:
            for j in (2 * g - 2, 2 * g - 1):
                wo_copy(j).start()
                x_copy(j).start()
        stage(prepare, quota[0], n_dc if g == 1 else 0, sizes[0])
        stage(read_in, quota[1], pieces[1] if g else 0, sizes[1])
        stage(read_out, quota[2], pieces[2] if g else 0, sizes[2])
        if g == 0:
            with jax.named_scope('wait_xt'):
                xt_copy.wait()
            for cp in group_copies(1):
                cp.start()
            w_copy(1).start()
            stage(first_weights, 0, n_dc)
            for c in range(2, n_slots):
                w_copy(c).start()
        stage(in_chunk, quota[3], pieces[3] if g else 0)
        stage(finish, quota[4] if g + 1 < n_groups else n_pre * n_rb, pieces[4] if g else 0)

    for cp in small + group_copies(0):
        cp.start()
    with jax.named_scope("wait_small"):
        for cp in small:
            cp.wait()
    for g in range(n_groups):
        ssm_group(g)
    assert progress == {"piece": n_tiles * n_dc, "unit": n_pre * n_rb}, progress
    with jax.named_scope("wait_x"):
        for g in range(n_groups):
            x_copy(g).wait()
            wo_copy(g).wait()
    for g in range(n_groups):
        outb_copy(g).start()

    scale = Dh ** -0.5
    qi = lax.broadcasted_iota(jnp.int32, (L, 128), 0)
    ki = lax.broadcasted_iota(jnp.int32, (L, 128), 1)
    keep = ((qi < n_mem) | (qi >= ki)) & (ki < L)
    masked = jnp.where(ki < L, -1000000000.0 / scale, -jnp.inf)
    zpad = jnp.zeros((128 - L, Dh), F32)
    n_og = n_heads // HG
    heads = [h % AG * (n_heads // AG) + h // AG for h in range(n_heads)]

    def step(s, cur, nxt):
        r = pl.ds(pl.multiple_of(s * seg, seg), seg)
        qs, ks, vs, es, os_, acc = {}, {}, {}, {}, {}, {}

        def proj(i, h):
            m = i * n_heads + h
            w = pltpu.bitcast(w_v[m], BF16)
            if m >= n_pre:
                return _dot(h_v[cur], w)
            known = pre_v[m, pl.ds(pl.multiple_of(s * PRE, PRE), PRE), :]
            return jnp.concatenate([_dot(h_v[cur, :L - PRE, :], w), known], axis=0)

        def scores(h):
            sc = jnp.where(keep, _dot(qs.pop(h), ks.pop(h), NT), masked)
            e = jnp.exp2((sc - jnp.max(sc, axis=1, keepdims=True)) * (scale * LOG2E))
            total = jnp.sum(e, axis=1, keepdims=True)
            inv = pl.reciprocal(total, approx=True)
            es[h] = (e, inv * (2.0 - total * inv))

        def mix(h):
            e, inv = es.pop(h)
            os_[h] = _dot(e, vs.pop(h)) * inv

        def oproj(j, g):
            hs = heads[g * HG:(g + 1) * HG]
            w = jnp.concatenate([wo_v[j, h * Dh // 2:(h + 1) * Dh // 2, :] for h in hs], axis=0)
            return _dot(jnp.concatenate([os_[h] for h in hs], axis=1), pltpu.bitcast(w, BF16))

        early = [divmod(t, n_og - 1) for t in range(Dm // 128 * (n_og - 1))]

        def oproj_early(count):
            for _ in range(count):
                j, g = early.pop(0)
                acc[j] = acc[j] + oproj(j, g) if g else oproj(j, g)

        for h0 in range(0, n_heads, AG):
            before = heads[max(h0 - AG, 0):h0]
            for i, h in enumerate(heads[h0:h0 + AG]):
                qs[h] = proj(0, h)
                if i == 1:
                    for hh in before:
                        scores(hh)
                ks[h] = jnp.concatenate([proj(1, h), zpad], axis=0).astype(BF16)
                if i == AG - 1:
                    for hh in before:
                        mix(hh)
                vs[h] = jnp.concatenate([proj(2, h), zpad], axis=0).astype(BF16)

        h_v[nxt, n_mem:, :] = x_v[jnp.minimum(s + 1, n_seg - 1)].astype(F32)

        oproj_early(3)
        for hh in heads[n_heads - AG:]:
            scores(hh)
        oproj_early(7)
        for hh in heads[n_heads - AG:]:
            mix(hh)
        oproj_early(3)
        for j in range(Dm // 128):
            oproj_early(sum(jj <= j for jj, _ in early))
            res = acc.pop(j) + oproj(j, n_og - 1)
            h_v[nxt, :n_mem, 128 * j:128 * (j + 1)] = res[:n_mem]
            outa_v[r, 128 * j:128 * (j + 1)] = res[n_mem:].astype(BF16)

    def steps(it, carry):
        for c in range(unroll):
            step(it * unroll + c, c % 2, (c + 1) % 2)
        outa_copy(it).start()
        return carry

    h_v[0, :n_mem, :] = mem0_v[...].astype(F32)
    h_v[0, n_mem:, :] = x_v[0].astype(F32)
    with jax.named_scope("steps"):
        lax.fori_loop(0, n_seg // unroll, steps, 0)

    for g in range(n_groups):
        outb_copy(g).wait()

    def drain(it, carry):
        outa_copy(it).wait()
        return carry

    lax.fori_loop(0, n_seg // unroll, drain, 0)


@functools.partial(jax.jit, static_argnames=("A_seg_len", "unroll", "quota", "pieces", "RB", "sizes", "n_pre", "do_b"))
def pallas_concat_heads__memory_aug_recurrent_mem_tr__ssm_conv_s4__prompt_kernel(
    A_x, A_mem0, A_Wq, A_Wk, A_Wv, A_Wo, A_seg_len,
    B_u, B_A_re, B_A_im, B_B_re, B_B_im, B_C_re, B_C_im, B_log_dt, B_Dskip,
    unroll=2, quota="20,18,16,26,10", pieces="0,0,0,12,0", RB=64, sizes="1,1,2", n_pre=80, do_b=True,
):
    Bsz, S, Dm = A_x.shape
    H, Dh = A_Wq.shape[1], A_Wq.shape[2]
    M = A_mem0.shape[1]
    D, N = B_A_re.shape
    seg = int(A_seg_len)
    assert Bsz == 1 and Dh == 128 and N == 128 and D == Dm and B_u.shape == A_x.shape
    n_seg = S // seg
    n_groups = D // GC
    n_slots = 3
    quota, pieces, sizes = (tuple(int(c) for c in v.split(",")) for v in (quota, pieces, sizes))

    def head_tiles(w):
        return w.reshape(Dm, H // HT, HT, Dh).transpose(0, 2, 1, 3).reshape(Dm * HT, H // HT * Dh)

    def pitched(pitch):
        return pltpu.VMEM(((GC + 8) * pitch, N), F32)

    any_spec = pl.BlockSpec(memory_space=pl.ANY)
    out = pl.pallas_call(
        functools.partial(_kernel, unroll=unroll, quota=quota, pieces=pieces, RB=RB, sizes=sizes, do_b=do_b),
        out_shape=jax.ShapeDtypeStruct((S, Dm + D), BF16),
        in_specs=[pl.BlockSpec(memory_space=pltpu.SMEM)] + [any_spec] * 15,
        out_specs=any_spec,
        scratch_shapes=[
            pltpu.VMEM((n_seg, seg, Dm), BF16),
            pltpu.VMEM((n_seg, PRE, Dm), BF16),
            pltpu.VMEM((n_seg * PRE, Dm), F32),
            pltpu.VMEM((n_groups, S, GC), BF16),
            pltpu.VMEM((6, D, N), BF16),
            pltpu.VMEM((n_slots, Dm * HT + 32, Dh), BF16),
            pltpu.VMEM((3 * H, Dm // 2, Dh), U32),
            pltpu.VMEM((Dm // 128, H * Dh // 2, 128), U32),
            pltpu.VMEM((n_pre, n_seg * PRE, Dh), F32),
            pltpu.VMEM((S, Dm), BF16),
            pltpu.VMEM((n_groups, S, GC), BF16),
            pltpu.VMEM((2, M + seg, Dm), F32),
            pitched(BPITCH), pitched(BPITCH),
            pltpu.VMEM((8, GC, N), F32),
            pltpu.VMEM((GC, TC, 2 * N), BF16),
            pitched(PITCH), pitched(PITCH),
            pitched(SPITCH), pitched(SPITCH),
            pitched(SPITCH), pitched(SPITCH),
            pitched(PITCH),
            pltpu.VMEM((GC * 8, T), F32),
            pltpu.VMEM((M, Dm), BF16),
            pltpu.VMEM((D,), BF16),
            pltpu.VMEM((D,), BF16),
            pltpu.SemaphoreType.DMA((3,)),
            pltpu.SemaphoreType.DMA(()),
            pltpu.SemaphoreType.DMA(()),
            pltpu.SemaphoreType.DMA((n_groups,)),
            pltpu.SemaphoreType.DMA((n_groups,)),
            pltpu.SemaphoreType.DMA((n_slots,)),
            pltpu.SemaphoreType.DMA(()),
            pltpu.SemaphoreType.DMA(()),
            pltpu.SemaphoreType.DMA(()),
        ],
        compiler_params=pltpu.CompilerParams(vmem_limit_bytes=120 * 1024 * 1024),
    )(np.zeros((1,), np.int32), A_x.reshape(n_seg, seg, Dm), A_mem0.reshape(M, Dm),
      head_tiles(A_Wq), head_tiles(A_Wk), head_tiles(A_Wv), A_Wo.reshape(H * Dh, Dm),
      B_u.reshape(S, D), B_A_re, B_A_im, B_B_re, B_B_im, B_C_re, B_C_im, B_log_dt, B_Dskip)
    return out.reshape(Bsz, S, Dm + D)
```

```python
import functools
import math

import jax
import jax.numpy as jnp
import numpy as np
from jax import lax
import jax.experimental.pallas as pl
import jax.experimental.pallas.tpu as pltpu

F32 = jnp.float32
BF16 = jnp.bfloat16
U32 = jnp.uint32

NN = (((1,), (0,)), ((), ()))
NT = (((1,), (1,)), ((), ()))
LOG2E = math.log2(math.e)

T = 128
TC = T // 2
GC = 128
PB = 32
PITCH = 17
SPITCH = 33
BPITCH = 9
HT = 8
DC = 128
PRE = 8
HG = 8
AG = 4


def _dot(a, b, dims=NN):
    return lax.dot_general(a, b, dims, preferred_element_type=F32)


def _cmul(ar, ai, br, bi):
    return ar * br - ai * bi, ar * bi + ai * br


def _reverse_chunks(v):
    row = lax.broadcasted_iota(jnp.int32, (8, v.shape[1]), 0)

    def reverse8(p):
        p = pltpu.roll(p, 4, 0)
        p = jnp.where((row & 2) == 0, pltpu.roll(p, 6, 0), pltpu.roll(p, 2, 0))
        return jnp.where((row & 1) == 0, pltpu.roll(p, 7, 0), pltpu.roll(p, 1, 0))

    order = [i ^ (TC // 8 - 1) for i in range(v.shape[0] // 8)]
    return jnp.concatenate([reverse8(v[8 * i:8 * i + 8]) for i in order], axis=0)


def _kernel(zero_ref, x_hbm, mem0_hbm, wq_hbm, wk_hbm, wv_hbm, wo_hbm,
            u_hbm, are_hbm, aim_hbm, bre_hbm, bim_hbm, cre_hbm, cim_hbm, ldt_hbm, dsk_hbm,
            out_hbm,
            x_v, xt_v, xp_v, u_v, par_v, stage_v, w_v, wo_v, pre_v, outa_v, outb_v, h_v,
            bre_v, bim_v, cf_v, p_v, uf_v, ur_v, sre_v, sim_v, gre_v, gim_v, y_v, taps_v,
            mem0_v, ldt_v, dsk_v,
            sem_s, sem_x, sem_xt, sem_u, sem_par, sem_w, sem_wo, sem_oa, sem_ob,
            *, unroll, quota, pieces, RB, sizes, pb, plag, ser, do_b):
    n_seg, seg, Dm = x_v.shape
    n_mem = mem0_v.shape[0]
    Dh = w_v.shape[2]
    n_heads = w_v.shape[0] // 3
    n_groups = Dm // GC
    n_blocks = n_seg * seg // T
    L = n_mem + seg
    n_slots = stage_v.shape[0]
    n_tiles = 3 * n_heads // HT
    n_dc = Dm // DC
    n_rb = n_seg * PRE // RB
    n_pre = pre_v.shape[0]

    always = zero_ref[0] == 0
    never = zero_ref[0] != 0

    def w_copy(c):
        i, tile = divmod(c, n_heads // HT)
        return pltpu.make_async_copy((wq_hbm, wk_hbm, wv_hbm)[i].at[:, pl.ds(tile * Dh, Dh)],
                                     stage_v.at[c % n_slots, pl.ds(0, Dm * HT), :], sem_w.at[c % n_slots])

    def wo_copy(j):
        return pltpu.make_async_copy(wo_hbm.at[:, pl.ds(128 * j, 128)], wo_v.at[j].bitcast(BF16), sem_wo)

    def x_copy(g):
        r = pl.ds(g * (n_seg // n_groups), n_seg // n_groups)
        return pltpu.make_async_copy(x_hbm.at[r], x_v.at[r], sem_x)

    def group_copies(g):
        ch = pl.ds(g * GC, GC)
        return [pltpu.make_async_copy(p.at[ch, :], par_v.at[i, ch, :], sem_par.at[g])
                for i, p in enumerate((are_hbm, aim_hbm, bre_hbm, bim_hbm, cre_hbm, cim_hbm))] + [
                    pltpu.make_async_copy(u_hbm.at[:, ch], u_v.at[g], sem_u.at[g])]

    def outb_copy(g):
        return pltpu.make_async_copy(outb_v.at[g], out_hbm.at[:, pl.ds(Dm + g * GC, GC)], sem_ob)

    def outa_copy(it):
        r = pl.ds(pl.multiple_of(it * unroll * seg, seg), unroll * seg)
        return pltpu.make_async_copy(outa_v.at[r, :], out_hbm.at[r, pl.ds(0, Dm)], sem_oa)

    xt_copy = pltpu.make_async_copy(x_hbm.at[:, pl.ds(seg - PRE, PRE), :], xt_v, sem_xt)
    small = [pltpu.make_async_copy(src, dst, sem_s.at[i]) for i, (src, dst) in
             enumerate(((ldt_hbm, ldt_v), (dsk_hbm, dsk_v), (mem0_hbm, mem0_v)))]

    def relayout(piece):
        c, pc = divmod(piece, n_dc)
        src = stage_v.at[c % n_slots].bitcast(U32)
        rows = slice(pc * DC // 2, (pc + 1) * DC // 2)
        done = []
        for pp in range(HT // 2):
            ev = src[pl.ds(pc * DC * HT // 2 + pp, DC // 2, stride=HT), :]
            od = src[pl.ds(pc * DC * HT // 2 + pp + HT // 2, DC // 2, stride=HT), :]
            done += [(ev & 0xFFFF) | (od << 16), (ev >> 16) | (od & jnp.uint32(0xFFFF0000))]
            w_v[c * HT + 2 * pp, rows, :] = done[-2]
            w_v[c * HT + 2 * pp + 1, rows, :] = done[-1]
        return [lax.bitcast_convert_type(v, F32) for v in done]

    def ahead(unit, size, after):
        m, rb = divmod(unit, n_rb)
        rows = slice(rb * RB, (rb + size) * RB)
        lhs = xp_v[rows, :]
        if after is not None:
            corner = jnp.where(never, after, lhs[:8, :128])
            lhs = jnp.concatenate([jnp.concatenate([corner, lhs[:8, 128:]], axis=1), lhs[8:]], axis=0)
        pre_v[m, rows, :] = _dot(lhs, pltpu.bitcast(w_v[m], BF16))

    progress = {"piece": 0, "unit": 0}

    def stage(body, n_units=0, n_pieces=0, size=2):
        p0 = progress["piece"]
        p1 = min(p0 + n_pieces, n_tiles * n_dc)
        u0 = progress["unit"]
        u1 = min(u0 + n_units, p0 // n_dc * HT * n_rb, n_pre * n_rb)
        progress.update(piece=p1, unit=u1)
        for c in range(-(-p0 // n_dc), -(-p1 // n_dc)):
            with jax.named_scope(f"wait_w{c}"):
                w_copy(c).wait()
        todo_p, todo_u, pending = list(range(p0, p1)), list(range(u0, u1, size)), []
        assert u0 % 2 == 0 and u1 % 2 == 0

        def fill(done, total, after=()):
            pending.extend(after)
            while todo_u and (todo_u[0] - u0) * total <= done * (u1 - u0):
                rows = [v[r:r + 8] for v in pending for r in range(0, v.shape[0], 8)]
                ahead(todo_u.pop(0), size, functools.reduce(jnp.add, rows) if rows else None)
                pending.clear()
            while todo_p and (todo_p[0] - p0) * total <= done * (p1 - p0 + 1):
                pending.extend(relayout(todo_p.pop(0)))

        with jax.named_scope(body.__name__ + ("+" if u1 > u0 else "")):
            @pl.when(always)
            def _():
                if do_b:
                    body(fill)
                fill(1, 1)

        for c in range(p0 // n_dc, p1 // n_dc):
            if c + n_slots < n_tiles:
                w_copy(c + n_slots).start()

    def chan(k):
        return slice(k * PITCH, k * PITCH + n_blocks)

    def states(k):
        return slice(k * SPITCH, k * SPITCH + 2 * n_blocks)

    def ssm_group(g):
        ch = slice(g * GC, (g + 1) * GC)

        def prepare(fill):
            fill(0, 1)
            dt = jnp.exp(ldt_v[ch].astype(F32).reshape(1, GC)).astype(BF16).astype(F32)
            dt = jnp.broadcast_to(dt, (GC, GC)).T
            done = [()] * plag
            for c in range(n_blocks):
                fill(c, n_blocks, done.pop(0))
                ub = u_v[g, c * T:(c + 1) * T, :].astype(F32)
                if c and ser & 2:
                    ub = jnp.where(never, flipped, ub)
                plain, flipped = ub.T, _reverse_chunks(ub).astype(BF16).T.astype(F32)
                uf_v[pl.ds(c, GC, stride=PITCH), :] = plain
                ur_v[pl.ds(c, GC, stride=PITCH), :] = flipped
                done.append((plain[-8:], flipped[-8:]))
                k0 = c * GC // n_blocks
                if k0 % pb:
                    continue
                a_re, a_im, b_re, b_im, c_re, c_im = (
                    par_v[i, g * GC + k0:g * GC + k0 + pb, :].astype(F32) for i in range(6))
                step = dt[k0:k0 + pb]
                if k0 and ser & 1:
                    step = jnp.where(never, wl[0], step)
                w_re, w_im = _cmul(c_re, c_im, step * b_re, step * b_im)
                mag = jnp.exp(step * a_re)
                l1 = (mag * jnp.cos(step * a_im), mag * jnp.sin(step * a_im))
                l2 = _cmul(*l1, *l1)
                l3 = _cmul(*l2, *l1)
                l4 = _cmul(*l2, *l2)
                pw = [(jnp.ones_like(mag), jnp.zeros_like(mag)), l1, l2, l3, l4,
                      _cmul(*l4, *l1), _cmul(*l4, *l2), _cmul(*l4, *l3)]
                for r in range(8):
                    bre_v[pl.ds(k0 * BPITCH + r, pb, stride=BPITCH), :] = pw[r][0]
                    bim_v[pl.ds(k0 * BPITCH + r, pb, stride=BPITCH), :] = pw[r][1]
                l8 = _cmul(*l4, *l4)
                lt = l8
                for _ in range(3):
                    lt = _cmul(*lt, *lt)
                wl = _cmul(w_re, w_im, *l1)
                for i, val in enumerate((lt[0], -lt[1], wl[0], wl[1], w_re, -w_im, *l8)):
                    cf_v[i, k0:k0 + pb, :] = val
                done[-1] += (*pw[5], *pw[6], *pw[7], *lt, *wl)

        def read_in(fill):
            even = lax.broadcasted_iota(jnp.int32, (n_blocks, T), 1) < TC
            for k in range(GC):
                if k % 2 == 0:
                    fill(k, GC)
                pr = [bre_v[k * BPITCH:k * BPITCH + 8, :]]
                pi = [bim_v[k * BPITCH:k * BPITCH + 8, :]]
                mr = jnp.broadcast_to(cf_v[6, k:k + 1, :], (8, 128))
                mi = jnp.broadcast_to(cf_v[7, k:k + 1, :], (8, 128))
                for _ in range(TC // 8 - 1):
                    nr, ni = _cmul(pr[-1], pi[-1], mr, mi)
                    pr.append(nr)
                    pi.append(ni)
                p_v[k] = jnp.concatenate(
                    [jnp.concatenate(pr, axis=0), jnp.concatenate(pi, axis=0)], axis=1).astype(BF16)
                ur = ur_v[chan(k), :]
                ur = jnp.concatenate([jnp.where(even, ur, 0.0), jnp.where(even, 0.0, ur)], axis=0)
                sre_v[states(k), :] = _dot(ur, jnp.concatenate(pr + pr, axis=0).astype(BF16))
                sim_v[states(k), :] = _dot(ur, jnp.concatenate(pi + pi, axis=0).astype(BF16))

        def scan(k0, width, last):
            ltr, lti, wlr, wli, gr, gi = (cf_v[i, k0:k0 + width, :] for i in range(6))
            if last is not None:
                wlr, wli = jnp.where(never, last, wlr), jnp.where(never, last, wli)
            nwlr = -wlr
            for c in range(2 * n_blocks):
                idx = pl.ds(k0 * SPITCH + (c % 2) * n_blocks + c // 2, width, stride=SPITCH)
                gre_v[idx, :] = gr
                gim_v[idx, :] = gi
                if c < 2 * n_blocks - 1:
                    xr, xi = sre_v[idx, :], sim_v[idx, :]
                    sr, si = wlr * xr - wli * xi, nwlr * xi - wli * xr
                    if c == 0:
                        gr, gi = sr, si
                    else:
                        gr, gi = _cmul(gr, gi, ltr, lti)
                        gr, gi = gr + sr, gi + si
            return gr

        def read_out(fill):
            has_state = lax.broadcasted_iota(jnp.int32, (n_blocks, T), 0) > 0
            width, lag = (8 if g else 16), 2
            last = None
            for k0 in range(0, GC + lag * width, width):
                if k0 < GC:
                    last = scan(k0, width, last)
                for k in range(k0 - lag * width, k0 - (lag - 1) * width):
                    if k % 2 == 0:
                        fill(k + lag * width, GC + lag * width)
                    if k < 0:
                        continue
                    gg = jnp.concatenate([gre_v[states(k), :], gim_v[states(k), :]], axis=1)
                    p = p_v[k]
                    y = _dot(gg, jnp.concatenate([p, jnp.zeros_like(p)], axis=0), NT)
                    taps_v[8 * k:8 * k + 8, :] = y[0:8, :] + pltpu.roll(y[0:8, :], TC, 1)
                    y_v[chan(k), :] = (jnp.where(has_state, y[:n_blocks], 0.0)
                                       + pltpu.roll(y[n_blocks:], TC, 1))

        def in_chunk(fill):
            ti = lax.broadcasted_iota(jnp.int32, (TC, T), 0)
            tj = lax.broadcasted_iota(jnp.int32, (TC, T), 1)
            causal_even = (tj >= ti) & (tj < TC)
            causal_odd = tj >= ti + TC
            for k in range(GC):
                if k % 2 == 0:
                    fill(k, GC)
                kb = jnp.broadcast_to(taps_v[8 * k:8 * k + 1, :], (TC, T))
                tz = pltpu.roll(kb, 0, 1, stride=1, stride_axis=0)
                tz = jnp.concatenate([jnp.where(causal_even, tz, 0.0),
                                      jnp.where(causal_odd, tz, 0.0)], axis=0)
                y_v[chan(k), :] += _dot(uf_v[chan(k), :], tz.astype(BF16))

        def finish(fill):
            dsk = dsk_v[ch].astype(F32).reshape(1, GC)
            done = [(), ()]
            for c in range(n_blocks):
                fill(c, n_blocks, done.pop(0))
                rows = slice(c * T, (c + 1) * T)
                yc = y_v[pl.ds(c, GC, stride=PITCH), :].T.astype(BF16).astype(F32)
                yc = yc + (u_v[g, rows, :].astype(F32) * dsk).astype(BF16).astype(F32)
                outb_v[g, rows, :] = yc.astype(BF16)
                done.append((yc,))

        def first_weights(fill):
            for s in range(n_seg):
                xp_v[s * PRE:(s + 1) * PRE, :] = xt_v[s].astype(F32)

        with jax.named_scope(f"wait_g{g}"):
            for cp in group_copies(g):
                cp.wait()
        if g == 0:
            w_copy(0).start()
            xt_copy.start()
        elif g + 1 < n_groups:
            for cp in group_copies(g + 1):
                cp.start()
        if 1 <= g <= n_groups // 2:
            for j in (2 * g - 2, 2 * g - 1):
                wo_copy(j).start()
                x_copy(j).start()
        stage(prepare, quota[0], n_dc if g == 1 else 0, sizes[0])
        stage(read_in, quota[1], pieces[1] if g else 0, sizes[1])
        stage(read_out, quota[2], pieces[2] if g else 0, sizes[2])
        if g == 0:
            with jax.named_scope('wait_xt'):
                xt_copy.wait()
            for cp in group_copies(1):
                cp.start()
            w_copy(1).start()
            stage(first_weights, 0, n_dc)
            for c in range(2, n_slots):
                w_copy(c).start()
        stage(in_chunk, quota[3], pieces[3] if g else 0)
        stage(finish, quota[4] if g + 1 < n_groups else n_pre * n_rb, pieces[4] if g else 0)

    for cp in small + group_copies(0):
        cp.start()
    with jax.named_scope("wait_small"):
        for cp in small:
            cp.wait()
    for g in range(n_groups):
        ssm_group(g)
    assert progress == {"piece": n_tiles * n_dc, "unit": n_pre * n_rb}, progress
    with jax.named_scope("wait_x"):
        for g in range(n_groups):
            x_copy(g).wait()
            wo_copy(g).wait()
    for g in range(n_groups):
        outb_copy(g).start()

    scale = Dh ** -0.5
    qi = lax.broadcasted_iota(jnp.int32, (L, 128), 0)
    ki = lax.broadcasted_iota(jnp.int32, (L, 128), 1)
    keep = ((qi < n_mem) | (qi >= ki)) & (ki < L)
    masked = jnp.where(ki < L, -1000000000.0 / scale, -jnp.inf)
    zpad = jnp.zeros((128 - L, Dh), F32)
    n_og = n_heads // HG
    heads = [h % AG * (n_heads // AG) + h // AG for h in range(n_heads)]

    def step(s, cur, nxt):
        r = pl.ds(pl.multiple_of(s * seg, seg), seg)
        qs, ks, vs, es, os_, acc = {}, {}, {}, {}, {}, {}

        def proj(i, h):
            m = i * n_heads + h
            w = pltpu.bitcast(w_v[m], BF16)
            if m >= n_pre:
                return _dot(h_v[cur], w)
            known = pre_v[m, pl.ds(pl.multiple_of(s * PRE, PRE), PRE), :]
            return jnp.concatenate([_dot(h_v[cur, :L - PRE, :], w), known], axis=0)

        def scores(h):
            sc = jnp.where(keep, _dot(qs.pop(h), ks.pop(h), NT), masked)
            e = jnp.exp2((sc - jnp.max(sc, axis=1, keepdims=True)) * (scale * LOG2E))
            total = jnp.sum(e, axis=1, keepdims=True)
            inv = pl.reciprocal(total, approx=True)
            es[h] = (e, inv * (2.0 - total * inv))

        def mix(h):
            e, inv = es.pop(h)
            os_[h] = _dot(e, vs.pop(h)) * inv

        def oproj(j, g):
            hs = heads[g * HG:(g + 1) * HG]
            w = jnp.concatenate([wo_v[j, h * Dh // 2:(h + 1) * Dh // 2, :] for h in hs], axis=0)
            return _dot(jnp.concatenate([os_[h] for h in hs], axis=1), pltpu.bitcast(w, BF16))

        early = [divmod(t, n_og - 1) for t in range(Dm // 128 * (n_og - 1))]

        def oproj_early(count):
            for _ in range(count):
                j, g = early.pop(0)
                acc[j] = acc[j] + oproj(j, g) if g else oproj(j, g)

        for h0 in range(0, n_heads, AG):
            before = heads[max(h0 - AG, 0):h0]
            for i, h in enumerate(heads[h0:h0 + AG]):
                qs[h] = proj(0, h)
                if i == 1:
                    for hh in before:
                        scores(hh)
                ks[h] = jnp.concatenate([proj(1, h), zpad], axis=0).astype(BF16)
                if i == AG - 1:
                    for hh in before:
                        mix(hh)
                vs[h] = jnp.concatenate([proj(2, h), zpad], axis=0).astype(BF16)

        h_v[nxt, n_mem:, :] = x_v[jnp.minimum(s + 1, n_seg - 1)].astype(F32)

        oproj_early(3)
        for hh in heads[n_heads - AG:]:
            scores(hh)
        oproj_early(7)
        for hh in heads[n_heads - AG:]:
            mix(hh)
        oproj_early(3)
        for j in range(Dm // 128):
            oproj_early(sum(jj <= j for jj, _ in early))
            res = acc.pop(j) + oproj(j, n_og - 1)
            h_v[nxt, :n_mem, 128 * j:128 * (j + 1)] = res[:n_mem]
            outa_v[r, 128 * j:128 * (j + 1)] = res[n_mem:].astype(BF16)

    def steps(it, carry):
        for c in range(unroll):
            step(it * unroll + c, c % 2, (c + 1) % 2)
        outa_copy(it).start()
        return carry

    h_v[0, :n_mem, :] = mem0_v[...].astype(F32)
    h_v[0, n_mem:, :] = x_v[0].astype(F32)
    with jax.named_scope("steps"):
        lax.fori_loop(0, n_seg // unroll, steps, 0)

    for g in range(n_groups):
        outb_copy(g).wait()

    def drain(it, carry):
        outa_copy(it).wait()
        return carry

    lax.fori_loop(0, n_seg // unroll, drain, 0)


@functools.partial(jax.jit, static_argnames=("A_seg_len", "unroll", "quota", "pieces", "RB", "sizes", "pb", "plag", "ser", "n_pre", "do_b"))
def pallas_concat_heads__memory_aug_recurrent_mem_tr__ssm_conv_s4__prompt_kernel(
    A_x, A_mem0, A_Wq, A_Wk, A_Wv, A_Wo, A_seg_len,
    B_u, B_A_re, B_A_im, B_B_re, B_B_im, B_C_re, B_C_im, B_log_dt, B_Dskip,
    unroll=2, quota="24,16,16,24,10", pieces="0,0,0,12,0", RB=64, sizes="1,1,2", pb=8, plag=3, ser=1, n_pre=80, do_b=True,
):
    Bsz, S, Dm = A_x.shape
    H, Dh = A_Wq.shape[1], A_Wq.shape[2]
    M = A_mem0.shape[1]
    D, N = B_A_re.shape
    seg = int(A_seg_len)
    assert Bsz == 1 and Dh == 128 and N == 128 and D == Dm and B_u.shape == A_x.shape
    n_seg = S // seg
    n_groups = D // GC
    n_slots = 3
    quota, pieces, sizes = (tuple(int(c) for c in v.split(",")) for v in (quota, pieces, sizes))

    def head_tiles(w):
        return w.reshape(Dm, H // HT, HT, Dh).transpose(0, 2, 1, 3).reshape(Dm * HT, H // HT * Dh)

    def pitched(pitch):
        return pltpu.VMEM(((GC + 8) * pitch, N), F32)

    any_spec = pl.BlockSpec(memory_space=pl.ANY)
    out = pl.pallas_call(
        functools.partial(_kernel, unroll=unroll, quota=quota, pieces=pieces, RB=RB, sizes=sizes, pb=pb, plag=plag, ser=ser, do_b=do_b),
        out_shape=jax.ShapeDtypeStruct((S, Dm + D), BF16),
        in_specs=[pl.BlockSpec(memory_space=pltpu.SMEM)] + [any_spec] * 15,
        out_specs=any_spec,
        scratch_shapes=[
            pltpu.VMEM((n_seg, seg, Dm), BF16),
            pltpu.VMEM((n_seg, PRE, Dm), BF16),
            pltpu.VMEM((n_seg * PRE, Dm), F32),
            pltpu.VMEM((n_groups, S, GC), BF16),
            pltpu.VMEM((6, D, N), BF16),
            pltpu.VMEM((n_slots, Dm * HT + 32, Dh), BF16),
            pltpu.VMEM((3 * H, Dm // 2, Dh), U32),
            pltpu.VMEM((Dm // 128, H * Dh // 2, 128), U32),
            pltpu.VMEM((n_pre, n_seg * PRE, Dh), F32),
            pltpu.VMEM((S, Dm), BF16),
            pltpu.VMEM((n_groups, S, GC), BF16),
            pltpu.VMEM((2, M + seg, Dm), F32),
            pitched(BPITCH), pitched(BPITCH),
            pltpu.VMEM((8, GC, N), F32),
            pltpu.VMEM((GC, TC, 2 * N), BF16),
            pitched(PITCH), pitched(PITCH),
            pitched(SPITCH), pitched(SPITCH),
            pitched(SPITCH), pitched(SPITCH),
            pitched(PITCH),
            pltpu.VMEM((GC * 8, T), F32),
            pltpu.VMEM((M, Dm), BF16),
            pltpu.VMEM((D,), BF16),
            pltpu.VMEM((D,), BF16),
            pltpu.SemaphoreType.DMA((3,)),
            pltpu.SemaphoreType.DMA(()),
            pltpu.SemaphoreType.DMA(()),
            pltpu.SemaphoreType.DMA((n_groups,)),
            pltpu.SemaphoreType.DMA((n_groups,)),
            pltpu.SemaphoreType.DMA((n_slots,)),
            pltpu.SemaphoreType.DMA(()),
            pltpu.SemaphoreType.DMA(()),
            pltpu.SemaphoreType.DMA(()),
        ],
        compiler_params=pltpu.CompilerParams(vmem_limit_bytes=120 * 1024 * 1024),
    )(np.zeros((1,), np.int32), A_x.reshape(n_seg, seg, Dm), A_mem0.reshape(M, Dm),
      head_tiles(A_Wq), head_tiles(A_Wk), head_tiles(A_Wv), A_Wo.reshape(H * Dh, Dm),
      B_u.reshape(S, D), B_A_re, B_A_im, B_B_re, B_B_im, B_C_re, B_C_im, B_log_dt, B_Dskip)
    return out.reshape(Bsz, S, Dm + D)
```

```python
import functools
import math

import jax
import jax.numpy as jnp
import numpy as np
from jax import lax
import jax.experimental.pallas as pl
import jax.experimental.pallas.tpu as pltpu

F32 = jnp.float32
BF16 = jnp.bfloat16
U32 = jnp.uint32

NN = (((1,), (0,)), ((), ()))
NT = (((1,), (1,)), ((), ()))
LOG2E = math.log2(math.e)

T = 128
TC = T // 2
GC = 128
PB = 8
PITCH = 17
SPITCH = 33
BPITCH = 9

HT = 8
DC = 128
N_SLOTS = 3
PRE = 8
RB = 64
HG = 8
AG = 4
UNROLL = 2


def _dot(a, b, dims=NN):
    return lax.dot_general(a, b, dims, preferred_element_type=F32)


def _cmul(ar, ai, br, bi):
    return ar * br - ai * bi, ar * bi + ai * br


def _reverse_chunks(v):
    row = lax.broadcasted_iota(jnp.int32, (8, v.shape[1]), 0)

    def reverse8(p):
        p = pltpu.roll(p, 4, 0)
        p = jnp.where((row & 2) == 0, pltpu.roll(p, 6, 0), pltpu.roll(p, 2, 0))
        return jnp.where((row & 1) == 0, pltpu.roll(p, 7, 0), pltpu.roll(p, 1, 0))

    order = [i ^ (TC // 8 - 1) for i in range(v.shape[0] // 8)]
    return jnp.concatenate([reverse8(v[8 * i:8 * i + 8]) for i in order], axis=0)


def _start(copies):
    for cp in copies:
        cp.start()


def _wait(copies):
    for cp in copies:
        cp.wait()


def _kernel(zero_ref, x_hbm, mem0_hbm, wq_hbm, wk_hbm, wv_hbm, wo_hbm,
            u_hbm, are_hbm, aim_hbm, bre_hbm, bim_hbm, cre_hbm, cim_hbm, ldt_hbm, dsk_hbm,
            out_hbm,
            x_v, xt_v, xp_v, u_v, par_v, stage_v, w_v, wo_v, pre_v, outa_v, outb_v, h_v,
            bre_v, bim_v, cf_v, p_v, uf_v, ur_v, sre_v, sim_v, gre_v, gim_v, y_v, taps_v,
            mem0_v, ldt_v, dsk_v,
            sem_s, sem_x, sem_xt, sem_g, sem_w, sem_wo, sem_oa, sem_ob):
    n_seg, seg, Dm = x_v.shape
    n_mem = mem0_v.shape[0]
    Dh = w_v.shape[2]
    n_heads = w_v.shape[0] // 3
    n_groups = Dm // GC
    n_blocks = n_seg * seg // T
    L = n_mem + seg
    n_tiles = 3 * n_heads // HT
    n_dc = Dm // DC
    n_rb = n_seg * PRE // RB
    n_pre = pre_v.shape[0]

    always = zero_ref[0] == 0
    never = zero_ref[0] != 0

    def w_copies(c):
        i, tile = divmod(c, n_heads // HT)
        rows = [pl.ds(r, Dm * HT // 4) for r in range(0, Dm * HT, Dm * HT // 4)]
        return [pltpu.make_async_copy((wq_hbm, wk_hbm, wv_hbm)[i].at[r, pl.ds(tile * Dh, Dh)],
                                      stage_v.at[c % N_SLOTS, r, :], sem_w.at[c % N_SLOTS]) for r in rows]

    def wo_copy(j):
        return pltpu.make_async_copy(wo_hbm.at[:, pl.ds(128 * j, 128)], wo_v.at[j].bitcast(BF16), sem_wo)

    def x_copy(j):
        r = pl.ds(j * (n_seg // n_groups), n_seg // n_groups)
        return pltpu.make_async_copy(x_hbm.at[r], x_v.at[r], sem_x)

    def group_copies(g):
        ch = pl.ds(g * GC, GC)
        return [pltpu.make_async_copy(p.at[ch, :], par_v.at[i, ch, :], sem_g.at[g])
                for i, p in enumerate((are_hbm, aim_hbm, bre_hbm, bim_hbm, cre_hbm, cim_hbm))] + [
                    pltpu.make_async_copy(u_hbm.at[:, ch], u_v.at[g], sem_g.at[g])]

    def outb_copy(g):
        return pltpu.make_async_copy(outb_v.at[g], out_hbm.at[:, pl.ds(Dm + g * GC, GC)], sem_ob)

    def outa_copy(it):
        r = pl.ds(pl.multiple_of(it * UNROLL * seg, seg), UNROLL * seg)
        return pltpu.make_async_copy(outa_v.at[r, :], out_hbm.at[r, pl.ds(0, Dm)], sem_oa)

    xt_copy = pltpu.make_async_copy(x_hbm.at[:, pl.ds(seg - PRE, PRE), :], xt_v, sem_xt)
    small = [pltpu.make_async_copy(src, dst, sem_s.at[i]) for i, (src, dst) in
             enumerate(((ldt_hbm, ldt_v), (dsk_hbm, dsk_v), (mem0_hbm, mem0_v)))]

    def relayout(piece):
        c, pc = divmod(piece, n_dc)
        src = stage_v.at[c % N_SLOTS].bitcast(U32)
        rows = slice(pc * DC // 2, (pc + 1) * DC // 2)
        done = []
        for pp in range(HT // 2):
            ev = src[pl.ds(pc * DC * HT // 2 + pp, DC // 2, stride=HT), :]
            od = src[pl.ds(pc * DC * HT // 2 + pp + HT // 2, DC // 2, stride=HT), :]
            done += [(ev & 0xFFFF) | (od << 16), (ev >> 16) | (od & jnp.uint32(0xFFFF0000))]
            w_v[c * HT + 2 * pp, rows, :] = done[-2]
            w_v[c * HT + 2 * pp + 1, rows, :] = done[-1]
        return [lax.bitcast_convert_type(v, F32) for v in done]

    def ahead(unit, size, after):
        m, rb = divmod(unit, n_rb)
        rows = slice(rb * RB, (rb + size) * RB)
        lhs = xp_v[rows, :]
        if after is not None:
            corner = jnp.where(never, after, lhs[:8, :128])
            lhs = jnp.concatenate([jnp.concatenate([corner, lhs[:8, 128:]], axis=1), lhs[8:]], axis=0)
        res = _dot(lhs, pltpu.bitcast(w_v[m], BF16))
        pre_v[m, rows, :] = res
        return res[-8:]

    progress = {"piece": 0, "unit": 0}

    def filler(n_units, size, n_pieces):
        p0 = progress["piece"]
        p1 = min(p0 + n_pieces, n_tiles * n_dc)
        u0 = progress["unit"]
        u1 = min(u0 + n_units, p0 // n_dc * HT * n_rb, n_pre * n_rb)
        progress.update(piece=p1, unit=u1)
        assert u0 % size == 0 and u1 % size == 0
        todo_p, todo_u = list(range(p0, p1)), list(range(u0, u1, size))
        pending, issued = [], []

        def fill(done, total, after=()):
            pending.extend(after)
            while todo_u and (todo_u[0] - u0) * total <= done * (u1 - u0):
                rows = [v[r:r + 8] for v in pending for r in range(0, v.shape[0], 8)]
                issued.append(ahead(todo_u.pop(0), size, functools.reduce(jnp.add, rows) if rows else None))
                pending.clear()
            while todo_p and (todo_p[0] - p0) * total <= done * (p1 - p0 + 1):
                pending.extend(relayout(todo_p.pop(0)))
            return issued

        return fill

    def stage(*parts):
        p0 = progress["piece"]
        fills = [filler(*part[1:]) for part in parts]
        p1 = progress["piece"]
        for c in range(-(-p0 // n_dc), -(-p1 // n_dc)):
            _wait(w_copies(c))

        @pl.when(always)
        def _():
            for part, fill in zip(parts, fills):
                part[0](fill)
                fill(1, 1)

        for c in range(p0 // n_dc, p1 // n_dc):
            if c + N_SLOTS < n_tiles:
                _start(w_copies(c + N_SLOTS))

    def chan(k):
        return slice(k * PITCH, k * PITCH + n_blocks)

    def states(k):
        return slice(k * SPITCH, k * SPITCH + 2 * n_blocks)

    def ssm_group(g):
        ch = slice(g * GC, (g + 1) * GC)

        def prepare(fill):
            dt = jnp.exp(ldt_v[ch].astype(F32).reshape(1, GC)).astype(BF16).astype(F32)
            dt = jnp.broadcast_to(dt, (GC, GC)).T
            done = [(), (), ()]
            for c in range(n_blocks):
                issued = fill(c, n_blocks, done.pop(0))
                ub = u_v[g, c * T:(c + 1) * T, :].astype(F32)
                plain, flipped = ub.T, _reverse_chunks(ub).astype(BF16).T.astype(F32)
                uf_v[pl.ds(c, GC, stride=PITCH), :] = plain
                ur_v[pl.ds(c, GC, stride=PITCH), :] = flipped
                done.append((plain[-8:], flipped[-8:]))
                for k0 in range(c * GC // n_blocks, (c + 1) * GC // n_blocks, PB):
                    a_re, a_im, b_re, b_im, c_re, c_im = (
                        par_v[i, g * GC + k0:g * GC + k0 + PB, :].astype(F32) for i in range(6))
                    step = dt[k0:k0 + PB]
                    if len(issued) > 1:
                        step = jnp.where(never, issued[-2], step)
                    w_re, w_im = _cmul(c_re, c_im, step * b_re, step * b_im)
                    mag = jnp.exp(step * a_re)
                    l1 = (mag * jnp.cos(step * a_im), mag * jnp.sin(step * a_im))
                    l2 = _cmul(*l1, *l1)
                    l3 = _cmul(*l2, *l1)
                    l4 = _cmul(*l2, *l2)
                    pw = [(jnp.ones_like(mag), jnp.zeros_like(mag)), l1, l2, l3, l4,
                          _cmul(*l4, *l1), _cmul(*l4, *l2), _cmul(*l4, *l3)]
                    for r in range(8):
                        bre_v[pl.ds(k0 * BPITCH + r, PB, stride=BPITCH), :] = pw[r][0]
                        bim_v[pl.ds(k0 * BPITCH + r, PB, stride=BPITCH), :] = pw[r][1]
                    l8 = _cmul(*l4, *l4)
                    lt = l8
                    for _ in range(3):
                        lt = _cmul(*lt, *lt)
                    wl = _cmul(w_re, w_im, *l1)
                    for i, val in enumerate((lt[0], -lt[1], wl[0], wl[1], w_re, -w_im, *l8)):
                        cf_v[i, k0:k0 + PB, :] = val
                    done[-1] += (*pw[5], *pw[6], *pw[7], *lt, *wl)

        def read_in(fill):
            even = lax.broadcasted_iota(jnp.int32, (n_blocks, T), 1) < TC
            for k in range(GC):
                if k % 2 == 0:
                    fill(k, GC)
                pr = [bre_v[k * BPITCH:k * BPITCH + 8, :]]
                pi = [bim_v[k * BPITCH:k * BPITCH + 8, :]]
                mr = jnp.broadcast_to(cf_v[6, k:k + 1, :], (8, 128))
                mi = jnp.broadcast_to(cf_v[7, k:k + 1, :], (8, 128))
                for _ in range(TC // 8 - 1):
                    nr, ni = _cmul(pr[-1], pi[-1], mr, mi)
                    pr.append(nr)
                    pi.append(ni)
                p_v[k] = jnp.concatenate(
                    [jnp.concatenate(pr, axis=0), jnp.concatenate(pi, axis=0)], axis=1).astype(BF16)
                ur = ur_v[chan(k), :]
                ur = jnp.concatenate([jnp.where(even, ur, 0.0), jnp.where(even, 0.0, ur)], axis=0)
                sre_v[states(k), :] = _dot(ur, jnp.concatenate(pr + pr, axis=0).astype(BF16))
                sim_v[states(k), :] = _dot(ur, jnp.concatenate(pi + pi, axis=0).astype(BF16))

        def scan(k0, width, last):
            ltr, lti, wlr, wli, gr, gi = (cf_v[i, k0:k0 + width, :] for i in range(6))
            if last is not None:
                wlr, wli = jnp.where(never, last, wlr), jnp.where(never, last, wli)
            nwlr = -wlr
            for c in range(2 * n_blocks):
                idx = pl.ds(k0 * SPITCH + (c % 2) * n_blocks + c // 2, width, stride=SPITCH)
                gre_v[idx, :] = gr
                gim_v[idx, :] = gi
                if c < 2 * n_blocks - 1:
                    xr, xi = sre_v[idx, :], sim_v[idx, :]
                    sr, si = wlr * xr - wli * xi, nwlr * xi - wli * xr
                    if c == 0:
                        gr, gi = sr, si
                    else:
                        gr, gi = _cmul(gr, gi, ltr, lti)
                        gr, gi = gr + sr, gi + si
            return gr

        def read_out(fill):
            has_state = lax.broadcasted_iota(jnp.int32, (n_blocks, T), 0) > 0
            width = 8 if g else 16
            lag = 2 * width
            last = None
            for k0 in range(0, GC + lag, width):
                if k0 < GC:
                    last = scan(k0, width, last)
                for k in range(k0 - lag, k0 - lag + width):
                    if k % 2 == 0:
                        fill(k + lag, GC + lag + 8)
                    if k < 0:
                        continue
                    gg = jnp.concatenate([gre_v[states(k), :], gim_v[states(k), :]], axis=1)
                    p = p_v[k]
                    y = _dot(gg, jnp.concatenate([p, jnp.zeros_like(p)], axis=0), NT)
                    taps_v[8 * k:8 * k + 8, :] = y[0:8, :] + pltpu.roll(y[0:8, :], TC, 1)
                    y_v[chan(k), :] = (jnp.where(has_state, y[:n_blocks], 0.0)
                                       + pltpu.roll(y[n_blocks:], TC, 1))

        def in_chunk(fill):
            ti = lax.broadcasted_iota(jnp.int32, (TC, T), 0)
            tj = lax.broadcasted_iota(jnp.int32, (TC, T), 1)
            causal_even = (tj >= ti) & (tj < TC)
            causal_odd = tj >= ti + TC
            for k in range(GC):
                if k % 2 == 0:
                    fill(k, GC)
                kb = jnp.broadcast_to(taps_v[8 * k:8 * k + 1, :], (TC, T))
                tz = pltpu.roll(kb, 0, 1, stride=1, stride_axis=0)
                tz = jnp.concatenate([jnp.where(causal_even, tz, 0.0),
                                      jnp.where(causal_odd, tz, 0.0)], axis=0)
                y_v[chan(k), :] += _dot(uf_v[chan(k), :], tz.astype(BF16))

        def finish(fill):
            dsk = dsk_v[ch].astype(F32).reshape(1, GC)
            done = [(), ()]
            for c in range(n_blocks):
                fill(c, n_blocks, done.pop(0))
                rows = slice(c * T, (c + 1) * T)
                yc = y_v[pl.ds(c, GC, stride=PITCH), :].T.astype(BF16).astype(F32)
                yc = yc + (u_v[g, rows, :].astype(F32) * dsk).astype(BF16).astype(F32)
                outb_v[g, rows, :] = yc.astype(BF16)
                done.append((yc,))

        return ((prepare, 20, 1, n_dc if g == 1 else 0),
                (read_in, 16, 1, 0),
                (read_out, 16, 2, 0),
                (in_chunk, 26, 2, n_tiles * n_dc // n_groups if g else 0),
                (finish, 8 if g + 1 < n_groups else n_pre * n_rb, 2, 0))

    def widen(fill):
        for s in range(n_seg):
            xp_v[s * PRE:(s + 1) * PRE, :] = xt_v[s].astype(F32)

    _start(small + group_copies(0))
    _wait(small)
    _start(w_copies(0) + [xt_copy])
    _wait(group_copies(0))
    leftover = ()
    for g in range(n_groups):
        prepare, read_in, read_out, in_chunk, finish = ssm_group(g)
        if 0 < g < n_groups - 1:
            _start(group_copies(g + 1))
        if 0 < g <= n_groups // 2:
            _start([make(j) for j in (2 * g - 2, 2 * g - 1) for make in (wo_copy, x_copy)])
        stage(*leftover, prepare)
        stage(read_in)
        stage(read_out)
        if g == 0:
            xt_copy.wait()
            _start(group_copies(1) + w_copies(1))
            stage((widen, 0, 1, n_dc))
            for c in range(2, N_SLOTS):
                _start(w_copies(c))
        stage(in_chunk)
        if g + 1 < n_groups:
            _wait(group_copies(g + 1))
        if 0 < g < n_groups - 1:
            leftover = (finish,)
        else:
            stage(finish)
    assert progress == {"piece": n_tiles * n_dc, "unit": n_pre * n_rb}
    _wait([make(j) for j in range(n_groups) for make in (x_copy, wo_copy)])
    _start([outb_copy(g) for g in range(n_groups)])

    scale = Dh ** -0.5
    qi = lax.broadcasted_iota(jnp.int32, (L, 128), 0)
    ki = lax.broadcasted_iota(jnp.int32, (L, 128), 1)
    keep = ((qi < n_mem) | (qi >= ki)) & (ki < L)
    masked = jnp.where(ki < L, -1000000000.0 / scale, -jnp.inf)
    zpad = jnp.zeros((128 - L, Dh), F32)
    n_og = n_heads // HG
    heads = [h % AG * (n_heads // AG) + h // AG for h in range(n_heads)]

    def step(s, cur, nxt):
        r = pl.ds(pl.multiple_of(s * seg, seg), seg)
        qs, ks, vs, es, os_, acc = {}, {}, {}, {}, {}, {}

        def proj(i, h):
            m = i * n_heads + h
            w = pltpu.bitcast(w_v[m], BF16)
            if m >= n_pre:
                return _dot(h_v[cur], w)
            known = pre_v[m, pl.ds(pl.multiple_of(s * PRE, PRE), PRE), :]
            return jnp.concatenate([_dot(h_v[cur, :L - PRE, :], w), known], axis=0)

        def scores(h):
            sc = jnp.where(keep, _dot(qs.pop(h), ks.pop(h), NT), masked)
            e = jnp.exp2((sc - jnp.max(sc, axis=1, keepdims=True)) * (scale * LOG2E))
            total = jnp.sum(e, axis=1, keepdims=True)
            inv = pl.reciprocal(total, approx=True)
            es[h] = (e, inv * (2.0 - total * inv))

        def mix(h):
            e, inv = es.pop(h)
            os_[h] = _dot(e, vs.pop(h)) * inv

        def oproj(j, g):
            hs = heads[g * HG:(g + 1) * HG]
            w = jnp.concatenate([wo_v[j, h * Dh // 2:(h + 1) * Dh // 2, :] for h in hs], axis=0)
            return _dot(jnp.concatenate([os_[h] for h in hs], axis=1), pltpu.bitcast(w, BF16))

        early = [divmod(t, n_og - 1) for t in range(Dm // 128 * (n_og - 1))]

        def oproj_early(count):
            for _ in range(count):
                j, g = early.pop(0)
                acc[j] = acc[j] + oproj(j, g) if g else oproj(j, g)

        for h0 in range(0, n_heads, AG):
            before = heads[max(h0 - AG, 0):h0]
            for i, h in enumerate(heads[h0:h0 + AG]):
                qs[h] = proj(0, h)
                if i == AG - 2:
                    for hh in before:
                        scores(hh)
                ks[h] = jnp.concatenate([proj(1, h), zpad], axis=0).astype(BF16)
                if i == AG - 1:
                    for hh in before:
                        mix(hh)
                vs[h] = jnp.concatenate([proj(2, h), zpad], axis=0).astype(BF16)

        h_v[nxt, n_mem:, :] = x_v[jnp.minimum(s + 1, n_seg - 1)].astype(F32)

        oproj_early(3)
        for hh in heads[n_heads - AG:]:
            scores(hh)
        oproj_early(7)
        for hh in heads[n_heads - AG:]:
            mix(hh)
        oproj_early(3)
        for j in range(Dm // 128):
            oproj_early(sum(jj <= j for jj, _ in early))
            res = acc.pop(j) + oproj(j, n_og - 1)
            h_v[nxt, :n_mem, 128 * j:128 * (j + 1)] = res[:n_mem]
            outa_v[r, 128 * j:128 * (j + 1)] = res[n_mem:].astype(BF16)

    def steps(it, carry):
        for c in range(UNROLL):
            step(it * UNROLL + c, c, (c + 1) % UNROLL)
        outa_copy(it).start()
        return carry

    h_v[0, :n_mem, :] = mem0_v[...].astype(F32)
    h_v[0, n_mem:, :] = x_v[0].astype(F32)
    lax.fori_loop(0, n_seg // UNROLL, steps, 0)

    def drain(it, carry):
        outa_copy(it).wait()
        return carry

    _wait([outb_copy(g) for g in range(n_groups)])
    lax.fori_loop(0, n_seg // UNROLL, drain, 0)


@functools.partial(jax.jit, static_argnames=("A_seg_len",))
def pallas_concat_heads__memory_aug_recurrent_mem_tr__ssm_conv_s4__prompt_kernel(
    A_x: jax.Array,
    A_mem0: jax.Array,
    A_Wq: jax.Array,
    A_Wk: jax.Array,
    A_Wv: jax.Array,
    A_Wo: jax.Array,
    A_seg_len: int,
    B_u: jax.Array,
    B_A_re: jax.Array,
    B_A_im: jax.Array,
    B_B_re: jax.Array,
    B_B_im: jax.Array,
    B_C_re: jax.Array,
    B_C_im: jax.Array,
    B_log_dt: jax.Array,
    B_Dskip: jax.Array,
):
    Bsz, S, Dm = A_x.shape
    H, Dh = A_Wq.shape[1], A_Wq.shape[2]
    M = A_mem0.shape[1]
    D, N = B_A_re.shape
    seg = int(A_seg_len)
    n_seg = S // seg
    n_groups = D // GC
    assert Bsz == 1 and Dh == 128 and N == 128 and D == Dm and B_u.shape == A_x.shape
    assert n_seg % UNROLL == 0 and M + seg <= 128
    n_pre = 2 * H + H // 2

    def head_tiles(w):
        return w.reshape(Dm, H // HT, HT, Dh).transpose(0, 2, 1, 3).reshape(Dm * HT, H // HT * Dh)

    def pitched(pitch):
        return pltpu.VMEM(((GC + 8) * pitch, N), F32)

    any_spec = pl.BlockSpec(memory_space=pl.ANY)
    out = pl.pallas_call(
        _kernel,
        out_shape=jax.ShapeDtypeStruct((S, Dm + D), BF16),
        in_specs=[pl.BlockSpec(memory_space=pltpu.SMEM)] + [any_spec] * 15,
        out_specs=any_spec,
        scratch_shapes=[
            pltpu.VMEM((n_seg, seg, Dm), BF16),
            pltpu.VMEM((n_seg, PRE, Dm), BF16),
            pltpu.VMEM((n_seg * PRE, Dm), F32),
            pltpu.VMEM((n_groups, S, GC), BF16),
            pltpu.VMEM((6, D, N), BF16),
            pltpu.VMEM((N_SLOTS, Dm * HT + 32, Dh), BF16),
            pltpu.VMEM((3 * H, Dm // 2, Dh), U32),
            pltpu.VMEM((Dm // 128, H * Dh // 2, 128), U32),
            pltpu.VMEM((n_pre, n_seg * PRE, Dh), F32),
            pltpu.VMEM((S, Dm), BF16),
            pltpu.VMEM((n_groups, S, GC), BF16),
            pltpu.VMEM((UNROLL, M + seg, Dm), F32),
            pitched(BPITCH), pitched(BPITCH),
            pltpu.VMEM((8, GC, N), F32),
            pltpu.VMEM((GC, TC, 2 * N), BF16),
            pitched(PITCH), pitched(PITCH),
            pitched(SPITCH), pitched(SPITCH),
            pitched(SPITCH), pitched(SPITCH),
            pitched(PITCH),
            pltpu.VMEM((GC * 8, T), F32),
            pltpu.VMEM((M, Dm), BF16),
            pltpu.VMEM((D,), BF16),
            pltpu.VMEM((D,), BF16),
            pltpu.SemaphoreType.DMA((3,)),
            pltpu.SemaphoreType.DMA(()),
            pltpu.SemaphoreType.DMA(()),
            pltpu.SemaphoreType.DMA((n_groups,)),
            pltpu.SemaphoreType.DMA((N_SLOTS,)),
            pltpu.SemaphoreType.DMA(()),
            pltpu.SemaphoreType.DMA(()),
            pltpu.SemaphoreType.DMA(()),
        ],
        compiler_params=pltpu.CompilerParams(
            vmem_limit_bytes=120 * 1024 * 1024, disable_bounds_checks=True),
    )(np.zeros((1,), np.int32), A_x.reshape(n_seg, seg, Dm), A_mem0.reshape(M, Dm),
      head_tiles(A_Wq), head_tiles(A_Wk), head_tiles(A_Wv), A_Wo.reshape(H * Dh, Dm),
      B_u.reshape(S, D), B_A_re, B_A_im, B_B_re, B_B_im, B_C_re, B_C_im, B_log_dt, B_Dskip)
    return out.reshape(Bsz, S, Dm + D)
```

```python
import functools
import math

import jax
import jax.numpy as jnp
import numpy as np
from jax import lax
import jax.experimental.pallas as pl
import jax.experimental.pallas.tpu as pltpu

F32 = jnp.float32
BF16 = jnp.bfloat16
U32 = jnp.uint32

NN = (((1,), (0,)), ((), ()))
NT = (((1,), (1,)), ((), ()))
LOG2E = math.log2(math.e)

T = 128
TC = T // 2
GC = 128
PB = 8
PITCH = 17
SPITCH = 33
BPITCH = 9

HT = 8
DC = 128
N_SLOTS = 3
PRE = 8
RB = 64
HG = 8
AG = 4
UNROLL = 2


def _dot(a, b, dims=NN):
    return lax.dot_general(a, b, dims, preferred_element_type=F32)


def _cmul(ar, ai, br, bi):
    return ar * br - ai * bi, ar * bi + ai * br


def _reverse_chunks(v):
    row = lax.broadcasted_iota(jnp.int32, (8, v.shape[1]), 0)

    def reverse8(p):
        p = pltpu.roll(p, 4, 0)
        p = jnp.where((row & 2) == 0, pltpu.roll(p, 6, 0), pltpu.roll(p, 2, 0))
        return jnp.where((row & 1) == 0, pltpu.roll(p, 7, 0), pltpu.roll(p, 1, 0))

    order = [i ^ (TC // 8 - 1) for i in range(v.shape[0] // 8)]
    return jnp.concatenate([reverse8(v[8 * i:8 * i + 8]) for i in order], axis=0)


def _start(copies):
    for cp in copies:
        cp.start()


def _wait(copies):
    for cp in copies:
        cp.wait()


def _kernel(zero_ref, x_hbm, mem0_hbm, wq_hbm, wk_hbm, wv_hbm, wo_hbm,
            u_hbm, are_hbm, aim_hbm, bre_hbm, bim_hbm, cre_hbm, cim_hbm, ldt_hbm, dsk_hbm,
            out_hbm,
            x_v, xt_v, xp_v, u_v, par_v, stage_v, w_v, wo_v, pre_v, outa_v, outb_v, h_v,
            bre_v, bim_v, cf_v, p_v, uf_v, ur_v, sre_v, sim_v, gre_v, gim_v, y_v, taps_v,
            mem0_v, ldt_v, dsk_v,
            sem_s, sem_x, sem_xt, sem_g, sem_w, sem_wo, sem_oa, sem_ob):
    n_seg, seg, Dm = x_v.shape
    n_mem = mem0_v.shape[0]
    Dh = w_v.shape[2]
    n_heads = w_v.shape[0] // 3
    n_groups = Dm // GC
    n_blocks = n_seg * seg // T
    L = n_mem + seg
    n_tiles = 3 * n_heads // HT
    n_dc = Dm // DC
    n_rb = n_seg * PRE // RB
    n_pre = pre_v.shape[0]

    zero = zero_ref[0]
    never = zero != 0

    def w_copies(c):
        i, tile = divmod(c, n_heads // HT)
        rows = [pl.ds(r, Dm * HT // 4) for r in range(0, Dm * HT, Dm * HT // 4)]
        return [pltpu.make_async_copy((wq_hbm, wk_hbm, wv_hbm)[i].at[r, pl.ds(tile * Dh, Dh)],
                                      stage_v.at[c % N_SLOTS, r, :], sem_w.at[c % N_SLOTS]) for r in rows]

    def wo_copy(j):
        return pltpu.make_async_copy(wo_hbm.at[:, pl.ds(128 * j, 128)], wo_v.at[j].bitcast(BF16), sem_wo)

    def x_copy(j):
        r = pl.ds(j * (n_seg // n_groups), n_seg // n_groups)
        return pltpu.make_async_copy(x_hbm.at[r], x_v.at[r], sem_x)

    def group_copies(g):
        ch = pl.ds(g * GC, GC)
        return [pltpu.make_async_copy(p.at[ch, :], par_v.at[i, ch, :], sem_g.at[g])
                for i, p in enumerate((are_hbm, aim_hbm, bre_hbm, bim_hbm, cre_hbm, cim_hbm))] + [
                    pltpu.make_async_copy(u_hbm.at[:, ch], u_v.at[g], sem_g.at[g])]

    def outb_copy(g):
        return pltpu.make_async_copy(outb_v.at[g], out_hbm.at[:, pl.ds(Dm + g * GC, GC)], sem_ob)

    def outa_copy(it):
        r = pl.ds(pl.multiple_of(it * UNROLL * seg, seg), UNROLL * seg)
        return pltpu.make_async_copy(outa_v.at[r, :], out_hbm.at[r, pl.ds(0, Dm)], sem_oa)

    xt_copy = pltpu.make_async_copy(x_hbm.at[:, pl.ds(seg - PRE, PRE), :], xt_v, sem_xt)
    small = [pltpu.make_async_copy(src, dst, sem_s.at[i]) for i, (src, dst) in
             enumerate(((ldt_hbm, ldt_v), (dsk_hbm, dsk_v), (mem0_hbm, mem0_v)))]

    def relayout(piece):
        c, pc = divmod(piece, n_dc)
        src = stage_v.at[c % N_SLOTS].bitcast(U32)
        rows = slice(pc * DC // 2, (pc + 1) * DC // 2)
        done = []
        for pp in range(HT // 2):
            ev = src[pl.ds(pc * DC * HT // 2 + pp, DC // 2, stride=HT), :]
            od = src[pl.ds(pc * DC * HT // 2 + pp + HT // 2, DC // 2, stride=HT), :]
            done += [(ev & 0xFFFF) | (od << 16), (ev >> 16) | (od & jnp.uint32(0xFFFF0000))]
            w_v[c * HT + 2 * pp, rows, :] = done[-2]
            w_v[c * HT + 2 * pp + 1, rows, :] = done[-1]
        return [lax.bitcast_convert_type(v, F32) for v in done]

    def ahead(unit, size, after):
        m, rb = divmod(unit, n_rb)
        rows = slice(rb * RB, (rb + size) * RB)
        lhs = xp_v[rows, :]
        if after is not None:
            corner = jnp.where(never, after, lhs[:8, :128])
            lhs = jnp.concatenate([jnp.concatenate([corner, lhs[:8, 128:]], axis=1), lhs[8:]], axis=0)
        res = _dot(lhs, pltpu.bitcast(w_v[m], BF16))
        pre_v[m, rows, :] = res
        return res[-8:]

    progress = {"piece": 0, "unit": 0, "stage": 0}

    def filler(n_units, size, n_pieces):
        p0 = progress["piece"]
        p1 = min(p0 + n_pieces, n_tiles * n_dc)
        u0 = progress["unit"]
        u1 = min(u0 + n_units, p0 // n_dc * HT * n_rb, n_pre * n_rb)
        progress.update(piece=p1, unit=u1)
        assert u0 % size == 0 and u1 % size == 0
        todo_p, todo_u = list(range(p0, p1)), list(range(u0, u1, size))
        pending, issued = [], []

        def fill(done, total, after=()):
            pending.extend(after)
            while todo_u and (todo_u[0] - u0) * total <= done * (u1 - u0):
                rows = [v[r:r + 8] for v in pending for r in range(0, v.shape[0], 8)]
                issued.append(ahead(todo_u.pop(0), size, functools.reduce(jnp.add, rows) if rows else None))
                pending.clear()
            while todo_p and (todo_p[0] - p0) * total <= done * (p1 - p0 + 1):
                pending.extend(relayout(todo_p.pop(0)))
            return issued

        return fill

    def stage(*parts):
        p0 = progress["piece"]
        fills = [filler(*part[1:]) for part in parts]
        p1 = progress["piece"]
        for c in range(-(-p0 // n_dc), -(-p1 // n_dc)):
            _wait(w_copies(c))

        progress["stage"] += 1

        @pl.when(zero < progress["stage"])
        def _():
            for part, fill in zip(parts, fills):
                part[0](fill)
                fill(1, 1)

        for c in range(p0 // n_dc, p1 // n_dc):
            if c + N_SLOTS < n_tiles:
                _start(w_copies(c + N_SLOTS))

    def chan(k):
        return slice(k * PITCH, k * PITCH + n_blocks)

    def states(k):
        return slice(k * SPITCH, k * SPITCH + 2 * n_blocks)

    def ssm_group(g):
        ch = slice(g * GC, (g + 1) * GC)

        def prepare(fill):
            dt = jnp.exp(ldt_v[ch].astype(F32).reshape(1, GC)).astype(BF16).astype(F32)
            dt = jnp.broadcast_to(dt, (GC, GC)).T
            done = [(), (), ()]
            for c in range(n_blocks):
                issued = fill(c, n_blocks, done.pop(0))
                ub = u_v[g, c * T:(c + 1) * T, :].astype(F32)
                plain, flipped = ub.T, _reverse_chunks(ub).astype(BF16).T.astype(F32)
                uf_v[pl.ds(c, GC, stride=PITCH), :] = plain
                ur_v[pl.ds(c, GC, stride=PITCH), :] = flipped
                done.append((plain[-8:], flipped[-8:]))
                for k0 in range(c * GC // n_blocks, (c + 1) * GC // n_blocks, PB):
                    a_re, a_im, b_re, b_im, c_re, c_im = (
                        par_v[i, g * GC + k0:g * GC + k0 + PB, :].astype(F32) for i in range(6))
                    step = dt[k0:k0 + PB]
                    if len(issued) > 1:
                        step = jnp.where(never, issued[-2], step)
                    w_re, w_im = _cmul(c_re, c_im, step * b_re, step * b_im)
                    mag = jnp.exp(step * a_re)
                    l1 = (mag * jnp.cos(step * a_im), mag * jnp.sin(step * a_im))
                    l2 = _cmul(*l1, *l1)
                    l3 = _cmul(*l2, *l1)
                    l4 = _cmul(*l2, *l2)
                    pw = [(jnp.ones_like(mag), jnp.zeros_like(mag)), l1, l2, l3, l4,
                          _cmul(*l4, *l1), _cmul(*l4, *l2), _cmul(*l4, *l3)]
                    for r in range(8):
                        bre_v[pl.ds(k0 * BPITCH + r, PB, stride=BPITCH), :] = pw[r][0]
                        bim_v[pl.ds(k0 * BPITCH + r, PB, stride=BPITCH), :] = pw[r][1]
                    l8 = _cmul(*l4, *l4)
                    lt = l8
                    for _ in range(3):
                        lt = _cmul(*lt, *lt)
                    wl = _cmul(w_re, w_im, *l1)
                    for i, val in enumerate((lt[0], -lt[1], wl[0], wl[1], w_re, -w_im, *l8)):
                        cf_v[i, k0:k0 + PB, :] = val
                    done[-1] += (*pw[5], *pw[6], *pw[7], *lt, *wl)

        def read_in(fill):
            even = lax.broadcasted_iota(jnp.int32, (n_blocks, T), 1) < TC
            for k in range(GC):
                if k % 2 == 0:
                    fill(k, GC)
                pr = [bre_v[k * BPITCH:k * BPITCH + 8, :]]
                pi = [bim_v[k * BPITCH:k * BPITCH + 8, :]]
                mr = jnp.broadcast_to(cf_v[6, k:k + 1, :], (8, 128))
                mi = jnp.broadcast_to(cf_v[7, k:k + 1, :], (8, 128))
                for _ in range(TC // 8 - 1):
                    nr, ni = _cmul(pr[-1], pi[-1], mr, mi)
                    pr.append(nr)
                    pi.append(ni)
                p_v[k] = jnp.concatenate(
                    [jnp.concatenate(pr, axis=0), jnp.concatenate(pi, axis=0)], axis=1).astype(BF16)
                ur = ur_v[chan(k), :]
                ur = jnp.concatenate([jnp.where(even, ur, 0.0), jnp.where(even, 0.0, ur)], axis=0)
                sre_v[states(k), :] = _dot(ur, jnp.concatenate(pr + pr, axis=0).astype(BF16))
                sim_v[states(k), :] = _dot(ur, jnp.concatenate(pi + pi, axis=0).astype(BF16))

        def scan(k0, width, last):
            ltr, lti, wlr, wli, gr, gi = (cf_v[i, k0:k0 + width, :] for i in range(6))
            if last is not None:
                wlr, wli = jnp.where(never, last, wlr), jnp.where(never, last, wli)
            nwlr = -wlr
            for c in range(2 * n_blocks):
                idx = pl.ds(k0 * SPITCH + (c % 2) * n_blocks + c // 2, width, stride=SPITCH)
                gre_v[idx, :] = gr
                gim_v[idx, :] = gi
                if c < 2 * n_blocks - 1:
                    xr, xi = sre_v[idx, :], sim_v[idx, :]
                    sr, si = wlr * xr - wli * xi, nwlr * xi - wli * xr
                    if c == 0:
                        gr, gi = sr, si
                    else:
                        gr, gi = _cmul(gr, gi, ltr, lti)
                        gr, gi = gr + sr, gi + si
            return gr

        def read_out(fill):
            has_state = lax.broadcasted_iota(jnp.int32, (n_blocks, T), 0) > 0
            width = 8 if g else 16
            lag = 2 * width
            last = None
            for k0 in range(0, GC + lag, width):
                if k0 < GC:
                    last = scan(k0, width, last)
                for k in range(k0 - lag, k0 - lag + width):
                    if k % 2 == 0:
                        fill(k + lag, GC + lag + 8)
                    if k < 0:
                        continue
                    gg = jnp.concatenate([gre_v[states(k), :], gim_v[states(k), :]], axis=1)
                    p = p_v[k]
                    y = _dot(gg, jnp.concatenate([p, jnp.zeros_like(p)], axis=0), NT)
                    taps_v[8 * k:8 * k + 8, :] = y[0:8, :] + pltpu.roll(y[0:8, :], TC, 1)
                    y_v[chan(k), :] = (jnp.where(has_state, y[:n_blocks], 0.0)
                                       + pltpu.roll(y[n_blocks:], TC, 1))

        def in_chunk(fill):
            ti = lax.broadcasted_iota(jnp.int32, (TC, T), 0)
            tj = lax.broadcasted_iota(jnp.int32, (TC, T), 1)
            causal_even = (tj >= ti) & (tj < TC)
            causal_odd = tj >= ti + TC
            for k in range(GC):
                if k % 2 == 0:
                    fill(k, GC)
                kb = jnp.broadcast_to(taps_v[8 * k:8 * k + 1, :], (TC, T))
                tz = pltpu.roll(kb, 0, 1, stride=1, stride_axis=0)
                tz = jnp.concatenate([jnp.where(causal_even, tz, 0.0),
                                      jnp.where(causal_odd, tz, 0.0)], axis=0)
                y_v[chan(k), :] += _dot(uf_v[chan(k), :], tz.astype(BF16))

        def finish(fill):
            dsk = dsk_v[ch].astype(F32).reshape(1, GC)
            done = [(), ()]
            for c in range(n_blocks):
                fill(c, n_blocks, done.pop(0))
                rows = slice(c * T, (c + 1) * T)
                yc = y_v[pl.ds(c, GC, stride=PITCH), :].T.astype(BF16).astype(F32)
                yc = yc + (u_v[g, rows, :].astype(F32) * dsk).astype(BF16).astype(F32)
                outb_v[g, rows, :] = yc.astype(BF16)
                done.append((yc,))

        return ((prepare, 20, 1, n_dc if g == 1 else 0),
                (read_in, 16, 1, 0),
                (read_out, 16, 2, 0),
                (in_chunk, 26, 2, n_tiles * n_dc // n_groups if g else 0),
                (finish, 8 if g + 1 < n_groups else n_pre * n_rb, 2, 0))

    def widen(fill):
        for s in range(n_seg):
            xp_v[s * PRE:(s + 1) * PRE, :] = xt_v[s].astype(F32)

    _start(small + group_copies(0))
    _wait(small)
    _start(w_copies(0) + [xt_copy])
    _wait(group_copies(0))
    leftover = ()
    for g in range(n_groups):
        prepare, read_in, read_out, in_chunk, finish = ssm_group(g)
        if 0 < g < n_groups - 1:
            _start(group_copies(g + 1))
        if 0 < g <= n_groups // 2:
            _start([make(j) for j in (2 * g - 2, 2 * g - 1) for make in (wo_copy, x_copy)])
        stage(*leftover, prepare)
        stage(read_in)
        stage(read_out)
        if g == 0:
            xt_copy.wait()
            _start(group_copies(1) + w_copies(1))
            stage((widen, 0, 1, n_dc))
            for c in range(2, N_SLOTS):
                _start(w_copies(c))
        stage(in_chunk)
        if g + 1 < n_groups:
            _wait(group_copies(g + 1))
        if 0 < g < n_groups - 1:
            leftover = (finish,)
        else:
            stage(finish)
    assert (progress["piece"], progress["unit"]) == (n_tiles * n_dc, n_pre * n_rb)
    _wait([make(j) for j in range(n_groups) for make in (x_copy, wo_copy)])
    _start([outb_copy(g) for g in range(n_groups)])

    scale = Dh ** -0.5
    qi = lax.broadcasted_iota(jnp.int32, (L, 128), 0)
    ki = lax.broadcasted_iota(jnp.int32, (L, 128), 1)
    keep = ((qi < n_mem) | (qi >= ki)) & (ki < L)
    masked = jnp.where(ki < L, -1000000000.0 / scale, -jnp.inf)
    zpad = jnp.zeros((128 - L, Dh), F32)
    n_og = n_heads // HG
    heads = [h % AG * (n_heads // AG) + h // AG for h in range(n_heads)]

    def step(s, cur, nxt):
        r = pl.ds(pl.multiple_of(s * seg, seg), seg)
        qs, ks, vs, es, os_, acc = {}, {}, {}, {}, {}, {}

        def proj(i, h):
            m = i * n_heads + h
            w = pltpu.bitcast(w_v[m], BF16)
            if m >= n_pre:
                return _dot(h_v[cur], w)
            known = pre_v[m, pl.ds(pl.multiple_of(s * PRE, PRE), PRE), :]
            return jnp.concatenate([_dot(h_v[cur, :L - PRE, :], w), known], axis=0)

        def scores(h):
            sc = jnp.where(keep, _dot(qs.pop(h), ks.pop(h), NT), masked)
            e = jnp.exp2((sc - jnp.max(sc, axis=1, keepdims=True)) * (scale * LOG2E))
            total = jnp.sum(e, axis=1, keepdims=True)
            inv = pl.reciprocal(total, approx=True)
            es[h] = (e, inv * (2.0 - total * inv))

        def mix(h):
            e, inv = es.pop(h)
            os_[h] = _dot(e, vs.pop(h)) * inv

        def oproj(j, g):
            hs = heads[g * HG:(g + 1) * HG]
            w = jnp.concatenate([wo_v[j, h * Dh // 2:(h + 1) * Dh // 2, :] for h in hs], axis=0)
            return _dot(jnp.concatenate([os_[h] for h in hs], axis=1), pltpu.bitcast(w, BF16))

        early = [divmod(t, n_og - 1) for t in range(Dm // 128 * (n_og - 1))]

        def oproj_early(count):
            for _ in range(count):
                j, g = early.pop(0)
                acc[j] = acc[j] + oproj(j, g) if g else oproj(j, g)

        for h0 in range(0, n_heads, AG):
            before = heads[max(h0 - AG, 0):h0]
            for i, h in enumerate(heads[h0:h0 + AG]):
                qs[h] = proj(0, h)
                if i == AG - 2:
                    for hh in before:
                        scores(hh)
                ks[h] = jnp.concatenate([proj(1, h), zpad], axis=0).astype(BF16)
                if i == AG - 1:
                    for hh in before:
                        mix(hh)
                vs[h] = jnp.concatenate([proj(2, h), zpad], axis=0).astype(BF16)

        h_v[nxt, n_mem:, :] = x_v[jnp.minimum(s + 1, n_seg - 1)].astype(F32)

        oproj_early(3)
        for hh in heads[n_heads - AG:]:
            scores(hh)
        oproj_early(7)
        for hh in heads[n_heads - AG:]:
            mix(hh)
        oproj_early(3)
        for j in range(Dm // 128):
            oproj_early(sum(jj <= j for jj, _ in early))
            res = acc.pop(j) + oproj(j, n_og - 1)
            h_v[nxt, :n_mem, 128 * j:128 * (j + 1)] = res[:n_mem]
            outa_v[r, 128 * j:128 * (j + 1)] = res[n_mem:].astype(BF16)

    def steps(it, carry):
        for c in range(UNROLL):
            step(it * UNROLL + c, c, (c + 1) % UNROLL)
        outa_copy(it).start()
        return carry

    h_v[0, :n_mem, :] = mem0_v[...].astype(F32)
    h_v[0, n_mem:, :] = x_v[0].astype(F32)
    lax.fori_loop(0, n_seg // UNROLL, steps, 0)

    def drain(it, carry):
        outa_copy(it).wait()
        return carry

    _wait([outb_copy(g) for g in range(n_groups)])
    lax.fori_loop(0, n_seg // UNROLL, drain, 0)


@functools.partial(jax.jit, static_argnames=("A_seg_len",))
def pallas_concat_heads__memory_aug_recurrent_mem_tr__ssm_conv_s4__prompt_kernel(
    A_x: jax.Array,
    A_mem0: jax.Array,
    A_Wq: jax.Array,
    A_Wk: jax.Array,
    A_Wv: jax.Array,
    A_Wo: jax.Array,
    A_seg_len: int,
    B_u: jax.Array,
    B_A_re: jax.Array,
    B_A_im: jax.Array,
    B_B_re: jax.Array,
    B_B_im: jax.Array,
    B_C_re: jax.Array,
    B_C_im: jax.Array,
    B_log_dt: jax.Array,
    B_Dskip: jax.Array,
):
    Bsz, S, Dm = A_x.shape
    H, Dh = A_Wq.shape[1], A_Wq.shape[2]
    M = A_mem0.shape[1]
    D, N = B_A_re.shape
    seg = int(A_seg_len)
    n_seg = S // seg
    n_groups = D // GC
    assert Bsz == 1 and Dh == 128 and N == 128 and D == Dm and B_u.shape == A_x.shape
    assert n_seg % UNROLL == 0 and M + seg <= 128
    n_pre = 2 * H + H // 2

    def head_tiles(w):
        return w.reshape(Dm, H // HT, HT, Dh).transpose(0, 2, 1, 3).reshape(Dm * HT, H // HT * Dh)

    def pitched(pitch):
        return pltpu.VMEM(((GC + 8) * pitch, N), F32)

    any_spec = pl.BlockSpec(memory_space=pl.ANY)
    out = pl.pallas_call(
        _kernel,
        out_shape=jax.ShapeDtypeStruct((S, Dm + D), BF16),
        in_specs=[pl.BlockSpec(memory_space=pltpu.SMEM)] + [any_spec] * 15,
        out_specs=any_spec,
        scratch_shapes=[
            pltpu.VMEM((n_seg, seg, Dm), BF16),
            pltpu.VMEM((n_seg, PRE, Dm), BF16),
            pltpu.VMEM((n_seg * PRE, Dm), F32),
            pltpu.VMEM((n_groups, S, GC), BF16),
            pltpu.VMEM((6, D, N), BF16),
            pltpu.VMEM((N_SLOTS, Dm * HT + 32, Dh), BF16),
            pltpu.VMEM((3 * H, Dm // 2, Dh), U32),
            pltpu.VMEM((Dm // 128, H * Dh // 2, 128), U32),
            pltpu.VMEM((n_pre, n_seg * PRE, Dh), F32),
            pltpu.VMEM((S, Dm), BF16),
            pltpu.VMEM((n_groups, S, GC), BF16),
            pltpu.VMEM((UNROLL, M + seg, Dm), F32),
            pitched(BPITCH), pitched(BPITCH),
            pltpu.VMEM((8, GC, N), F32),
            pltpu.VMEM((GC, TC, 2 * N), BF16),
            pitched(PITCH), pitched(PITCH),
            pitched(SPITCH), pitched(SPITCH),
            pitched(SPITCH), pitched(SPITCH),
            pitched(PITCH),
            pltpu.VMEM((GC * 8, T), F32),
            pltpu.VMEM((M, Dm), BF16),
            pltpu.VMEM((D,), BF16),
            pltpu.VMEM((D,), BF16),
            pltpu.SemaphoreType.DMA((3,)),
            pltpu.SemaphoreType.DMA(()),
            pltpu.SemaphoreType.DMA(()),
            pltpu.SemaphoreType.DMA((n_groups,)),
            pltpu.SemaphoreType.DMA((N_SLOTS,)),
            pltpu.SemaphoreType.DMA(()),
            pltpu.SemaphoreType.DMA(()),
            pltpu.SemaphoreType.DMA(()),
        ],
        compiler_params=pltpu.CompilerParams(
            vmem_limit_bytes=120 * 1024 * 1024, disable_bounds_checks=True),
    )(np.zeros((1,), np.int32), A_x.reshape(n_seg, seg, Dm), A_mem0.reshape(M, Dm),
      head_tiles(A_Wq), head_tiles(A_Wk), head_tiles(A_Wv), A_Wo.reshape(H * Dh, Dm),
      B_u.reshape(S, D), B_A_re, B_A_im, B_B_re, B_B_im, B_C_re, B_C_im, B_log_dt, B_Dskip)
    return out.reshape(Bsz, S, Dm + D)
```

```python
import functools
import math

import jax
import jax.numpy as jnp
import numpy as np
from jax import lax
import jax.experimental.pallas as pl
import jax.experimental.pallas.tpu as pltpu

F32 = jnp.float32
BF16 = jnp.bfloat16
U32 = jnp.uint32

NN = (((1,), (0,)), ((), ()))
NT = (((1,), (1,)), ((), ()))
LOG2E = math.log2(math.e)

T = 128
TC = T // 2
GC = 128
GROUPS = (1, 2, 2, 2, 1)
PB = 8
PITCH = 17
SPITCH = 33
BPITCH = 9

HT = 8
DC = 128
N_SLOTS = 3
PRE = 8
RB = 64
HG = 8
AG = 4
UNROLL = 2


def _dot(a, b, dims=NN):
    return lax.dot_general(a, b, dims, preferred_element_type=F32)


def _cmul(ar, ai, br, bi):
    return ar * br - ai * bi, ar * bi + ai * br


def _reverse_chunks(v):
    row = lax.broadcasted_iota(jnp.int32, (8, v.shape[1]), 0)

    def reverse8(p):
        p = pltpu.roll(p, 4, 0)
        p = jnp.where((row & 2) == 0, pltpu.roll(p, 6, 0), pltpu.roll(p, 2, 0))
        return jnp.where((row & 1) == 0, pltpu.roll(p, 7, 0), pltpu.roll(p, 1, 0))

    order = [i ^ (TC // 8 - 1) for i in range(v.shape[0] // 8)]
    return jnp.concatenate([reverse8(v[8 * i:8 * i + 8]) for i in order], axis=0)


def _start(copies):
    for cp in copies:
        cp.start()


def _wait(copies):
    for cp in copies:
        cp.wait()


def _kernel(zero_ref, x_hbm, mem0_hbm, wq_hbm, wk_hbm, wv_hbm, wo_hbm,
            u_hbm, are_hbm, aim_hbm, bre_hbm, bim_hbm, cre_hbm, cim_hbm, ldt_hbm, dsk_hbm,
            out_hbm,
            x_v, xt_v, xp_v, u_v, par_v, stage_v, w_v, wo_v, pre_v, outa_v, outb_v, h_v,
            bre_v, bim_v, cf_v, p_v, uf_v, ur_v, sre_v, sim_v, gre_v, gim_v, y_v, taps_v,
            mem0_v, ldt_v, dsk_v,
            sem_s, sem_x, sem_xt, sem_g, sem_w, sem_wo, sem_oa, sem_ob):
    n_seg, seg, Dm = x_v.shape
    n_mem = mem0_v.shape[0]
    Dh = w_v.shape[2]
    n_heads = w_v.shape[0] // 3
    n_groups = Dm // GC
    n_blocks = n_seg * seg // T
    L = n_mem + seg
    n_tiles = 3 * n_heads // HT
    n_dc = Dm // DC
    n_rb = n_seg * PRE // RB
    n_pre = pre_v.shape[0]

    zero = zero_ref[0]
    never = zero != 0

    def w_copies(c):
        i, tile = divmod(c, n_heads // HT)
        rows = [pl.ds(r, Dm * HT // 4) for r in range(0, Dm * HT, Dm * HT // 4)]
        return [pltpu.make_async_copy((wq_hbm, wk_hbm, wv_hbm)[i].at[r, pl.ds(tile * Dh, Dh)],
                                      stage_v.at[c % N_SLOTS, r, :], sem_w.at[c % N_SLOTS]) for r in rows]

    def wo_copy(j):
        return pltpu.make_async_copy(wo_hbm.at[:, pl.ds(128 * j, 128)], wo_v.at[j].bitcast(BF16), sem_wo)

    def x_copy(j):
        r = pl.ds(j * (n_seg // n_groups), n_seg // n_groups)
        return pltpu.make_async_copy(x_hbm.at[r], x_v.at[r], sem_x)

    def group_copies(g):
        ch = pl.ds(g * GC, GC)
        return [pltpu.make_async_copy(p.at[ch, :], par_v.at[i, ch, :], sem_g.at[g])
                for i, p in enumerate((are_hbm, aim_hbm, bre_hbm, bim_hbm, cre_hbm, cim_hbm))] + [
                    pltpu.make_async_copy(u_hbm.at[:, ch], u_v.at[g], sem_g.at[g])]

    def outb_copy(g):
        return pltpu.make_async_copy(outb_v.at[g], out_hbm.at[:, pl.ds(Dm + g * GC, GC)], sem_ob)

    def outa_copy(it):
        r = pl.ds(pl.multiple_of(it * UNROLL * seg, seg), UNROLL * seg)
        return pltpu.make_async_copy(outa_v.at[r, :], out_hbm.at[r, pl.ds(0, Dm)], sem_oa)

    xt_copy = pltpu.make_async_copy(x_hbm.at[:, pl.ds(seg - PRE, PRE), :], xt_v, sem_xt)
    small = [pltpu.make_async_copy(src, dst, sem_s.at[i]) for i, (src, dst) in
             enumerate(((ldt_hbm, ldt_v), (dsk_hbm, dsk_v), (mem0_hbm, mem0_v)))]

    def relayout(piece):
        c, pc = divmod(piece, n_dc)
        src = stage_v.at[c % N_SLOTS].bitcast(U32)
        rows = slice(pc * DC // 2, (pc + 1) * DC // 2)
        done = []
        for pp in range(HT // 2):
            ev = src[pl.ds(pc * DC * HT // 2 + pp, DC // 2, stride=HT), :]
            od = src[pl.ds(pc * DC * HT // 2 + pp + HT // 2, DC // 2, stride=HT), :]
            done += [(ev & 0xFFFF) | (od << 16), (ev >> 16) | (od & jnp.uint32(0xFFFF0000))]
            w_v[c * HT + 2 * pp, rows, :] = done[-2]
            w_v[c * HT + 2 * pp + 1, rows, :] = done[-1]
        return [lax.bitcast_convert_type(v, F32) for v in done]

    def ahead(unit, size, after):
        m, rb = divmod(unit, n_rb)
        rows = slice(rb * RB, (rb + size) * RB)
        lhs = xp_v[rows, :]
        if after is not None:
            corner = jnp.where(never, after, lhs[:8, :128])
            lhs = jnp.concatenate([jnp.concatenate([corner, lhs[:8, 128:]], axis=1), lhs[8:]], axis=0)
        res = _dot(lhs, pltpu.bitcast(w_v[m], BF16))
        pre_v[m, rows, :] = res
        return res[-8:]

    progress = {"piece": 0, "unit": 0, "stage": 0}

    def filler(n_units, size, n_pieces):
        p0 = progress["piece"]
        p1 = min(p0 + n_pieces, n_tiles * n_dc)
        u0 = progress["unit"]
        u1 = min(u0 + n_units, p0 // n_dc * HT * n_rb, n_pre * n_rb)
        progress.update(piece=p1, unit=u1)
        assert u0 % size == 0 and u1 % size == 0
        todo_p, todo_u = list(range(p0, p1)), list(range(u0, u1, size))
        pending, issued = [], []

        def fill(done, total, after=()):
            pending.extend(after)
            while todo_u and (todo_u[0] - u0) * total <= done * (u1 - u0):
                rows = [v[r:r + 8] for v in pending for r in range(0, v.shape[0], 8)]
                issued.append(ahead(todo_u.pop(0), size, functools.reduce(jnp.add, rows) if rows else None))
                pending.clear()
            while todo_p and (todo_p[0] - p0) * total <= done * (p1 - p0 + 1):
                pending.extend(relayout(todo_p.pop(0)))
            return issued

        return fill

    def stage(*parts):
        p0 = progress["piece"]
        fills = [filler(*part[1:]) for part in parts]
        p1 = progress["piece"]
        for c in range(-(-p0 // n_dc), -(-p1 // n_dc)):
            _wait(w_copies(c))

        progress["stage"] += 1

        @pl.when(zero < progress["stage"])
        def _():
            for part, fill in zip(parts, fills):
                part[0](fill)
                fill(1, 1)

        for c in range(p0 // n_dc, p1 // n_dc):
            if c and c + N_SLOTS < n_tiles:
                _start(w_copies(c + N_SLOTS))

    def chan(k):
        return slice(k * PITCH, k * PITCH + n_blocks)

    def states(k):
        return slice(k * SPITCH, k * SPITCH + 2 * n_blocks)

    def ssm_group(g0, nb):
        n_ch = nb * GC

        def prepare(fill):
            done = [(), (), ()]
            for b in range(nb):
                g = g0 + b
                dt = jnp.exp(ldt_v[g * GC:(g + 1) * GC].astype(F32).reshape(1, GC)).astype(BF16).astype(F32)
                dt = jnp.broadcast_to(dt, (GC, GC)).T
                for c in range(n_blocks):
                    issued = fill(b * n_blocks + c, nb * n_blocks, done.pop(0))
                    ub = u_v[g, c * T:(c + 1) * T, :].astype(F32)
                    plain, flipped = ub.T, _reverse_chunks(ub).astype(BF16).T.astype(F32)
                    uf_v[pl.ds(b * GC * PITCH + c, GC, stride=PITCH), :] = plain
                    ur_v[pl.ds(b * GC * PITCH + c, GC, stride=PITCH), :] = flipped
                    done.append((plain[-8:], flipped[-8:]))
                    for d0 in range(c * GC // n_blocks, (c + 1) * GC // n_blocks, PB):
                        k0 = b * GC + d0
                        a_re, a_im, b_re, b_im, c_re, c_im = (
                            par_v[i, g * GC + d0:g * GC + d0 + PB, :].astype(F32) for i in range(6))
                        step = dt[d0:d0 + PB]
                        if len(issued) > 1:
                            step = jnp.where(never, issued[-2], step)
                        w_re, w_im = _cmul(c_re, c_im, step * b_re, step * b_im)
                        mag = jnp.exp(step * a_re)
                        l1 = (mag * jnp.cos(step * a_im), mag * jnp.sin(step * a_im))
                        l2 = _cmul(*l1, *l1)
                        l3 = _cmul(*l2, *l1)
                        l4 = _cmul(*l2, *l2)
                        pw = [(jnp.ones_like(mag), jnp.zeros_like(mag)), l1, l2, l3, l4,
                              _cmul(*l4, *l1), _cmul(*l4, *l2), _cmul(*l4, *l3)]
                        for r in range(8):
                            bre_v[pl.ds(k0 * BPITCH + r, PB, stride=BPITCH), :] = pw[r][0]
                            bim_v[pl.ds(k0 * BPITCH + r, PB, stride=BPITCH), :] = pw[r][1]
                        l8 = _cmul(*l4, *l4)
                        lt = l8
                        for _ in range(3):
                            lt = _cmul(*lt, *lt)
                        wl = _cmul(w_re, w_im, *l1)
                        for i, val in enumerate((lt[0], -lt[1], wl[0], wl[1], w_re, -w_im, *l8)):
                            cf_v[i, k0:k0 + PB, :] = val
                        done[-1] += (*pw[5], *pw[6], *pw[7], *lt, *wl)

        def read_in(fill):
            even = lax.broadcasted_iota(jnp.int32, (n_blocks, T), 1) < TC
            for k in range(n_ch):
                if k % 2 == 0:
                    fill(k, n_ch)
                pr = [bre_v[k * BPITCH:k * BPITCH + 8, :]]
                pi = [bim_v[k * BPITCH:k * BPITCH + 8, :]]
                mr = jnp.broadcast_to(cf_v[6, k:k + 1, :], (8, 128))
                mi = jnp.broadcast_to(cf_v[7, k:k + 1, :], (8, 128))
                for _ in range(TC // 8 - 1):
                    nr, ni = _cmul(pr[-1], pi[-1], mr, mi)
                    pr.append(nr)
                    pi.append(ni)
                p_v[k] = jnp.concatenate(
                    [jnp.concatenate(pr, axis=0), jnp.concatenate(pi, axis=0)], axis=1).astype(BF16)
                ur = ur_v[chan(k), :]
                ur = jnp.concatenate([jnp.where(even, ur, 0.0), jnp.where(even, 0.0, ur)], axis=0)
                sre_v[states(k), :] = _dot(ur, jnp.concatenate(pr + pr, axis=0).astype(BF16))
                sim_v[states(k), :] = _dot(ur, jnp.concatenate(pi + pi, axis=0).astype(BF16))

        def scan(k0, width, last):
            ltr, lti, wlr, wli, gr, gi = (cf_v[i, k0:k0 + width, :] for i in range(6))
            if last is not None:
                wlr, wli = jnp.where(never, last, wlr), jnp.where(never, last, wli)
            nwlr = -wlr
            for c in range(2 * n_blocks):
                idx = pl.ds(k0 * SPITCH + (c % 2) * n_blocks + c // 2, width, stride=SPITCH)
                gre_v[idx, :] = gr
                gim_v[idx, :] = gi
                if c < 2 * n_blocks - 1:
                    xr, xi = sre_v[idx, :], sim_v[idx, :]
                    sr, si = wlr * xr - wli * xi, nwlr * xi - wli * xr
                    if c == 0:
                        gr, gi = sr, si
                    else:
                        gr, gi = _cmul(gr, gi, ltr, lti)
                        gr, gi = gr + sr, gi + si
            return gr

        def read_out(fill):
            has_state = lax.broadcasted_iota(jnp.int32, (n_blocks, T), 0) > 0
            width = 8 if g0 else 16
            lag = 2 * width
            last = None
            for k0 in range(0, n_ch + lag, width):
                if k0 < n_ch:
                    last = scan(k0, width, last)
                for k in range(k0 - lag, k0 - lag + width):
                    if k % 2 == 0:
                        fill(k + lag, n_ch + lag + 8)
                    if k < 0:
                        continue
                    gg = jnp.concatenate([gre_v[states(k), :], gim_v[states(k), :]], axis=1)
                    p = p_v[k]
                    y = _dot(gg, jnp.concatenate([p, jnp.zeros_like(p)], axis=0), NT)
                    taps_v[8 * k:8 * k + 8, :] = y[0:8, :] + pltpu.roll(y[0:8, :], TC, 1)
                    y_v[chan(k), :] = (jnp.where(has_state, y[:n_blocks], 0.0)
                                       + pltpu.roll(y[n_blocks:], TC, 1))

        def in_chunk(fill):
            ti = lax.broadcasted_iota(jnp.int32, (TC, T), 0)
            tj = lax.broadcasted_iota(jnp.int32, (TC, T), 1)
            causal_even = (tj >= ti) & (tj < TC)
            causal_odd = tj >= ti + TC
            for k in range(n_ch):
                if k % 2 == 0:
                    fill(k, n_ch)
                kb = jnp.broadcast_to(taps_v[8 * k:8 * k + 1, :], (TC, T))
                tz = pltpu.roll(kb, 0, 1, stride=1, stride_axis=0)
                tz = jnp.concatenate([jnp.where(causal_even, tz, 0.0),
                                      jnp.where(causal_odd, tz, 0.0)], axis=0)
                y_v[chan(k), :] += _dot(uf_v[chan(k), :], tz.astype(BF16))

        def finish(fill):
            done = [(), ()]
            for b in range(nb):
                g = g0 + b
                dsk = dsk_v[g * GC:(g + 1) * GC].astype(F32).reshape(1, GC)
                for c in range(n_blocks):
                    fill(b * n_blocks + c, nb * n_blocks, done.pop(0))
                    rows = slice(c * T, (c + 1) * T)
                    yc = y_v[pl.ds(b * GC * PITCH + c, GC, stride=PITCH), :].T.astype(BF16).astype(F32)
                    yc = yc + (u_v[g, rows, :].astype(F32) * dsk).astype(BF16).astype(F32)
                    outb_v[g, rows, :] = yc.astype(BF16)
                    done.append((yc,))

        return ((prepare, 20 * nb, 1, n_dc if g0 == 1 else 0),
                (read_in, 16 * nb, 1, n_dc if g0 == 1 and nb > 1 else 0),
                (read_out, 16 * nb, 2, 0),
                (in_chunk, 26 * nb, 2, nb * n_tiles * n_dc // n_groups if g0 else 0),
                (finish, 8 * nb if g0 + nb < n_groups else n_pre * n_rb, 2, 0))

    def widen(fill):
        for s in range(n_seg):
            xp_v[s * PRE:(s + 1) * PRE, :] = xt_v[s].astype(F32)

    _start(small + group_copies(0))
    _wait(small)
    _start(w_copies(0) + [xt_copy])
    _wait(group_copies(0))
    leftover = ()
    late = [make(j) for j in range(n_groups) for make in (wo_copy, x_copy)]
    for i, nb in enumerate(GROUPS):
        g0 = sum(GROUPS[:i])
        following = [cp for g in range(g0 + nb, sum(GROUPS[:i + 2])) for cp in group_copies(g)]
        prepare, read_in, read_out, in_chunk, finish = ssm_group(g0, nb)
        if i:
            _start(following)
        if i > 1:
            _start(late[:4 * nb])
            late = late[4 * nb:]
        stage(*leftover, prepare)
        if i == 1:
            _start(w_copies(N_SLOTS))
        stage(read_in)
        if i == 0:
            _start(following)
        stage(read_out)
        if i == 0:
            xt_copy.wait()
            _start(w_copies(1))
            stage((widen, 0, 1, n_dc))
            for c in range(2, N_SLOTS):
                _start(w_copies(c))
        stage(in_chunk)
        if 0 < i < len(GROUPS) - 1:
            leftover = (finish,)
        else:
            stage(finish)
        _wait(following)
    assert not late
    assert (progress["piece"], progress["unit"]) == (n_tiles * n_dc, n_pre * n_rb)
    _wait([make(j) for j in range(n_groups) for make in (x_copy, wo_copy)])
    _start([outb_copy(g) for g in range(n_groups)])

    scale = Dh ** -0.5
    qi = lax.broadcasted_iota(jnp.int32, (L, 128), 0)
    ki = lax.broadcasted_iota(jnp.int32, (L, 128), 1)
    keep = ((qi < n_mem) | (qi >= ki)) & (ki < L)
    masked = jnp.where(ki < L, -1000000000.0 / scale, -jnp.inf)
    zpad = jnp.zeros((128 - L, Dh), F32)
    n_og = n_heads // HG
    heads = [h % AG * (n_heads // AG) + h // AG for h in range(n_heads)]

    def step(s, cur, nxt):
        r = pl.ds(pl.multiple_of(s * seg, seg), seg)
        qs, ks, vs, es, os_, acc = {}, {}, {}, {}, {}, {}

        def proj(i, h):
            m = i * n_heads + h
            w = pltpu.bitcast(w_v[m], BF16)
            if m >= n_pre:
                return _dot(h_v[cur], w)
            known = pre_v[m, pl.ds(pl.multiple_of(s * PRE, PRE), PRE), :]
            return jnp.concatenate([_dot(h_v[cur, :L - PRE, :], w), known], axis=0)

        def scores(h):
            sc = jnp.where(keep, _dot(qs.pop(h), ks.pop(h), NT), masked)
            e = jnp.exp2((sc - jnp.max(sc, axis=1, keepdims=True)) * (scale * LOG2E))
            total = jnp.sum(e, axis=1, keepdims=True)
            inv = pl.reciprocal(total, approx=True)
            es[h] = (e, inv * (2.0 - total * inv))

        def mix(h):
            e, inv = es.pop(h)
            os_[h] = _dot(e, vs.pop(h)) * inv

        def oproj(j, g):
            hs = heads[g * HG:(g + 1) * HG]
            w = jnp.concatenate([wo_v[j, h * Dh // 2:(h + 1) * Dh // 2, :] for h in hs], axis=0)
            return _dot(jnp.concatenate([os_[h] for h in hs], axis=1), pltpu.bitcast(w, BF16))

        early = [divmod(t, n_og - 1) for t in range(Dm // 128 * (n_og - 1))]

        def oproj_early(count):
            for _ in range(count):
                j, g = early.pop(0)
                acc[j] = acc[j] + oproj(j, g) if g else oproj(j, g)

        for h0 in range(0, n_heads, AG):
            before = heads[max(h0 - AG, 0):h0]
            if h0 == 2 * AG:
                h_v[nxt, n_mem:, :] = x_v[jnp.minimum(s + 1, n_seg - 1)].astype(F32)
            for i, h in enumerate(heads[h0:h0 + AG]):
                qs[h] = proj(0, h)
                if i == AG - 2:
                    for hh in before:
                        scores(hh)
                ks[h] = jnp.concatenate([proj(1, h), zpad], axis=0).astype(BF16)
                if i == AG - 1:
                    for hh in before:
                        mix(hh)
                vs[h] = jnp.concatenate([proj(2, h), zpad], axis=0).astype(BF16)

        oproj_early(3)
        for hh in heads[n_heads - AG:]:
            scores(hh)
        oproj_early(7)
        for hh in heads[n_heads - AG:]:
            mix(hh)
        oproj_early(3)
        for j in range(Dm // 128):
            oproj_early(sum(jj <= j for jj, _ in early))
            res = acc.pop(j) + oproj(j, n_og - 1)
            h_v[nxt, :n_mem, 128 * j:128 * (j + 1)] = res[:n_mem]
            outa_v[r, 128 * j:128 * (j + 1)] = res[n_mem:].astype(BF16)

    def steps(it, carry):
        for c in range(UNROLL):
            step(it * UNROLL + c, c, (c + 1) % UNROLL)
        outa_copy(it).start()
        return carry

    h_v[0, :n_mem, :] = mem0_v[...].astype(F32)
    h_v[0, n_mem:, :] = x_v[0].astype(F32)
    lax.fori_loop(0, n_seg // UNROLL, steps, 0)

    def drain(it, carry):
        outa_copy(it).wait()
        return carry

    _wait([outb_copy(g) for g in range(n_groups)])
    lax.fori_loop(0, n_seg // UNROLL, drain, 0)


@functools.partial(jax.jit, static_argnames=("A_seg_len",))
def pallas_concat_heads__memory_aug_recurrent_mem_tr__ssm_conv_s4__prompt_kernel(
    A_x: jax.Array,
    A_mem0: jax.Array,
    A_Wq: jax.Array,
    A_Wk: jax.Array,
    A_Wv: jax.Array,
    A_Wo: jax.Array,
    A_seg_len: int,
    B_u: jax.Array,
    B_A_re: jax.Array,
    B_A_im: jax.Array,
    B_B_re: jax.Array,
    B_B_im: jax.Array,
    B_C_re: jax.Array,
    B_C_im: jax.Array,
    B_log_dt: jax.Array,
    B_Dskip: jax.Array,
):
    Bsz, S, Dm = A_x.shape
    H, Dh = A_Wq.shape[1], A_Wq.shape[2]
    M = A_mem0.shape[1]
    D, N = B_A_re.shape
    seg = int(A_seg_len)
    n_seg = S // seg
    n_groups = D // GC
    assert Bsz == 1 and Dh == 128 and N == 128 and D == Dm and B_u.shape == A_x.shape
    assert n_seg % UNROLL == 0 and M + seg <= 128 and sum(GROUPS) == n_groups
    n_pre = 2 * H + H // 2

    def head_tiles(w):
        return w.reshape(Dm, H // HT, HT, Dh).transpose(0, 2, 1, 3).reshape(Dm * HT, H // HT * Dh)

    n_ch = max(GROUPS) * GC

    def pitched(pitch):
        return pltpu.VMEM(((n_ch + 8) * pitch, N), F32)

    any_spec = pl.BlockSpec(memory_space=pl.ANY)
    out = pl.pallas_call(
        _kernel,
        out_shape=jax.ShapeDtypeStruct((S, Dm + D), BF16),
        in_specs=[pl.BlockSpec(memory_space=pltpu.SMEM)] + [any_spec] * 15,
        out_specs=any_spec,
        scratch_shapes=[
            pltpu.VMEM((n_seg, seg, Dm), BF16),
            pltpu.VMEM((n_seg, PRE, Dm), BF16),
            pltpu.VMEM((n_seg * PRE, Dm), F32),
            pltpu.VMEM((n_groups, S, GC), BF16),
            pltpu.VMEM((6, D, N), BF16),
            pltpu.VMEM((N_SLOTS, Dm * HT + 32, Dh), BF16),
            pltpu.VMEM((3 * H, Dm // 2, Dh), U32),
            pltpu.VMEM((Dm // 128, H * Dh // 2, 128), U32),
            pltpu.VMEM((n_pre, n_seg * PRE, Dh), F32),
            pltpu.VMEM((S, Dm), BF16),
            pltpu.VMEM((n_groups, S, GC), BF16),
            pltpu.VMEM((UNROLL, M + seg, Dm), F32),
            pitched(BPITCH), pitched(BPITCH),
            pltpu.VMEM((8, n_ch, N), F32),
            pltpu.VMEM((n_ch, TC, 2 * N), BF16),
            pitched(PITCH), pitched(PITCH),
            pitched(SPITCH), pitched(SPITCH),
            pitched(SPITCH), pitched(SPITCH),
            pitched(PITCH),
            pltpu.VMEM((n_ch * 8, T), F32),
            pltpu.VMEM((M, Dm), BF16),
            pltpu.VMEM((D,), BF16),
            pltpu.VMEM((D,), BF16),
            pltpu.SemaphoreType.DMA((3,)),
            pltpu.SemaphoreType.DMA(()),
            pltpu.SemaphoreType.DMA(()),
            pltpu.SemaphoreType.DMA((n_groups,)),
            pltpu.SemaphoreType.DMA((N_SLOTS,)),
            pltpu.SemaphoreType.DMA(()),
            pltpu.SemaphoreType.DMA(()),
            pltpu.SemaphoreType.DMA(()),
        ],
        compiler_params=pltpu.CompilerParams(
            vmem_limit_bytes=124 * 1024 * 1024, disable_bounds_checks=True),
    )(np.zeros((1,), np.int32), A_x.reshape(n_seg, seg, Dm), A_mem0.reshape(M, Dm),
      head_tiles(A_Wq), head_tiles(A_Wk), head_tiles(A_Wv), A_Wo.reshape(H * Dh, Dm),
      B_u.reshape(S, D), B_A_re, B_A_im, B_B_re, B_B_im, B_C_re, B_C_im, B_log_dt, B_Dskip)
    return out.reshape(Bsz, S, Dm + D)
```
